```python
import jax
import jax.numpy as jnp

def _softmax(x, axis=-1):
    return jax.nn.softmax(x, axis=axis)

def _gelu(x):
    return jax.nn.gelu(x, approximate=True)

def _silu(x):
    return jax.nn.silu(x)

def _sigmoid(x):
    return jax.nn.sigmoid(x)

def _layernorm(x, axis=-1, eps=1e-05):
    m = jnp.mean(x, axis=axis, keepdims=True)
    v = jnp.var(x, axis=axis, keepdims=True)
    return (x - m) / jnp.sqrt(v + eps)

def _scatter_add(tgt, idx, src, axis=0):
    return tgt.at[idx].add(src)

def _segment_sum(src, seg, n):
    return jax.ops.segment_sum(src, seg, n)

class _Rng:

    def __init__(self, key):
        self._k = key

    def _next(self):
        self._k, sub = jax.random.split(self._k)
        return sub

    def normal(self, shape):
        return jax.random.normal(self._next(), shape, dtype=jnp.bfloat16)

    def randint(self, lo, hi, shape):
        return jax.random.randint(self._next(), shape, lo, hi, dtype=jnp.int32)

    def uniform(self, shape, lo=0.0, hi=1.0):
        return jax.random.uniform(self._next(), shape, jnp.bfloat16, lo, hi)

    def permutation(self, n):
        return jax.random.permutation(self._next(), n)
kernel_name = 'sequential_preLN__ssm_conv_s4__mixer_gmlp__prompt'

def _fwd_setup_inputs():
    _rng = _Rng(jax.random.key(int.from_bytes(__import__("os").urandom(4), "little")))
    _w = lambda a: (lambda t: t.astype(jnp.bfloat16) if jnp.issubdtype(t.dtype, jnp.floating) else t)(jnp.asarray(a))

    def _A_setup():
        B, L, D, N = (1, 2048, 576, 128)
        A_re = -jnp.exp((lambda *s: _rng.normal(s) * 0.05)(D, N))
        A_im = jnp.pi * (lambda *s: _rng.normal(s) * 0.05)(D, N)
        B_re = (lambda *s: _rng.normal(s) * 0.05)(D, N)
        B_im = (lambda *s: _rng.normal(s) * 0.05)(D, N)
        C_re = (lambda *s: _rng.normal(s) * 0.05)(D, N)
        C_im = (lambda *s: _rng.normal(s) * 0.05)(D, N)
        log_dt = (lambda *s: _rng.normal(s) * 0.05)(D) * 0.5 - 4.0
        Dskip = (lambda *s: _rng.normal(s) * 0.05)(D)
        return {'u': _w((lambda *s: _rng.normal(s) * 0.05)(B, L, D)), 'A_re': _w(A_re), 'A_im': _w(A_im), 'B_re': _w(B_re), 'B_im': _w(B_im), 'C_re': _w(C_re), 'C_im': _w(C_im), 'log_dt': _w(log_dt), 'Dskip': _w(Dskip)}
    _A_in = _A_setup()

    def _B_setup():
        B, S, D, F = (1, 2048, 576, 4608)
        Fh = F // 2
        return {'x': _w((lambda *s: _rng.normal(s) * 0.05)(B, S, D)), 'w_in': _w((lambda *s: _rng.normal(s) * 0.05)(D, 2 * Fh)), 'w_sp': _w(0.01 * (lambda *s: _rng.normal(s) * 0.05)(S, S)), 'b_sp': _w(1.0 + 0.01 * (lambda *s: _rng.normal(s) * 0.05)(S)), 'w_out': _w((lambda *s: _rng.normal(s) * 0.05)(Fh, D))}
    _B_in = _B_setup()
    return {'A_u': _A_in['u'], 'A_A_re': _A_in['A_re'], 'A_A_im': _A_in['A_im'], 'A_B_re': _A_in['B_re'], 'A_B_im': _A_in['B_im'], 'A_C_re': _A_in['C_re'], 'A_C_im': _A_in['C_im'], 'A_log_dt': _A_in['log_dt'], 'A_Dskip': _A_in['Dskip'], 'B_x': _B_in['x'], 'B_w_in': _B_in['w_in'], 'B_w_sp': _B_in['w_sp'], 'B_b_sp': _B_in['b_sp'], 'B_w_out': _B_in['w_out']}

def _fwd_reference(A_u, A_A_re, A_A_im, A_B_re, A_B_im, A_C_re, A_C_im, A_log_dt, A_Dskip, B_x, B_w_in, B_w_sp, B_b_sp, B_w_out):

    def _A_ref(u, A_re, A_im, B_re, B_im, C_re, C_im, log_dt, Dskip):
        Bsz, L, D = u.shape
        dt = jnp.exp(log_dt)[:, None]
        A = A_re + 1j * A_im
        Bc = B_re + 1j * B_im
        Cc = C_re + 1j * C_im
        logdA = dt * A
        dB = dt * Bc
        l = (lambda x, dt: x.astype(dt))(jnp.arange(L), A_re.dtype)
        P = jnp.exp(logdA[:, :, None] * l[None, None, :])
        K = jnp.einsum('dn,dnl,dn->dl', Cc, P, dB).real
        L2 = 2 * L
        Kp = jnp.pad(K, ((0, 0), (0, L)))
        up = (lambda x, *d: x.transpose(*d))(u, 0, 2, 1)
        up = jnp.pad(up, ((0, 0), (0, 0), (0, L)))
        Kf = (lambda x, axes=(-2, -1): jnp.fft.rfft2(x.astype(jnp.float32), axes=axes))(Kp[:, None, :], axes=(-2, -1))
        Uf = (lambda x, axes=(-2, -1): jnp.fft.rfft2(x.astype(jnp.float32), axes=axes))(up[:, :, None, :], axes=(-2, -1))
        Yf = Uf * Kf[None, :, :, :]
        y = (lambda x, s, axes=(-2, -1): jnp.fft.irfft2(x, s=s, axes=axes).astype(jnp.bfloat16))(Yf, (1, L2), axes=(-2, -1))[:, :, 0, :L]
        y = (lambda x, *d: x.transpose(*d))(y, 0, 2, 1) + u * Dskip[None, None, :]
        return y

    def _B_ref(x, w_in, w_sp, b_sp, w_out):
        B, S, D = x.shape
        F = w_in.shape[-1]
        Fh = F // 2
        z = _gelu(jnp.einsum('bsd,df->bsf', x, w_in))
        z1 = z[..., :Fh].copy()
        z2 = _layernorm(z[..., Fh:], axis=-1)
        g = jnp.einsum('ts,bsf->btf', w_sp, z2) + b_sp[None, :, None]
        return jnp.einsum('bsf,fd->bsd', z1 * g, w_out)
    x = A_u
    h = x + _A_ref(_layernorm(x, axis=-1), A_A_re, A_A_im, A_B_re, A_B_im, A_C_re, A_C_im, A_log_dt, A_Dskip)
    h2 = h + _B_ref(_layernorm(h, axis=-1), B_w_in, B_w_sp, B_b_sp, B_w_out)
    return h2

def setup_inputs():
    _inp = _fwd_setup_inputs()
    _gk = jax.random.fold_in(jax.random.key(int.from_bytes(__import__("os").urandom(4), "little")), 2 ** 31 - 1)
    _shapes = [[1, 2048, 576]]
    _dtypes = ['bfloat16']
    _gks = jax.random.split(_gk, len(_shapes))
    _gs = [jax.random.normal(k, s, dtype=jnp.dtype(d)) * 0.05 for k, s, d in zip(_gks, _shapes, _dtypes)]
    _inp['grad_out'] = _gs[0]
    return _inp

def reference(A_u, A_A_re, A_A_im, A_B_re, A_B_im, A_C_re, A_C_im, A_log_dt, A_Dskip, B_w_in, B_w_sp, B_b_sp, B_w_out, B_x, grad_out):
    _const = dict(B_x=B_x)

    def _f(*_d):
        return _fwd_reference(**{'A_u': _d[0], 'A_A_re': _d[1], 'A_A_im': _d[2], 'A_B_re': _d[3], 'A_B_im': _d[4], 'A_C_re': _d[5], 'A_C_im': _d[6], 'A_log_dt': _d[7], 'A_Dskip': _d[8], 'B_w_in': _d[9], 'B_w_sp': _d[10], 'B_b_sp': _d[11], 'B_w_out': _d[12], **_const})
    _out, _vjp = jax.vjp(_f, A_u, A_A_re, A_A_im, A_B_re, A_B_im, A_C_re, A_C_im, A_log_dt, A_Dskip, B_w_in, B_w_sp, B_b_sp, B_w_out)
    _grads = _vjp(grad_out)
    _out0 = jnp.asarray(_out)
    return (_out0, *[jnp.asarray(_g) for _g in _grads])
```

```python
import functools
import math

import jax
import jax.numpy as jnp
from jax import lax
import jax.experimental.pallas as pl
import jax.experimental.pallas.tpu as pltpu

F32 = jnp.float32
BF = jnp.bfloat16
L = 2048
D = 576
DP = 640
N = 128
FH = 2304
FF = 4608
NJ = 768
TM = 256
NT = L // TM
GC = math.sqrt(2.0 / math.pi)


def _dot(a, b):
    return jnp.dot(a, b, preferred_element_type=F32)


def _dot_nt(a, b):
    return lax.dot_general(a, b, (((1,), (1,)), ((), ())), preferred_element_type=F32)


def _dot_tn(a, b):
    return lax.dot_general(a, b, (((0,), (0,)), ((), ())), preferred_element_type=F32)


def _ln(x):
    m = jnp.mean(x, axis=-1, keepdims=True)
    c = x - m
    v = jnp.mean(c * c, axis=-1, keepdims=True)
    r = lax.rsqrt(v + 1e-5)
    return c * r, r


def _lnb(dy, y, r):
    return r * (dy - jnp.mean(dy, axis=-1, keepdims=True)
                - y * jnp.mean(dy * y, axis=-1, keepdims=True))


def _gelu(a):
    t = jnp.tanh(GC * (a + 0.044715 * a * a * a))
    return 0.5 * a * (1.0 + t)


def _dgelu(a):
    t = jnp.tanh(GC * (a + 0.044715 * a * a * a))
    return 0.5 * (1.0 + t) + 0.5 * a * (1.0 - t * t) * GC * (1.0 + 3 * 0.044715 * a * a)


def _rows(i, t=TM):
    return pl.ds(pl.multiple_of(i * t, t), t)


def _gen_dft(f_ref):
    def body(ch_ref, sh_ref):
        s2 = 2 * lax.broadcasted_iota(jnp.int32, (256, L), 1) + 1
        k1 = lax.broadcasted_iota(jnp.int32, (256, L), 0)
        ang = ((s2 * (16 * k1)) & 16383).astype(F32) * (math.pi / 8192.0)
        ch_ref[...] = jnp.cos(ang)
        sh_ref[...] = jnp.sin(ang)
        s2l = 2 * lax.broadcasted_iota(jnp.int32, (8, L), 1) + 1
        k0 = lax.broadcasted_iota(jnp.int32, (8, L), 0)
        angl = ((s2l * (2 * k0 + 1)) & 16383).astype(F32) * (math.pi / 8192.0)
        cl = jnp.cos(angl)
        sl = jnp.sin(angl)

        def step(i, carry):
            cs, ss = [], []
            for r in range(2):
                ch = ch_ref[pl.ds(2 * i + r, 1), :]
                sh = sh_ref[pl.ds(2 * i + r, 1), :]
                cs.append(ch * cl - sh * sl)
                ss.append(-(sh * cl + ch * sl))
            f_ref[pl.ds(pl.multiple_of(i * 16, 16), 16), :] = jnp.concatenate(cs, 0).astype(BF)
            f_ref[pl.ds(pl.multiple_of(L + i * 16, 16), 16), :] = jnp.concatenate(ss, 0).astype(BF)
            return carry
        lax.fori_loop(0, 128, step, 0)
    pl.run_scoped(body, pltpu.VMEM((256, L), F32), pltpu.VMEM((256, L), F32))


def _lval(j):
    return jnp.where(j <= 256, j,
                     jnp.where(j <= 384, 256 + 2 * (j - 256),
                               jnp.where(j <= 512, 512 + 4 * (j - 384),
                                         jnp.where(j <= 640, 1024 + 8 * (j - 512), -1)))).astype(F32)


def _phase(i0, n):
    k = lax.broadcasted_iota(jnp.int32, (n, 1), 0) + i0
    ph = (2 * k + 1).astype(F32) * (math.pi / 8192.0)
    return jnp.cos(ph), jnp.sin(ph)


SEGS = ((0, 32, 0), (32, 48, 1), (48, 64, 2), (64, 81, 3))


def _kernel(x_ref, do_ref, are_ref, aim_ref, bre_ref, bim_ref, cre_ref, cim_ref,
            ldt_ref, dsk_ref, win_ref, wsp_ref, bsp_ref, wout_ref,
            out_ref, dx_ref, dare_ref, daim_ref, dbre_ref, dbim_ref, dcre_ref, dcim_ref,
            dldt_ref, ddsk_ref, dwin_ref, dwsp_ref, dbsp_ref, dwout_ref,
            uf_ref, kf_ref, h_ref, mul_ref, gp_ref):
    dsk = dsk_ref[...].astype(F32)
    dt = jnp.exp(ldt_ref[...].astype(F32)).astype(BF).astype(F32)
    lar = dt * are_ref[...].astype(F32)
    lai = dt * aim_ref[...].astype(F32)
    for p in range(4):
        e = jnp.exp(lar * (2.0 ** p))
        mul_ref[p, 0] = e * jnp.cos(lai * (2.0 ** p))
        mul_ref[p, 1] = e * jnp.sin(lai * (2.0 ** p))

    def ln_x(i, c):
        r = _rows(i)
        u, _ = _ln(x_ref[r, :].astype(F32))
        dx_ref[r, :] = u.astype(BF)
        return c
    lax.fori_loop(0, NT, ln_x, 0)

    def s4_fwd(f_ref, kp_ref, k_ref, z_ref):
        _gen_dft(f_ref)
        kp_ref[...] = jnp.zeros(kp_ref.shape, F32)

        def chunk(c, cc):
            ns = pl.ds(pl.multiple_of((c % 2) * 64, 64), 64)
            ds_ = pl.ds(pl.multiple_of((c // 2) * 128, 128), 128)
            dtc = jnp.exp(ldt_ref[:, ds_].astype(F32)).astype(BF).astype(F32)
            br = dtc * bre_ref[ns, ds_].astype(F32)
            bi = dtc * bim_ref[ns, ds_].astype(F32)
            cr = cre_ref[ns, ds_].astype(F32)
            ci = cim_ref[ns, ds_].astype(F32)
            pr = cr * br - ci * bi
            pi_ = cr * bi + ci * br
            for (j0, j1, p) in SEGS:
                mr = mul_ref[p, 0, ns, ds_]
                mi = mul_ref[p, 1, ns, ds_]

                def step(j, carry):
                    pr, pi_ = carry
                    rows = []
                    for _ in range(8):
                        rows.append(jnp.sum(pr, axis=0, keepdims=True))
                        pr, pi_ = pr * mr - pi_ * mi, pr * mi + pi_ * mr
                    js = pl.ds(pl.multiple_of(j * 8, 8), 8)
                    kp_ref[c // 2, js, :] = kp_ref[c // 2, js, :] + jnp.concatenate(rows, 0)
                    return pr, pi_
                pr, pi_ = lax.fori_loop(j0, j1, step, (pr, pi_))
            return cc
        lax.fori_loop(0, 10, chunk, 0)

        kpb = jnp.concatenate([kp_ref[c] for c in range(5)], 1)[:, :D].astype(BF)
        lj = _lval(lax.broadcasted_iota(jnp.int32, (TM, NJ), 1))

        def expand(i, c):
            lr = (lax.broadcasted_iota(jnp.int32, (TM, NJ), 0) + i * TM).astype(F32)
            m = (lr.astype(BF).astype(F32) == lj).astype(BF)
            k_ref[_rows(i), :] = _dot(m, kpb).astype(BF)
            return c
        lax.fori_loop(0, NT, expand, 0)

        def fwd_dft(i, c):
            r = _rows(i)
            f = f_ref[r, :]
            uf_ref[r, :] = _dot(f, dx_ref[...]).astype(BF)
            kf_ref[r, :] = _dot(f, k_ref[...]).astype(BF)
            return c
        lax.fori_loop(0, 2 * NT, fwd_dft, 0)

        def prod(i, c):
            r = _rows(i)
            r2 = pl.ds(pl.multiple_of(L + i * TM, TM), TM)
            ur, ui = uf_ref[r, :].astype(F32), uf_ref[r2, :].astype(F32)
            kr, ki = kf_ref[r, :].astype(F32), kf_ref[r2, :].astype(F32)
            pc, ps = _phase(i * TM, TM)
            zr = ur * kr - ui * ki
            zi = ur * ki + ui * kr
            z_ref[r, :] = (zr * pc - zi * ps).astype(BF)
            z_ref[r2, :] = (zi * pc + zr * ps).astype(BF)
            return c
        lax.fori_loop(0, NT, prod, 0)

        def inv(i, c):
            r = _rows(i)
            r2 = pl.ds(pl.multiple_of(L + i * TM, TM), TM)
            y = (_dot(f_ref[r, :], z_ref[0:L, :]) + _dot(f_ref[r2, :], z_ref[L:2 * L, :])) * (2.0 / 4096.0)
            h_ref[r, :] = x_ref[r, :].astype(F32) + y + dx_ref[r, :].astype(F32) * dsk
            return c
        lax.fori_loop(0, NT, inv, 0)

    pl.run_scoped(s4_fwd, pltpu.VMEM((2 * L, L), BF), pltpu.VMEM((5, NJ, 128), F32),
                  pltpu.VMEM((L, D), BF), pltpu.VMEM((2 * L, D), BF))

    def gmlp(a_ref, z2_ref, g_ref, r2_ref, acc_ref):
        def f1(i, c):
            r = _rows(i)
            hn, _ = _ln(h_ref[r, :])
            a = _dot(hn.astype(BF), win_ref[...]).astype(BF)
            a_ref[r, :] = a
            z2n, rr = _ln(_gelu(a[:, FH:].astype(F32)).astype(BF).astype(F32))
            z2_ref[r, :] = z2n.astype(BF)
            r2_ref[r, :] = rr
            return c
        lax.fori_loop(0, NT, f1, 0)
        acc_ref[...] = jnp.zeros(acc_ref.shape, F32)

        def f2(i, c):
            r = _rows(i)
            g = (_dot(wsp_ref[r, :], z2_ref[...]) + bsp_ref[r, :].astype(F32)).astype(BF).astype(F32)
            a1 = a_ref[r, 0:FH].astype(F32)
            z1 = _gelu(a1).astype(BF).astype(F32)
            q = (z1 * g).astype(BF)
            out_ref[r, :] = (h_ref[r, :] + _dot(q, wout_ref[...])).astype(BF)
            do = do_ref[r, :]
            dq = _dot_nt(do, wout_ref[...])
            acc_ref[...] += _dot_tn(q, do)
            dg = (dq * z1).astype(BF)
            g_ref[r, :] = dg
            dbsp_ref[r, :] = jnp.sum(dg.astype(F32), axis=1, keepdims=True).astype(BF)
            a_ref[r, 0:FH] = (dq * g * _dgelu(a1)).astype(BF)
            dwsp_ref[r, :] = _dot_nt(dg, z2_ref[...]).astype(BF)
            return c
        lax.fori_loop(0, NT, f2, 0)
        dwout_ref[...] = acc_ref[...].astype(BF)

        def f3(i, c):
            r = _rows(i)
            dz2n = _dot_tn(wsp_ref[:, r], g_ref[...])
            dz2 = _lnb(dz2n, z2_ref[r, :].astype(F32), r2_ref[r, :])
            a_ref[r, FH:FF] = (dz2 * _dgelu(a_ref[r, FH:FF].astype(F32))).astype(BF)
            return c
        lax.fori_loop(0, NT, f3, 0)

        def f4(i, c):
            r = _rows(i)
            hn, _ = _ln(h_ref[r, :])
            z2_ref[r, 0:D] = hn.astype(BF)
            return c
        lax.fori_loop(0, NT, f4, 0)

        def f5(i, c):
            cs = pl.ds(pl.multiple_of(i * 512, 512), 512)
            dwin_ref[:, cs] = _dot_tn(z2_ref[:, 0:D], a_ref[:, cs]).astype(BF)
            return c
        lax.fori_loop(0, FF // 512, f5, 0)

        def f6(i, c):
            r = _rows(i)
            hn, rh = _ln(h_ref[r, :])
            dhn = _dot_nt(a_ref[r, :], win_ref[...])
            h_ref[r, :] = do_ref[r, :].astype(F32) + _lnb(dhn, hn.astype(BF).astype(F32), rh)
            return c
        lax.fori_loop(0, NT, f6, 0)

    pl.run_scoped(gmlp, pltpu.VMEM((L, FF), BF), pltpu.VMEM((L, FH), BF), pltpu.VMEM((L, FH), BF),
                  pltpu.VMEM((L, 1), F32), pltpu.VMEM((FH, D), F32))

    def s4_bwd(f_ref, dyb_ref, dk_ref, dsum_ref):
        _gen_dft(f_ref)
        dsum_ref[...] = jnp.zeros(dsum_ref.shape, F32)

        def cast(i, c):
            r = _rows(i)
            dh = h_ref[r, :]
            dyb_ref[r, :] = dh.astype(BF)
            dsum_ref[...] += jnp.sum(dh * dx_ref[r, :].astype(F32), axis=0, keepdims=True)
            return c
        lax.fori_loop(0, NT, cast, 0)
        ddsk_ref[...] = dsum_ref[...].astype(BF)

        def spec(i, c):
            r = _rows(i)
            r2 = pl.ds(pl.multiple_of(L + i * TM, TM), TM)
            yr = _dot(f_ref[r, :], dyb_ref[...])
            yi = _dot(f_ref[r2, :], dyb_ref[...])
            pc, ps = _phase(i * TM, TM)
            for ref in (kf_ref, uf_ref):
                kr, ki = ref[r, :].astype(F32), ref[r2, :].astype(F32)
                zr = yr * kr + yi * ki
                zi = yi * kr - yr * ki
                ref[r, :] = (zr * pc + zi * ps).astype(BF)
                ref[r2, :] = (zi * pc - zr * ps).astype(BF)
            return c
        lax.fori_loop(0, NT, spec, 0)

        def inv(i, c):
            r = _rows(i)
            r2 = pl.ds(pl.multiple_of(L + i * TM, TM), TM)
            f1_, f2_ = f_ref[r, :], f_ref[r2, :]
            dh = h_ref[r, :]
            du = (_dot(f1_, kf_ref[0:L, :]) + _dot(f2_, kf_ref[L:2 * L, :])) * (2.0 / 4096.0) + dh * dsk
            dk = (_dot(f1_, uf_ref[0:L, :]) + _dot(f2_, uf_ref[L:2 * L, :])) * (2.0 / 4096.0)
            dkh = dk.astype(BF)
            dk_ref[r, 0:D] = dkh
            dk_ref[r, DP:DP + D] = (dk - dkh.astype(F32)).astype(BF)
            u, rx = _ln(x_ref[r, :].astype(F32))
            dx_ref[r, :] = (dh + _lnb(du, u.astype(BF).astype(F32), rx)).astype(BF)
            return c
        dk_ref[:, D:DP] = jnp.zeros((L, DP - D), BF)
        dk_ref[:, DP + D:2 * DP] = jnp.zeros((L, DP - D), BF)
        lax.fori_loop(0, NT, inv, 0)

        def seg(i, c):
            lj = _lval(lax.broadcasted_iota(jnp.int32, (128, L), 0) + i * 128)
            lr = lax.broadcasted_iota(jnp.int32, (128, L), 1).astype(F32)
            mt = (lr.astype(BF).astype(F32) == lj).astype(BF)
            gg = _dot(mt, dk_ref[...])
            gg = gg[:, 0:DP] + gg[:, DP:2 * DP]
            rr = pl.ds(pl.multiple_of(i * 128, 128), 128)
            g1 = gg * lj[:, 0:1]
            for c5 in range(5):
                gp_ref[0, c5, rr, :] = gg[:, c5 * 128:(c5 + 1) * 128]
                gp_ref[1, c5, rr, :] = g1[:, c5 * 128:(c5 + 1) * 128]
            return c
        lax.fori_loop(0, NJ // 128, seg, 0)

    pl.run_scoped(s4_bwd, pltpu.VMEM((2 * L, L), BF), pltpu.VMEM((L, D), BF),
                  pltpu.VMEM((L, 2 * DP), BF), pltpu.VMEM((1, D), F32))

    def ssm_bwd(ddt_ref):
        ddt_ref[...] = jnp.zeros(ddt_ref.shape, F32)

        def chunk(c, cc):
            ns = pl.ds(pl.multiple_of((c % 4) * 32, 32), 32)
            ds_ = pl.ds(pl.multiple_of((c // 4) * 128, 128), 128)
            pr = jnp.ones((32, 128), F32)
            z = jnp.zeros((32, 128), F32)
            st = (pr, z, z, z, z, z)
            for (j0, j1, p) in SEGS:
                mr = mul_ref[p, 0, ns, ds_]
                mi = mul_ref[p, 1, ns, ds_]

                def step(j, carry):
                    pr, pi_, s0r, s0i, s1r, s1i = carry
                    js = pl.ds(pl.multiple_of(j * 8, 8), 8)
                    g0t = gp_ref[0, c // 4, js, :]
                    g1t = gp_ref[1, c // 4, js, :]
                    for t in range(8):
                        g0 = g0t[t:t + 1, :]
                        g1 = g1t[t:t + 1, :]
                        s0r, s0i = s0r + g0 * pr, s0i + g0 * pi_
                        s1r, s1i = s1r + g1 * pr, s1i + g1 * pi_
                        pr, pi_ = pr * mr - pi_ * mi, pr * mi + pi_ * mr
                    return (pr, pi_, s0r, s0i, s1r, s1i)
                st = lax.fori_loop(j0, j1, step, st)
            _, _, s0r, s0i, s1r, s1i = st
            dtc = jnp.exp(ldt_ref[:, ds_].astype(F32)).astype(BF).astype(F32)
            ar, ai = are_ref[ns, ds_].astype(F32), aim_ref[ns, ds_].astype(F32)
            b_r, b_i = bre_ref[ns, ds_].astype(F32), bim_ref[ns, ds_].astype(F32)
            cr, ci = cre_ref[ns, ds_].astype(F32), cim_ref[ns, ds_].astype(F32)
            br, bi = dtc * b_r, dtc * b_i
            dcre_ref[ns, ds_] = (s0r * br - s0i * bi).astype(BF)
            dcim_ref[ns, ds_] = (-(s0r * bi + s0i * br)).astype(BF)
            dbr = cr * s0r - ci * s0i
            dbi = -(cr * s0i + ci * s0r)
            dbre_ref[ns, ds_] = (dtc * dbr).astype(BF)
            dbim_ref[ns, ds_] = (dtc * dbi).astype(BF)
            wr = cr * br - ci * bi
            wi = cr * bi + ci * br
            dlr = wr * s1r - wi * s1i
            dli = -(wr * s1i + wi * s1r)
            dare_ref[ns, ds_] = (dtc * dlr).astype(BF)
            daim_ref[ns, ds_] = (dtc * dli).astype(BF)
            ddt_ref[:, ds_] += jnp.sum(dlr * ar + dli * ai + dbr * b_r + dbi * b_i, axis=0, keepdims=True)
            return cc
        lax.fori_loop(0, 20, chunk, 0)
        dldt_ref[...] = (ddt_ref[...] * dt).astype(BF)
    pl.run_scoped(ssm_bwd, pltpu.VMEM((1, DP), F32))


@jax.jit
def pallas_sequential_preLN__ssm_conv_s4__mixer_gmlp__prompt_kernel(
    A_u: jax.Array,
    A_A_re: jax.Array,
    A_A_im: jax.Array,
    A_B_re: jax.Array,
    A_B_im: jax.Array,
    A_C_re: jax.Array,
    A_C_im: jax.Array,
    A_log_dt: jax.Array,
    A_Dskip: jax.Array,
    B_x: jax.Array,
    B_w_in: jax.Array,
    B_w_sp: jax.Array,
    B_b_sp: jax.Array,
    B_w_out: jax.Array,
    grad_out: jax.Array,
):
    tp = lambda a: jnp.pad(a.T, ((0, 0), (0, DP - D)))
    args = (A_u[0], grad_out[0], tp(A_A_re), tp(A_A_im), tp(A_B_re), tp(A_B_im), tp(A_C_re), tp(A_C_im),
            jnp.pad(A_log_dt[None, :], ((0, 0), (0, DP - D))), A_Dskip[None, :],
            B_w_in, B_w_sp, B_b_sp[:, None], B_w_out)
    sds = lambda *s: jax.ShapeDtypeStruct(s, BF)
    out_shape = (sds(L, D), sds(L, D), sds(N, DP), sds(N, DP), sds(N, DP), sds(N, DP), sds(N, DP), sds(N, DP),
                 sds(1, DP), sds(1, D), sds(D, FF), sds(L, L), sds(L, 1), sds(FH, D))
    vm = pl.BlockSpec(memory_space=pltpu.VMEM)
    res = pl.pallas_call(
        _kernel,
        in_specs=[vm] * len(args),
        out_specs=tuple([vm] * len(out_shape)),
        out_shape=out_shape,
        scratch_shapes=[pltpu.VMEM((2 * L, D), BF), pltpu.VMEM((2 * L, D), BF), pltpu.VMEM((L, D), F32),
                        pltpu.VMEM((4, 2, N, DP), F32), pltpu.VMEM((2, 5, NJ, 128), F32)],
        compiler_params=pltpu.CompilerParams(vmem_limit_bytes=120 * 1024 * 1024),
    )(*args)
    (out, dx, dare, daim, dbre, dbim, dcre, dcim, dldt, ddsk, dwin, dwsp, dbsp, dwout) = res
    ut = lambda a: a[:, :D].T
    return (out[None], dx[None], ut(dare), ut(daim), ut(dbre), ut(dbim), ut(dcre), ut(dcim),
            dldt[0, :D], ddsk[0], dwin, dwsp, dbsp[:, 0], dwout)
```

```python
import functools
import math

import jax
import jax.numpy as jnp
from jax import lax
import jax.experimental.pallas as pl
import jax.experimental.pallas.tpu as pltpu

F32 = jnp.float32
BF = jnp.bfloat16
L = 2048
D = 576
DP = 640
N = 128
FH = 2304
FF = 4608
NJ = 768
TM = 256
NT = L // TM
GC = math.sqrt(2.0 / math.pi)


def _dot(a, b):
    return jnp.dot(a, b, preferred_element_type=F32)


def _dot_nt(a, b):
    return lax.dot_general(a, b, (((1,), (1,)), ((), ())), preferred_element_type=F32)


def _dot_tn(a, b):
    return lax.dot_general(a, b, (((0,), (0,)), ((), ())), preferred_element_type=F32)


def _ln(x):
    m = jnp.mean(x, axis=-1, keepdims=True)
    c = x - m
    v = jnp.mean(c * c, axis=-1, keepdims=True)
    r = lax.rsqrt(v + 1e-5)
    return c * r, r


def _lnb(dy, y, r):
    return r * (dy - jnp.mean(dy, axis=-1, keepdims=True)
                - y * jnp.mean(dy * y, axis=-1, keepdims=True))


def _gelu(a):
    t = jnp.tanh(GC * (a + 0.044715 * a * a * a))
    return 0.5 * a * (1.0 + t)


def _dgelu(a):
    t = jnp.tanh(GC * (a + 0.044715 * a * a * a))
    return 0.5 * (1.0 + t) + 0.5 * a * (1.0 - t * t) * GC * (1.0 + 3 * 0.044715 * a * a)


def _loop(name, lo, hi, body):
    with jax.named_scope(name):
        lax.fori_loop(lo, hi, body, 0)


def _rows(i, t=TM):
    return pl.ds(pl.multiple_of(i * t, t), t)


CB = 256
PB = L // CB


def _dft_mats():
    k = lax.broadcasted_iota(jnp.int32, (CB, CB), 0)
    t = lax.broadcasted_iota(jnp.int32, (CB, CB), 1)
    ang = (((2 * k + 1) * t) & (4 * CB - 1)).astype(F32) * (math.pi / (2 * CB))
    ff = jnp.concatenate([jnp.cos(ang), -jnp.sin(ang)], 0).astype(BF)
    t = lax.broadcasted_iota(jnp.int32, (2 * CB, CB), 0)
    k = lax.broadcasted_iota(jnp.int32, (2 * CB, CB), 1)
    ang = (((2 * k + 1) * t) & (4 * CB - 1)).astype(F32) * (math.pi / (2 * CB))
    fi = jnp.concatenate([jnp.cos(ang), -jnp.sin(ang)], 1).astype(BF)
    return ff, fi


def _lval(j):
    return jnp.where(j <= 256, j,
                     jnp.where(j <= 384, 256 + 2 * (j - 256),
                               jnp.where(j <= 512, 512 + 4 * (j - 384),
                                         jnp.where(j <= 640, 1024 + 8 * (j - 512), -1)))).astype(F32)


SEGS = ((0, 32, 0), (32, 48, 1), (48, 64, 2), (64, 81, 3))


def _kernel(x_ref, do_ref, are_ref, aim_ref, bre_ref, bim_ref, cre_ref, cim_ref,
            ldt_ref, dsk_ref, win_ref, wsp_ref, bsp_ref, wout_ref,
            out_ref, dx_ref, dare_ref, daim_ref, dbre_ref, dbim_ref, dcre_ref, dcim_ref,
            dldt_ref, ddsk_ref, dwin_ref, dwsp_ref, dbsp_ref, dwout_ref,
            uf_ref, kf_ref, h_ref, mul_ref, gp_ref):
    dsk = dsk_ref[...].astype(F32)
    dt = jnp.exp(ldt_ref[...].astype(F32)).astype(BF).astype(F32)
    lar = dt * are_ref[...].astype(F32)
    lai = dt * aim_ref[...].astype(F32)
    for p in range(4):
        e = jnp.exp(lar * (2.0 ** p))
        mul_ref[p, 0] = e * jnp.cos(lai * (2.0 ** p))
        mul_ref[p, 1] = e * jnp.sin(lai * (2.0 ** p))

    def ln_x(i, c):
        r = _rows(i)
        u, _ = _ln(x_ref[r, :].astype(F32))
        dx_ref[r, :] = u.astype(BF)
        return c
    _loop('ln_x', 0, NT, ln_x)

    def s4_fwd(kp_ref, zr_ref, zi_ref, car_ref):
        ff, fi = _dft_mats()
        kp_ref[...] = jnp.zeros(kp_ref.shape, F32)

        def chunk(c, cc):
            ns = pl.ds(pl.multiple_of((c % 2) * 64, 64), 64)
            ds_ = pl.ds(pl.multiple_of((c // 2) * 128, 128), 128)
            dtc = jnp.exp(ldt_ref[:, ds_].astype(F32)).astype(BF).astype(F32)
            br = dtc * bre_ref[ns, ds_].astype(F32)
            bi = dtc * bim_ref[ns, ds_].astype(F32)
            cr = cre_ref[ns, ds_].astype(F32)
            ci = cim_ref[ns, ds_].astype(F32)
            pr = cr * br - ci * bi
            pi_ = cr * bi + ci * br
            for (j0, j1, p) in SEGS:
                mr = mul_ref[p, 0, ns, ds_]
                mi = mul_ref[p, 1, ns, ds_]

                def step(j, carry):
                    pr, pi_ = carry
                    rows = []
                    for _ in range(8):
                        rows.append(jnp.sum(pr, axis=0, keepdims=True))
                        pr, pi_ = pr * mr - pi_ * mi, pr * mi + pi_ * mr
                    js = pl.ds(pl.multiple_of(j * 8, 8), 8)
                    kp_ref[c // 2, js, :] = kp_ref[c // 2, js, :] + jnp.concatenate(rows, 0)
                    return pr, pi_
                pr, pi_ = lax.fori_loop(j0, j1, step, (pr, pi_))
            return cc
        _loop('chunk', 0, 10, chunk)

        kpb = jnp.concatenate([kp_ref[c] for c in range(5)], 1)[:, :D].astype(BF)
        lj = _lval(lax.broadcasted_iota(jnp.int32, (CB, NJ), 1))

        def fwd_dft(i, c):
            lr = (lax.broadcasted_iota(jnp.int32, (CB, NJ), 0) + i * CB).astype(F32)
            m = (lr.astype(BF).astype(F32) == lj).astype(BF)
            kf_ref[i] = _dot(ff, _dot(m, kpb).astype(BF)).astype(BF)
            uf_ref[i] = _dot(ff, dx_ref[_rows(i, CB), :]).astype(BF)
            return c
        _loop('fwd_dft', 0, PB, fwd_dft)
        car_ref[...] = jnp.zeros(car_ref.shape, F32)

        def inv(i, c):
            zr_ref[...] = jnp.zeros(zr_ref.shape, F32)
            zi_ref[...] = jnp.zeros(zi_ref.shape, F32)

            def mac(j, cc):
                ur, ui = uf_ref[i - j, 0:CB, :].astype(F32), uf_ref[i - j, CB:2 * CB, :].astype(F32)
                kr, ki = kf_ref[j, 0:CB, :].astype(F32), kf_ref[j, CB:2 * CB, :].astype(F32)
                zr_ref[...] += ur * kr - ui * ki
                zi_ref[...] += ur * ki + ui * kr
                return cc
            lax.fori_loop(0, i + 1, mac, 0)
            z = jnp.concatenate([zr_ref[...].astype(BF), zi_ref[...].astype(BF)], 0)
            yy = _dot(fi, z) * (1.0 / CB)
            r = _rows(i, CB)
            h_ref[r, :] = (x_ref[r, :].astype(F32) + yy[0:CB] + car_ref[...]
                           + dx_ref[r, :].astype(F32) * dsk)
            car_ref[...] = yy[CB:2 * CB]
            return c
        _loop('inv', 0, PB, inv)

    pl.run_scoped(s4_fwd, pltpu.VMEM((5, NJ, 128), F32), pltpu.VMEM((CB, D), F32),
                  pltpu.VMEM((CB, D), F32), pltpu.VMEM((CB, D), F32))

    def gmlp(a_ref, z2_ref, g_ref, r2_ref, acc_ref):
        def f1(i, c):
            r = _rows(i)
            hn, _ = _ln(h_ref[r, :])
            a = _dot(hn.astype(BF), win_ref[...]).astype(BF)
            a_ref[r, :] = a
            z2n, rr = _ln(_gelu(a[:, FH:].astype(F32)).astype(BF).astype(F32))
            z2_ref[r, :] = z2n.astype(BF)
            r2_ref[r, :] = rr
            return c
        _loop('f1', 0, NT, f1)
        acc_ref[...] = jnp.zeros(acc_ref.shape, F32)

        def f2(i, c):
            r = _rows(i)
            g = (_dot(wsp_ref[r, :], z2_ref[...]) + bsp_ref[r, :].astype(F32)).astype(BF).astype(F32)
            a1 = a_ref[r, 0:FH].astype(F32)
            z1 = _gelu(a1).astype(BF).astype(F32)
            q = (z1 * g).astype(BF)
            out_ref[r, :] = (h_ref[r, :] + _dot(q, wout_ref[...])).astype(BF)
            do = do_ref[r, :]
            dq = _dot_nt(do, wout_ref[...])
            acc_ref[...] += _dot_tn(q, do)
            dg = (dq * z1).astype(BF)
            g_ref[r, :] = dg
            dbsp_ref[r, :] = jnp.sum(dg.astype(F32), axis=1, keepdims=True).astype(BF)
            a_ref[r, 0:FH] = (dq * g * _dgelu(a1)).astype(BF)
            dwsp_ref[r, :] = _dot_nt(dg, z2_ref[...]).astype(BF)
            return c
        _loop('f2', 0, NT, f2)
        dwout_ref[...] = acc_ref[...].astype(BF)

        def f3(i, c):
            r = _rows(i)
            dz2n = _dot_tn(wsp_ref[:, r], g_ref[...])
            dz2 = _lnb(dz2n, z2_ref[r, :].astype(F32), r2_ref[r, :])
            a_ref[r, FH:FF] = (dz2 * _dgelu(a_ref[r, FH:FF].astype(F32))).astype(BF)
            return c
        _loop('f3', 0, NT, f3)

        def f4(i, c):
            r = _rows(i)
            hn, _ = _ln(h_ref[r, :])
            z2_ref[r, 0:D] = hn.astype(BF)
            return c
        _loop('f4', 0, NT, f4)

        def f5(i, c):
            cs = pl.ds(pl.multiple_of(i * 512, 512), 512)
            dwin_ref[:, cs] = _dot_tn(z2_ref[:, 0:D], a_ref[:, cs]).astype(BF)
            return c
        _loop('f5', 0, FF // 512, f5)

        def f6(i, c):
            r = _rows(i)
            hn, rh = _ln(h_ref[r, :])
            dhn = _dot_nt(a_ref[r, :], win_ref[...])
            h_ref[r, :] = do_ref[r, :].astype(F32) + _lnb(dhn, hn.astype(BF).astype(F32), rh)
            return c
        _loop('f6', 0, NT, f6)

    pl.run_scoped(gmlp, pltpu.VMEM((L, FF), BF), pltpu.VMEM((L, FH), BF), pltpu.VMEM((L, FH), BF),
                  pltpu.VMEM((L, 1), F32), pltpu.VMEM((FH, D), F32))

    def s4_bwd(dyf_ref, dk_ref, dsum_ref, zr_ref, zi_ref, car_ref):
        ff, fi = _dft_mats()
        dsum_ref[...] = jnp.zeros(dsum_ref.shape, F32)

        def cast(i, c):
            r = _rows(i, CB)
            dh = h_ref[r, :]
            dyf_ref[i] = _dot(ff, dh.astype(BF)).astype(BF)
            dsum_ref[...] += jnp.sum(dh * dx_ref[r, :].astype(F32), axis=0, keepdims=True)
            return c
        _loop('cast', 0, PB, cast)
        ddsk_ref[...] = dsum_ref[...].astype(BF)

        def corr(rr, ref):
            zr_ref[...] = jnp.zeros(zr_ref.shape, F32)
            zi_ref[...] = jnp.zeros(zi_ref.shape, F32)

            def mac(j, cc):
                yr, yi = dyf_ref[rr + j, 0:CB, :].astype(F32), dyf_ref[rr + j, CB:2 * CB, :].astype(F32)
                kr, ki = ref[j, 0:CB, :].astype(F32), ref[j, CB:2 * CB, :].astype(F32)
                zr_ref[...] += yr * kr + yi * ki
                zi_ref[...] += yi * kr - yr * ki
                return cc
            lax.fori_loop(0, PB - rr, mac, 0)
            z = jnp.concatenate([zr_ref[...].astype(BF), zi_ref[...].astype(BF)], 0)
            yy = _dot(fi, z) * (1.0 / CB)
            res = yy[0:CB] + car_ref[...]
            car_ref[...] = -yy[CB:2 * CB]
            return res

        def inv_dk(i, c):
            rr = PB - 1 - i
            r = _rows(rr, CB)
            dk = corr(rr, uf_ref)
            dkh = dk.astype(BF)
            dk_ref[r, 0:D] = dkh
            dk_ref[r, DP:DP + D] = (dk - dkh.astype(F32)).astype(BF)
            return c

        def inv_du(i, c):
            rr = PB - 1 - i
            r = _rows(rr, CB)
            dh = h_ref[r, :]
            du = corr(rr, kf_ref) + dh * dsk
            u, rx = _ln(x_ref[r, :].astype(F32))
            dx_ref[r, :] = (dh + _lnb(du, u.astype(BF).astype(F32), rx)).astype(BF)
            return c
        dk_ref[:, D:DP] = jnp.zeros((L, DP - D), BF)
        dk_ref[:, DP + D:2 * DP] = jnp.zeros((L, DP - D), BF)
        car_ref[...] = jnp.zeros(car_ref.shape, F32)
        _loop('inv_dk', 0, PB, inv_dk)
        car_ref[...] = jnp.zeros(car_ref.shape, F32)
        _loop('inv_du', 0, PB, inv_du)

        def seg(i, c):
            lj = _lval(lax.broadcasted_iota(jnp.int32, (128, L), 0) + i * 128)
            lr = lax.broadcasted_iota(jnp.int32, (128, L), 1).astype(F32)
            mt = (lr.astype(BF).astype(F32) == lj).astype(BF)
            gg = _dot(mt, dk_ref[...])
            gg = gg[:, 0:DP] + gg[:, DP:2 * DP]
            rr = pl.ds(pl.multiple_of(i * 128, 128), 128)
            g1 = gg * lj[:, 0:1]
            for c5 in range(5):
                gp_ref[0, c5, rr, :] = gg[:, c5 * 128:(c5 + 1) * 128]
                gp_ref[1, c5, rr, :] = g1[:, c5 * 128:(c5 + 1) * 128]
            return c
        _loop('seg', 0, NJ // 128, seg)

    pl.run_scoped(s4_bwd, pltpu.VMEM((PB, 2 * CB, D), BF),
                  pltpu.VMEM((L, 2 * DP), BF), pltpu.VMEM((1, D), F32), pltpu.VMEM((CB, D), F32),
                  pltpu.VMEM((CB, D), F32), pltpu.VMEM((CB, D), F32))

    def ssm_bwd(ddt_ref):
        ddt_ref[...] = jnp.zeros(ddt_ref.shape, F32)

        def chunk(c, cc):
            ns = pl.ds(pl.multiple_of((c % 4) * 32, 32), 32)
            ds_ = pl.ds(pl.multiple_of((c // 4) * 128, 128), 128)
            pr = jnp.ones((32, 128), F32)
            z = jnp.zeros((32, 128), F32)
            st = (pr, z, z, z, z, z)
            for (j0, j1, p) in SEGS:
                mr = mul_ref[p, 0, ns, ds_]
                mi = mul_ref[p, 1, ns, ds_]

                def step(j, carry):
                    pr, pi_, s0r, s0i, s1r, s1i = carry
                    js = pl.ds(pl.multiple_of(j * 8, 8), 8)
                    g0t = gp_ref[0, c // 4, js, :]
                    g1t = gp_ref[1, c // 4, js, :]
                    for t in range(8):
                        g0 = g0t[t:t + 1, :]
                        g1 = g1t[t:t + 1, :]
                        s0r, s0i = s0r + g0 * pr, s0i + g0 * pi_
                        s1r, s1i = s1r + g1 * pr, s1i + g1 * pi_
                        pr, pi_ = pr * mr - pi_ * mi, pr * mi + pi_ * mr
                    return (pr, pi_, s0r, s0i, s1r, s1i)
                st = lax.fori_loop(j0, j1, step, st)
            _, _, s0r, s0i, s1r, s1i = st
            dtc = jnp.exp(ldt_ref[:, ds_].astype(F32)).astype(BF).astype(F32)
            ar, ai = are_ref[ns, ds_].astype(F32), aim_ref[ns, ds_].astype(F32)
            b_r, b_i = bre_ref[ns, ds_].astype(F32), bim_ref[ns, ds_].astype(F32)
            cr, ci = cre_ref[ns, ds_].astype(F32), cim_ref[ns, ds_].astype(F32)
            br, bi = dtc * b_r, dtc * b_i
            dcre_ref[ns, ds_] = (s0r * br - s0i * bi).astype(BF)
            dcim_ref[ns, ds_] = (-(s0r * bi + s0i * br)).astype(BF)
            dbr = cr * s0r - ci * s0i
            dbi = -(cr * s0i + ci * s0r)
            dbre_ref[ns, ds_] = (dtc * dbr).astype(BF)
            dbim_ref[ns, ds_] = (dtc * dbi).astype(BF)
            wr = cr * br - ci * bi
            wi = cr * bi + ci * br
            dlr = wr * s1r - wi * s1i
            dli = -(wr * s1i + wi * s1r)
            dare_ref[ns, ds_] = (dtc * dlr).astype(BF)
            daim_ref[ns, ds_] = (dtc * dli).astype(BF)
            ddt_ref[:, ds_] += jnp.sum(dlr * ar + dli * ai + dbr * b_r + dbi * b_i, axis=0, keepdims=True)
            return cc
        _loop('chunk', 0, 20, chunk)
        dldt_ref[...] = (ddt_ref[...] * dt).astype(BF)
    pl.run_scoped(ssm_bwd, pltpu.VMEM((1, DP), F32))


@jax.jit
def pallas_sequential_preLN__ssm_conv_s4__mixer_gmlp__prompt_kernel(
    A_u: jax.Array,
    A_A_re: jax.Array,
    A_A_im: jax.Array,
    A_B_re: jax.Array,
    A_B_im: jax.Array,
    A_C_re: jax.Array,
    A_C_im: jax.Array,
    A_log_dt: jax.Array,
    A_Dskip: jax.Array,
    B_x: jax.Array,
    B_w_in: jax.Array,
    B_w_sp: jax.Array,
    B_b_sp: jax.Array,
    B_w_out: jax.Array,
    grad_out: jax.Array,
):
    tp = lambda a: jnp.pad(a.T, ((0, 0), (0, DP - D)))
    args = (A_u[0], grad_out[0], tp(A_A_re), tp(A_A_im), tp(A_B_re), tp(A_B_im), tp(A_C_re), tp(A_C_im),
            jnp.pad(A_log_dt[None, :], ((0, 0), (0, DP - D))), A_Dskip[None, :],
            B_w_in, B_w_sp, B_b_sp[:, None], B_w_out)
    sds = lambda *s: jax.ShapeDtypeStruct(s, BF)
    out_shape = (sds(L, D), sds(L, D), sds(N, DP), sds(N, DP), sds(N, DP), sds(N, DP), sds(N, DP), sds(N, DP),
                 sds(1, DP), sds(1, D), sds(D, FF), sds(L, L), sds(L, 1), sds(FH, D))
    vm = pl.BlockSpec(memory_space=pltpu.VMEM)
    res = pl.pallas_call(
        _kernel,
        in_specs=[vm] * len(args),
        out_specs=tuple([vm] * len(out_shape)),
        out_shape=out_shape,
        scratch_shapes=[pltpu.VMEM((PB, 2 * CB, D), BF), pltpu.VMEM((PB, 2 * CB, D), BF), pltpu.VMEM((L, D), F32),
                        pltpu.VMEM((4, 2, N, DP), F32), pltpu.VMEM((2, 5, NJ, 128), F32)],
        compiler_params=pltpu.CompilerParams(vmem_limit_bytes=120 * 1024 * 1024),
    )(*args)
    (out, dx, dare, daim, dbre, dbim, dcre, dcim, dldt, ddsk, dwin, dwsp, dbsp, dwout) = res
    ut = lambda a: a[:, :D].T
    return (out[None], dx[None], ut(dare), ut(daim), ut(dbre), ut(dbim), ut(dcre), ut(dcim),
            dldt[0, :D], ddsk[0], dwin, dwsp, dbsp[:, 0], dwout)
```

```python
import functools
import math

import jax
import jax.numpy as jnp
from jax import lax
import jax.experimental.pallas as pl
import jax.experimental.pallas.tpu as pltpu

F32 = jnp.float32
BF = jnp.bfloat16
L = 2048
D = 576
DP = 640
N = 128
FH = 2304
FF = 4608
NJ = 768
TM = 256
NT = L // TM
GC = math.sqrt(2.0 / math.pi)


def _dot(a, b):
    return jnp.dot(a, b, preferred_element_type=F32)


def _dot_nt(a, b):
    return lax.dot_general(a, b, (((1,), (1,)), ((), ())), preferred_element_type=F32)


def _dot_tn(a, b):
    return lax.dot_general(a, b, (((0,), (0,)), ((), ())), preferred_element_type=F32)


def _ln(x):
    m = jnp.mean(x, axis=-1, keepdims=True)
    c = x - m
    v = jnp.mean(c * c, axis=-1, keepdims=True)
    r = lax.rsqrt(v + 1e-5)
    return c * r, r


def _lnb(dy, y, r):
    return r * (dy - jnp.mean(dy, axis=-1, keepdims=True)
                - y * jnp.mean(dy * y, axis=-1, keepdims=True))


def _gelu(a):
    t = jnp.tanh(GC * (a + 0.044715 * a * a * a))
    return 0.5 * a * (1.0 + t)


def _dgelu(a):
    t = jnp.tanh(GC * (a + 0.044715 * a * a * a))
    return 0.5 * (1.0 + t) + 0.5 * a * (1.0 - t * t) * GC * (1.0 + 3 * 0.044715 * a * a)


def _loop(name, lo, hi, body):
    with jax.named_scope(name):
        lax.fori_loop(lo, hi, body, 0)


def _rows(i, t=TM):
    return pl.ds(pl.multiple_of(i * t, t), t)


CB = 256
PB = L // CB


def _dft_mats():
    k = lax.broadcasted_iota(jnp.int32, (CB, CB), 0)
    t = lax.broadcasted_iota(jnp.int32, (CB, CB), 1)
    ang = (((2 * k + 1) * t) & (4 * CB - 1)).astype(F32) * (math.pi / (2 * CB))
    ff = jnp.concatenate([jnp.cos(ang), -jnp.sin(ang)], 0).astype(BF)
    t = lax.broadcasted_iota(jnp.int32, (2 * CB, CB), 0)
    k = lax.broadcasted_iota(jnp.int32, (2 * CB, CB), 1)
    ang = (((2 * k + 1) * t) & (4 * CB - 1)).astype(F32) * (math.pi / (2 * CB))
    fi = jnp.concatenate([jnp.cos(ang), -jnp.sin(ang)], 1).astype(BF)
    return ff, fi


def _lval(j):
    return jnp.where(j <= 256, j,
                     jnp.where(j <= 384, 256 + 2 * (j - 256),
                               jnp.where(j <= 512, 512 + 4 * (j - 384),
                                         jnp.where(j <= 640, 1024 + 8 * (j - 512), -1)))).astype(F32)


SEGS = ((0, 32, 0), (32, 48, 1), (48, 64, 2), (64, 81, 3))


def _kernel(x_hbm, do_hbm, are_ref, aim_ref, bre_ref, bim_ref, cre_ref, cim_ref,
            ldt_ref, dsk_ref, win_hbm, wsp_hbm, bsp_ref, wout_hbm,
            out_hbm, dx_hbm, dare_ref, daim_ref, dbre_ref, dbim_ref, dcre_ref, dcim_ref,
            dldt_ref, ddsk_ref, dwin_hbm, dwsp_hbm, dbsp_ref, dwout_hbm,
            uf_ref, kf_ref, h_ref, mul_ref, gp_ref,
            x_ref, do_ref, win_ref, wsp_ref, wout_ref,
            out_ref, dx_ref, dwin_ref, dwsp_ref, dwout_ref, sems):
    cin = [pltpu.make_async_copy(a, b, sems.at[i]) for i, (a, b) in enumerate(
        ((x_hbm, x_ref), (win_hbm, win_ref), (wsp_hbm, wsp_ref), (wout_hbm, wout_ref), (do_hbm, do_ref)))]
    cout = [pltpu.make_async_copy(a, b, sems.at[5 + i]) for i, (a, b) in enumerate(
        ((out_ref, out_hbm), (dwsp_ref, dwsp_hbm), (dwout_ref, dwout_hbm), (dwin_ref, dwin_hbm),
         (dx_ref, dx_hbm)))]
    for cp in cin:
        cp.start()
    dsk = dsk_ref[...].astype(F32)
    dt = jnp.exp(ldt_ref[...].astype(F32)).astype(BF).astype(F32)
    lar = dt * are_ref[...].astype(F32)
    lai = dt * aim_ref[...].astype(F32)
    for p in range(4):
        e = jnp.exp(lar * (2.0 ** p))
        mul_ref[p, 0] = e * jnp.cos(lai * (2.0 ** p))
        mul_ref[p, 1] = e * jnp.sin(lai * (2.0 ** p))

    cin[0].wait()
    def ln_x(i, c):
        r = _rows(i)
        u, _ = _ln(x_ref[r, :].astype(F32))
        dx_ref[r, :] = u.astype(BF)
        return c
    _loop('ln_x', 0, NT, ln_x)

    def s4_fwd(kp_ref, zr_ref, zi_ref, car_ref):
        ff, fi = _dft_mats()
        kp_ref[...] = jnp.zeros(kp_ref.shape, F32)

        def chunk(c, cc):
            ns = pl.ds(pl.multiple_of((c % 2) * 64, 64), 64)
            ds_ = pl.ds(pl.multiple_of((c // 2) * 128, 128), 128)
            dtc = jnp.exp(ldt_ref[:, ds_].astype(F32)).astype(BF).astype(F32)
            br = dtc * bre_ref[ns, ds_].astype(F32)
            bi = dtc * bim_ref[ns, ds_].astype(F32)
            cr = cre_ref[ns, ds_].astype(F32)
            ci = cim_ref[ns, ds_].astype(F32)
            pr = cr * br - ci * bi
            pi_ = cr * bi + ci * br
            for (j0, j1, p) in SEGS:
                mr = mul_ref[p, 0, ns, ds_]
                mi = mul_ref[p, 1, ns, ds_]

                def step(j, carry):
                    pr, pi_ = carry
                    rows = []
                    for _ in range(8):
                        rows.append(jnp.sum(pr, axis=0, keepdims=True))
                        pr, pi_ = pr * mr - pi_ * mi, pr * mi + pi_ * mr
                    js = pl.ds(pl.multiple_of(j * 8, 8), 8)
                    kp_ref[c // 2, js, :] = kp_ref[c // 2, js, :] + jnp.concatenate(rows, 0)
                    return pr, pi_
                pr, pi_ = lax.fori_loop(j0, j1, step, (pr, pi_))
            return cc
        _loop('chunk', 0, 10, chunk)

        kpb = jnp.concatenate([kp_ref[c] for c in range(5)], 1)[:, :D].astype(BF)
        lj = _lval(lax.broadcasted_iota(jnp.int32, (CB, NJ), 1))

        def fwd_dft(i, c):
            lr = (lax.broadcasted_iota(jnp.int32, (CB, NJ), 0) + i * CB).astype(F32)
            m = (lr.astype(BF).astype(F32) == lj).astype(BF)
            kf_ref[i] = _dot(ff, _dot(m, kpb).astype(BF)).astype(BF)
            uf_ref[i] = _dot(ff, dx_ref[_rows(i, CB), :]).astype(BF)
            return c
        _loop('fwd_dft', 0, PB, fwd_dft)
        car_ref[...] = jnp.zeros(car_ref.shape, F32)

        def inv(i, c):
            zr_ref[...] = jnp.zeros(zr_ref.shape, F32)
            zi_ref[...] = jnp.zeros(zi_ref.shape, F32)

            def mac(j, cc):
                ur, ui = uf_ref[i - j, 0:CB, :].astype(F32), uf_ref[i - j, CB:2 * CB, :].astype(F32)
                kr, ki = kf_ref[j, 0:CB, :].astype(F32), kf_ref[j, CB:2 * CB, :].astype(F32)
                zr_ref[...] += ur * kr - ui * ki
                zi_ref[...] += ur * ki + ui * kr
                return cc
            lax.fori_loop(0, i + 1, mac, 0)
            z = jnp.concatenate([zr_ref[...].astype(BF), zi_ref[...].astype(BF)], 0)
            yy = _dot(fi, z) * (1.0 / CB)
            r = _rows(i, CB)
            h_ref[r, :] = (x_ref[r, :].astype(F32) + yy[0:CB] + car_ref[...]
                           + dx_ref[r, :].astype(F32) * dsk)
            car_ref[...] = yy[CB:2 * CB]
            return c
        _loop('inv', 0, PB, inv)

    pl.run_scoped(s4_fwd, pltpu.VMEM((5, NJ, 128), F32), pltpu.VMEM((CB, D), F32),
                  pltpu.VMEM((CB, D), F32), pltpu.VMEM((CB, D), F32))

    def gmlp(a_ref, z2_ref, g_ref, r2_ref, acc_ref):
        for cp in cin[1:]:
            cp.wait()
        def f1(i, c):
            r = _rows(i)
            hn, _ = _ln(h_ref[r, :])
            a = _dot(hn.astype(BF), win_ref[...]).astype(BF)
            a_ref[r, :] = a
            z2n, rr = _ln(_gelu(a[:, FH:].astype(F32)).astype(BF).astype(F32))
            z2_ref[r, :] = z2n.astype(BF)
            r2_ref[r, :] = rr
            return c
        _loop('f1', 0, NT, f1)
        acc_ref[...] = jnp.zeros(acc_ref.shape, F32)

        def f2(i, c):
            r = _rows(i)
            g = (_dot(wsp_ref[r, :], z2_ref[...]) + bsp_ref[r, :].astype(F32)).astype(BF).astype(F32)
            a1 = a_ref[r, 0:FH].astype(F32)
            z1 = _gelu(a1).astype(BF).astype(F32)
            q = (z1 * g).astype(BF)
            out_ref[r, :] = (h_ref[r, :] + _dot(q, wout_ref[...])).astype(BF)
            do = do_ref[r, :]
            dq = _dot_nt(do, wout_ref[...])
            acc_ref[...] += _dot_tn(q, do)
            dg = (dq * z1).astype(BF)
            g_ref[r, :] = dg
            dbsp_ref[r, :] = jnp.sum(dg.astype(F32), axis=1, keepdims=True).astype(BF)
            a_ref[r, 0:FH] = (dq * g * _dgelu(a1)).astype(BF)
            dwsp_ref[r, :] = _dot_nt(dg, z2_ref[...]).astype(BF)
            return c
        _loop('f2', 0, NT, f2)
        dwout_ref[...] = acc_ref[...].astype(BF)
        for cp in cout[0:3]:
            cp.start()

        def f3(i, c):
            r = _rows(i)
            dz2n = _dot_tn(wsp_ref[:, r], g_ref[...])
            dz2 = _lnb(dz2n, z2_ref[r, :].astype(F32), r2_ref[r, :])
            a_ref[r, FH:FF] = (dz2 * _dgelu(a_ref[r, FH:FF].astype(F32))).astype(BF)
            return c
        _loop('f3', 0, NT, f3)

        def f4(i, c):
            r = _rows(i)
            hn, _ = _ln(h_ref[r, :])
            z2_ref[r, 0:D] = hn.astype(BF)
            return c
        _loop('f4', 0, NT, f4)

        def f5(i, c):
            cs = pl.ds(pl.multiple_of(i * 512, 512), 512)
            dwin_ref[:, cs] = _dot_tn(z2_ref[:, 0:D], a_ref[:, cs]).astype(BF)
            return c
        _loop('f5', 0, FF // 512, f5)
        cout[3].start()

        def f6(i, c):
            r = _rows(i)
            hn, rh = _ln(h_ref[r, :])
            dhn = _dot_nt(a_ref[r, :], win_ref[...])
            h_ref[r, :] = do_ref[r, :].astype(F32) + _lnb(dhn, hn.astype(BF).astype(F32), rh)
            return c
        _loop('f6', 0, NT, f6)

    pl.run_scoped(gmlp, pltpu.VMEM((L, FF), BF), pltpu.VMEM((L, FH), BF), pltpu.VMEM((L, FH), BF),
                  pltpu.VMEM((L, 1), F32), pltpu.VMEM((FH, D), F32))

    def s4_bwd(dyf_ref, dk_ref, dsum_ref, zr_ref, zi_ref, car_ref):
        ff, fi = _dft_mats()
        dsum_ref[...] = jnp.zeros(dsum_ref.shape, F32)

        def cast(i, c):
            r = _rows(i, CB)
            dh = h_ref[r, :]
            dyf_ref[i] = _dot(ff, dh.astype(BF)).astype(BF)
            dsum_ref[...] += jnp.sum(dh * dx_ref[r, :].astype(F32), axis=0, keepdims=True)
            return c
        _loop('cast', 0, PB, cast)
        ddsk_ref[...] = dsum_ref[...].astype(BF)

        def corr(rr, ref):
            zr_ref[...] = jnp.zeros(zr_ref.shape, F32)
            zi_ref[...] = jnp.zeros(zi_ref.shape, F32)

            def mac(j, cc):
                yr, yi = dyf_ref[rr + j, 0:CB, :].astype(F32), dyf_ref[rr + j, CB:2 * CB, :].astype(F32)
                kr, ki = ref[j, 0:CB, :].astype(F32), ref[j, CB:2 * CB, :].astype(F32)
                zr_ref[...] += yr * kr + yi * ki
                zi_ref[...] += yi * kr - yr * ki
                return cc
            lax.fori_loop(0, PB - rr, mac, 0)
            z = jnp.concatenate([zr_ref[...].astype(BF), zi_ref[...].astype(BF)], 0)
            yy = _dot(fi, z) * (1.0 / CB)
            res = yy[0:CB] + car_ref[...]
            car_ref[...] = -yy[CB:2 * CB]
            return res

        def inv_dk(i, c):
            rr = PB - 1 - i
            r = _rows(rr, CB)
            dk = corr(rr, uf_ref)
            dkh = dk.astype(BF)
            dk_ref[r, 0:D] = dkh
            dk_ref[r, DP:DP + D] = (dk - dkh.astype(F32)).astype(BF)
            return c

        def inv_du(i, c):
            rr = PB - 1 - i
            r = _rows(rr, CB)
            dh = h_ref[r, :]
            du = corr(rr, kf_ref) + dh * dsk
            u, rx = _ln(x_ref[r, :].astype(F32))
            dx_ref[r, :] = (dh + _lnb(du, u.astype(BF).astype(F32), rx)).astype(BF)
            return c
        dk_ref[:, D:DP] = jnp.zeros((L, DP - D), BF)
        dk_ref[:, DP + D:2 * DP] = jnp.zeros((L, DP - D), BF)
        car_ref[...] = jnp.zeros(car_ref.shape, F32)
        _loop('inv_dk', 0, PB, inv_dk)
        car_ref[...] = jnp.zeros(car_ref.shape, F32)
        _loop('inv_du', 0, PB, inv_du)
        cout[4].start()

        def seg(i, c):
            lj = _lval(lax.broadcasted_iota(jnp.int32, (128, L), 0) + i * 128)
            lr = lax.broadcasted_iota(jnp.int32, (128, L), 1).astype(F32)
            mt = (lr.astype(BF).astype(F32) == lj).astype(BF)
            gg = _dot(mt, dk_ref[...])
            gg = gg[:, 0:DP] + gg[:, DP:2 * DP]
            rr = pl.ds(pl.multiple_of(i * 128, 128), 128)
            g1 = gg * lj[:, 0:1]
            for c5 in range(5):
                gp_ref[0, c5, rr, :] = gg[:, c5 * 128:(c5 + 1) * 128]
                gp_ref[1, c5, rr, :] = g1[:, c5 * 128:(c5 + 1) * 128]
            return c
        _loop('seg', 0, NJ // 128, seg)

    pl.run_scoped(s4_bwd, pltpu.VMEM((PB, 2 * CB, D), BF),
                  pltpu.VMEM((L, 2 * DP), BF), pltpu.VMEM((1, D), F32), pltpu.VMEM((CB, D), F32),
                  pltpu.VMEM((CB, D), F32), pltpu.VMEM((CB, D), F32))

    def ssm_bwd(ddt_ref):
        ddt_ref[...] = jnp.zeros(ddt_ref.shape, F32)

        def chunk(c, cc):
            ns = pl.ds(pl.multiple_of((c % 4) * 32, 32), 32)
            ds_ = pl.ds(pl.multiple_of((c // 4) * 128, 128), 128)
            pr = jnp.ones((32, 128), F32)
            z = jnp.zeros((32, 128), F32)
            st = (pr, z, z, z, z, z)
            for (j0, j1, p) in SEGS:
                mr = mul_ref[p, 0, ns, ds_]
                mi = mul_ref[p, 1, ns, ds_]

                def step(j, carry):
                    pr, pi_, s0r, s0i, s1r, s1i = carry
                    js = pl.ds(pl.multiple_of(j * 8, 8), 8)
                    g0t = gp_ref[0, c // 4, js, :]
                    g1t = gp_ref[1, c // 4, js, :]
                    for t in range(8):
                        g0 = g0t[t:t + 1, :]
                        g1 = g1t[t:t + 1, :]
                        s0r, s0i = s0r + g0 * pr, s0i + g0 * pi_
                        s1r, s1i = s1r + g1 * pr, s1i + g1 * pi_
                        pr, pi_ = pr * mr - pi_ * mi, pr * mi + pi_ * mr
                    return (pr, pi_, s0r, s0i, s1r, s1i)
                st = lax.fori_loop(j0, j1, step, st)
            _, _, s0r, s0i, s1r, s1i = st
            dtc = jnp.exp(ldt_ref[:, ds_].astype(F32)).astype(BF).astype(F32)
            ar, ai = are_ref[ns, ds_].astype(F32), aim_ref[ns, ds_].astype(F32)
            b_r, b_i = bre_ref[ns, ds_].astype(F32), bim_ref[ns, ds_].astype(F32)
            cr, ci = cre_ref[ns, ds_].astype(F32), cim_ref[ns, ds_].astype(F32)
            br, bi = dtc * b_r, dtc * b_i
            dcre_ref[ns, ds_] = (s0r * br - s0i * bi).astype(BF)
            dcim_ref[ns, ds_] = (-(s0r * bi + s0i * br)).astype(BF)
            dbr = cr * s0r - ci * s0i
            dbi = -(cr * s0i + ci * s0r)
            dbre_ref[ns, ds_] = (dtc * dbr).astype(BF)
            dbim_ref[ns, ds_] = (dtc * dbi).astype(BF)
            wr = cr * br - ci * bi
            wi = cr * bi + ci * br
            dlr = wr * s1r - wi * s1i
            dli = -(wr * s1i + wi * s1r)
            dare_ref[ns, ds_] = (dtc * dlr).astype(BF)
            daim_ref[ns, ds_] = (dtc * dli).astype(BF)
            ddt_ref[:, ds_] += jnp.sum(dlr * ar + dli * ai + dbr * b_r + dbi * b_i, axis=0, keepdims=True)
            return cc
        _loop('chunk', 0, 20, chunk)
        dldt_ref[...] = (ddt_ref[...] * dt).astype(BF)
    pl.run_scoped(ssm_bwd, pltpu.VMEM((1, DP), F32))
    for cp in cout:
        cp.wait()


@jax.jit
def pallas_sequential_preLN__ssm_conv_s4__mixer_gmlp__prompt_kernel(
    A_u: jax.Array,
    A_A_re: jax.Array,
    A_A_im: jax.Array,
    A_B_re: jax.Array,
    A_B_im: jax.Array,
    A_C_re: jax.Array,
    A_C_im: jax.Array,
    A_log_dt: jax.Array,
    A_Dskip: jax.Array,
    B_x: jax.Array,
    B_w_in: jax.Array,
    B_w_sp: jax.Array,
    B_b_sp: jax.Array,
    B_w_out: jax.Array,
    grad_out: jax.Array,
):
    tp = lambda a: jnp.pad(a.T, ((0, 0), (0, DP - D)))
    args = (A_u[0], grad_out[0], tp(A_A_re), tp(A_A_im), tp(A_B_re), tp(A_B_im), tp(A_C_re), tp(A_C_im),
            jnp.pad(A_log_dt[None, :], ((0, 0), (0, DP - D))), A_Dskip[None, :],
            B_w_in, B_w_sp, B_b_sp[:, None], B_w_out)
    sds = lambda *s: jax.ShapeDtypeStruct(s, BF)
    out_shape = (sds(L, D), sds(L, D), sds(N, DP), sds(N, DP), sds(N, DP), sds(N, DP), sds(N, DP), sds(N, DP),
                 sds(1, DP), sds(1, D), sds(D, FF), sds(L, L), sds(L, 1), sds(FH, D))
    vm = pl.BlockSpec(memory_space=pltpu.VMEM)
    an = pl.BlockSpec(memory_space=pl.ANY)
    res = pl.pallas_call(
        _kernel,
        in_specs=[an, an] + [vm] * 8 + [an, an, vm, an],
        out_specs=(an, an) + (vm,) * 8 + (an, an, vm, an),
        out_shape=out_shape,
        scratch_shapes=[pltpu.VMEM((PB, 2 * CB, D), BF), pltpu.VMEM((PB, 2 * CB, D), BF), pltpu.VMEM((L, D), F32),
                        pltpu.VMEM((4, 2, N, DP), F32), pltpu.VMEM((2, 5, NJ, 128), F32),
                        pltpu.VMEM((L, D), BF), pltpu.VMEM((L, D), BF), pltpu.VMEM((D, FF), BF),
                        pltpu.VMEM((L, L), BF), pltpu.VMEM((FH, D), BF),
                        pltpu.VMEM((L, D), BF), pltpu.VMEM((L, D), BF), pltpu.VMEM((D, FF), BF),
                        pltpu.VMEM((L, L), BF), pltpu.VMEM((FH, D), BF),
                        pltpu.SemaphoreType.DMA((10,))],
        compiler_params=pltpu.CompilerParams(vmem_limit_bytes=120 * 1024 * 1024),
    )(*args)
    (out, dx, dare, daim, dbre, dbim, dcre, dcim, dldt, ddsk, dwin, dwsp, dbsp, dwout) = res
    ut = lambda a: a[:, :D].T
    return (out[None], dx[None], ut(dare), ut(daim), ut(dbre), ut(dbim), ut(dcre), ut(dcim),
            dldt[0, :D], ddsk[0], dwin, dwsp, dbsp[:, 0], dwout)
```

```python
import functools
import math

import jax
import jax.numpy as jnp
from jax import lax
import jax.experimental.pallas as pl
import jax.experimental.pallas.tpu as pltpu

F32 = jnp.float32
BF = jnp.bfloat16
L = 2048
D = 576
DP = 640
N = 128
FH = 2304
FF = 4608
NJ = 768
TM = 256
NT = L // TM
GC = math.sqrt(2.0 / math.pi)


def _dot(a, b):
    return jnp.dot(a, b, preferred_element_type=F32)


def _dot_nt(a, b):
    return lax.dot_general(a, b, (((1,), (1,)), ((), ())), preferred_element_type=F32)


def _dot_tn(a, b):
    return lax.dot_general(a, b, (((0,), (0,)), ((), ())), preferred_element_type=F32)


def _ln(x):
    m = jnp.mean(x, axis=-1, keepdims=True)
    c = x - m
    v = jnp.mean(c * c, axis=-1, keepdims=True)
    r = lax.rsqrt(v + 1e-5)
    return c * r, r


def _lnb(dy, y, r):
    return r * (dy - jnp.mean(dy, axis=-1, keepdims=True)
                - y * jnp.mean(dy * y, axis=-1, keepdims=True))


def _gelu(a):
    t = jnp.tanh(GC * (a + 0.044715 * a * a * a))
    return 0.5 * a * (1.0 + t)


def _dgelu(a):
    t = jnp.tanh(GC * (a + 0.044715 * a * a * a))
    return 0.5 * (1.0 + t) + 0.5 * a * (1.0 - t * t) * GC * (1.0 + 3 * 0.044715 * a * a)


def _loop(name, lo, hi, body):
    with jax.named_scope(name):
        lax.fori_loop(lo, hi, body, 0)


def _rows(i, t=TM):
    return pl.ds(pl.multiple_of(i * t, t), t)


CB = 256
PB = L // CB


def _dft_mats():
    k = lax.broadcasted_iota(jnp.int32, (CB, CB), 0)
    t = lax.broadcasted_iota(jnp.int32, (CB, CB), 1)
    ang = (((2 * k + 1) * t) & (4 * CB - 1)).astype(F32) * (math.pi / (2 * CB))
    ff = jnp.concatenate([jnp.cos(ang), -jnp.sin(ang)], 0).astype(BF)
    t = lax.broadcasted_iota(jnp.int32, (2 * CB, CB), 0)
    k = lax.broadcasted_iota(jnp.int32, (2 * CB, CB), 1)
    ang = (((2 * k + 1) * t) & (4 * CB - 1)).astype(F32) * (math.pi / (2 * CB))
    fi = jnp.concatenate([jnp.cos(ang), -jnp.sin(ang)], 1).astype(BF)
    return ff, fi


def _lval(j):
    return jnp.where(j <= 256, j,
                     jnp.where(j <= 384, 256 + 2 * (j - 256),
                               jnp.where(j <= 512, 512 + 4 * (j - 384),
                                         jnp.where(j <= 640, 1024 + 8 * (j - 512), -1)))).astype(F32)


SEGS = ((0, 32, 0), (32, 48, 1), (48, 64, 2), (64, 81, 3))


def _kernel(x_hbm, do_hbm, are_ref, aim_ref, bre_ref, bim_ref, cre_ref, cim_ref,
            ldt_ref, dsk_ref, win_hbm, wsp_hbm, bsp_ref, wout_hbm,
            out_hbm, dx_hbm, dare_ref, daim_ref, dbre_ref, dbim_ref, dcre_ref, dcim_ref,
            dldt_ref, ddsk_ref, dwin_hbm, dwsp_hbm, dbsp_ref, dwout_hbm,
            uf_ref, kf_ref, h_ref, mul_ref, gp_ref,
            win_ref, wsp_ref, wout_ref,
            out_ref, dx_ref, dwin_ref, dwsp_ref, dwout_ref, x_ref, do_ref, u_ref, sems):
    xt_ref, dot_ref = out_ref, dx_ref
    cin = [pltpu.make_async_copy(a, b, sems.at[i]) for i, (a, b) in enumerate(
        ((x_hbm, xt_ref), (win_hbm, win_ref), (wsp_hbm, wsp_ref), (wout_hbm, wout_ref), (do_hbm, dot_ref)))]
    cout = [pltpu.make_async_copy(a, b, sems.at[5 + i]) for i, (a, b) in enumerate(
        ((out_ref, out_hbm), (dwsp_ref, dwsp_hbm), (dwout_ref, dwout_hbm), (dwin_ref, dwin_hbm),
         (dx_ref, dx_hbm)))]
    for cp in cin:
        cp.start()
    dsk = dsk_ref[...].astype(F32)
    dt = jnp.exp(ldt_ref[...].astype(F32)).astype(BF).astype(F32)
    lar = dt * are_ref[...].astype(F32)
    lai = dt * aim_ref[...].astype(F32)
    for p in range(4):
        e = jnp.exp(lar * (2.0 ** p))
        mul_ref[p, 0] = e * jnp.cos(lai * (2.0 ** p))
        mul_ref[p, 1] = e * jnp.sin(lai * (2.0 ** p))

    cin[0].wait()
    def ln_x(i, c):
        r = _rows(i)
        x = xt_ref[:, r].astype(F32).T
        x_ref[r, :] = x.astype(BF)
        u, _ = _ln(x)
        u_ref[r, :] = u.astype(BF)
        return c
    _loop('ln_x', 0, NT, ln_x)

    def s4_fwd(kp_ref, zr_ref, zi_ref, car_ref):
        ff, fi = _dft_mats()
        kp_ref[...] = jnp.zeros(kp_ref.shape, F32)

        def chunk(c, cc):
            ns = pl.ds(pl.multiple_of((c % 2) * 64, 64), 64)
            ds_ = pl.ds(pl.multiple_of((c // 2) * 128, 128), 128)
            dtc = jnp.exp(ldt_ref[:, ds_].astype(F32)).astype(BF).astype(F32)
            br = dtc * bre_ref[ns, ds_].astype(F32)
            bi = dtc * bim_ref[ns, ds_].astype(F32)
            cr = cre_ref[ns, ds_].astype(F32)
            ci = cim_ref[ns, ds_].astype(F32)
            pr = cr * br - ci * bi
            pi_ = cr * bi + ci * br
            for (j0, j1, p) in SEGS:
                mr = mul_ref[p, 0, ns, ds_]
                mi = mul_ref[p, 1, ns, ds_]

                def step(j, carry):
                    pr, pi_ = carry
                    rows = []
                    for _ in range(8):
                        rows.append(jnp.sum(pr, axis=0, keepdims=True))
                        pr, pi_ = pr * mr - pi_ * mi, pr * mi + pi_ * mr
                    js = pl.ds(pl.multiple_of(j * 8, 8), 8)
                    kp_ref[c // 2, js, :] = kp_ref[c // 2, js, :] + jnp.concatenate(rows, 0)
                    return pr, pi_
                pr, pi_ = lax.fori_loop(j0, j1, step, (pr, pi_))
            return cc
        _loop('chunk', 0, 10, chunk)

        kpb = jnp.concatenate([kp_ref[c] for c in range(5)], 1)[:, :D].astype(BF)
        lj = _lval(lax.broadcasted_iota(jnp.int32, (CB, NJ), 1))

        def fwd_dft(i, c):
            lr = (lax.broadcasted_iota(jnp.int32, (CB, NJ), 0) + i * CB).astype(F32)
            m = (lr.astype(BF).astype(F32) == lj).astype(BF)
            kf_ref[i] = _dot(ff, _dot(m, kpb).astype(BF)).astype(BF)
            uf_ref[i] = _dot(ff, u_ref[_rows(i, CB), :]).astype(BF)
            return c
        _loop('fwd_dft', 0, PB, fwd_dft)
        car_ref[...] = jnp.zeros(car_ref.shape, F32)

        def inv(i, c):
            zr_ref[...] = jnp.zeros(zr_ref.shape, F32)
            zi_ref[...] = jnp.zeros(zi_ref.shape, F32)

            def mac(j, cc):
                ur, ui = uf_ref[i - j, 0:CB, :].astype(F32), uf_ref[i - j, CB:2 * CB, :].astype(F32)
                kr, ki = kf_ref[j, 0:CB, :].astype(F32), kf_ref[j, CB:2 * CB, :].astype(F32)
                zr_ref[...] += ur * kr - ui * ki
                zi_ref[...] += ur * ki + ui * kr
                return cc
            lax.fori_loop(0, i + 1, mac, 0)
            z = jnp.concatenate([zr_ref[...].astype(BF), zi_ref[...].astype(BF)], 0)
            yy = _dot(fi, z) * (1.0 / CB)
            r = _rows(i, CB)
            h_ref[r, :] = (x_ref[r, :].astype(F32) + yy[0:CB] + car_ref[...]
                           + u_ref[r, :].astype(F32) * dsk)
            car_ref[...] = yy[CB:2 * CB]
            return c
        _loop('inv', 0, PB, inv)

    pl.run_scoped(s4_fwd, pltpu.VMEM((5, NJ, 128), F32), pltpu.VMEM((CB, D), F32),
                  pltpu.VMEM((CB, D), F32), pltpu.VMEM((CB, D), F32))

    def gmlp(a_ref, z2_ref, g_ref, r2_ref, acc_ref):
        for cp in cin[1:]:
            cp.wait()
        def f1(i, c):
            r = _rows(i)
            hn, _ = _ln(h_ref[r, :])
            a = _dot(hn.astype(BF), win_ref[...]).astype(BF)
            a_ref[r, :] = a
            z2n, rr = _ln(_gelu(a[:, FH:].astype(F32)).astype(BF).astype(F32))
            z2_ref[r, :] = z2n.astype(BF)
            r2_ref[r, :] = rr
            return c
        _loop('f1', 0, NT, f1)
        acc_ref[...] = jnp.zeros(acc_ref.shape, F32)

        def f2(i, c):
            r = _rows(i)
            g = (_dot(wsp_ref[r, :], z2_ref[...]) + bsp_ref[r, :].astype(F32)).astype(BF).astype(F32)
            a1 = a_ref[r, 0:FH].astype(F32)
            z1 = _gelu(a1).astype(BF).astype(F32)
            q = (z1 * g).astype(BF)
            out_ref[:, r] = (h_ref[r, :] + _dot_nt(q, wout_ref[...])).T.astype(BF)
            dot_ = dot_ref[:, r]
            do = dot_.astype(F32).T.astype(BF)
            do_ref[r, :] = do
            dq = _dot(do, wout_ref[...])
            acc_ref[...] += _dot(dot_, q)
            dg = (dq * z1).astype(BF)
            g_ref[r, :] = dg
            dbsp_ref[r, :] = jnp.sum(dg.astype(F32), axis=1, keepdims=True).astype(BF)
            a_ref[r, 0:FH] = (dq * g * _dgelu(a1)).astype(BF)
            dwsp_ref[r, :] = _dot_nt(dg, z2_ref[...]).astype(BF)
            return c
        _loop('f2', 0, NT, f2)
        dwout_ref[...] = acc_ref[...].astype(BF)
        for cp in cout[0:3]:
            cp.start()

        def f3(i, c):
            r = _rows(i)
            dz2n = _dot_tn(wsp_ref[:, r], g_ref[...])
            dz2 = _lnb(dz2n, z2_ref[r, :].astype(F32), r2_ref[r, :])
            a_ref[r, FH:FF] = (dz2 * _dgelu(a_ref[r, FH:FF].astype(F32))).astype(BF)
            return c
        _loop('f3', 0, NT, f3)

        def f4(i, c):
            r = _rows(i)
            hn, _ = _ln(h_ref[r, :])
            z2_ref[r, 0:D] = hn.astype(BF)
            return c
        _loop('f4', 0, NT, f4)

        def f5(i, c):
            cs = pl.ds(pl.multiple_of(i * 512, 512), 512)
            dwin_ref[:, cs] = _dot_tn(z2_ref[:, 0:D], a_ref[:, cs]).astype(BF)
            return c
        _loop('f5', 0, FF // 512, f5)
        cout[3].start()

        def f6(i, c):
            r = _rows(i)
            hn, rh = _ln(h_ref[r, :])
            dhn = _dot_nt(a_ref[r, :], win_ref[...])
            h_ref[r, :] = do_ref[r, :].astype(F32) + _lnb(dhn, hn.astype(BF).astype(F32), rh)
            return c
        _loop('f6', 0, NT, f6)

    pl.run_scoped(gmlp, pltpu.VMEM((L, FF), BF), pltpu.VMEM((L, FH), BF), pltpu.VMEM((L, FH), BF),
                  pltpu.VMEM((L, 1), F32), pltpu.VMEM((D, FH), F32))

    def s4_bwd(dyf_ref, dk_ref, dsum_ref, zr_ref, zi_ref, car_ref):
        ff, fi = _dft_mats()
        dsum_ref[...] = jnp.zeros(dsum_ref.shape, F32)

        def cast(i, c):
            r = _rows(i, CB)
            dh = h_ref[r, :]
            dyf_ref[i] = _dot(ff, dh.astype(BF)).astype(BF)
            dsum_ref[...] += jnp.sum(dh * u_ref[r, :].astype(F32), axis=0, keepdims=True)
            return c
        _loop('cast', 0, PB, cast)
        ddsk_ref[...] = dsum_ref[...].astype(BF)

        def corr(rr, ref):
            zr_ref[...] = jnp.zeros(zr_ref.shape, F32)
            zi_ref[...] = jnp.zeros(zi_ref.shape, F32)

            def mac(j, cc):
                yr, yi = dyf_ref[rr + j, 0:CB, :].astype(F32), dyf_ref[rr + j, CB:2 * CB, :].astype(F32)
                kr, ki = ref[j, 0:CB, :].astype(F32), ref[j, CB:2 * CB, :].astype(F32)
                zr_ref[...] += yr * kr + yi * ki
                zi_ref[...] += yi * kr - yr * ki
                return cc
            lax.fori_loop(0, PB - rr, mac, 0)
            z = jnp.concatenate([zr_ref[...].astype(BF), zi_ref[...].astype(BF)], 0)
            yy = _dot(fi, z) * (1.0 / CB)
            res = yy[0:CB] + car_ref[...]
            car_ref[...] = -yy[CB:2 * CB]
            return res

        def inv_dk(i, c):
            rr = PB - 1 - i
            r = _rows(rr, CB)
            dk = corr(rr, uf_ref)
            dkh = dk.astype(BF)
            dk_ref[r, 0:D] = dkh
            dk_ref[r, DP:DP + D] = (dk - dkh.astype(F32)).astype(BF)
            return c

        def inv_du(i, c):
            rr = PB - 1 - i
            r = _rows(rr, CB)
            dh = h_ref[r, :]
            du = corr(rr, kf_ref) + dh * dsk
            u, rx = _ln(x_ref[r, :].astype(F32))
            dx_ref[:, r] = (dh + _lnb(du, u.astype(BF).astype(F32), rx)).T.astype(BF)
            return c
        dk_ref[:, D:DP] = jnp.zeros((L, DP - D), BF)
        dk_ref[:, DP + D:2 * DP] = jnp.zeros((L, DP - D), BF)
        car_ref[...] = jnp.zeros(car_ref.shape, F32)
        _loop('inv_dk', 0, PB, inv_dk)
        car_ref[...] = jnp.zeros(car_ref.shape, F32)
        _loop('inv_du', 0, PB, inv_du)
        cout[4].start()

        def seg(i, c):
            lj = _lval(lax.broadcasted_iota(jnp.int32, (128, L), 0) + i * 128)
            lr = lax.broadcasted_iota(jnp.int32, (128, L), 1).astype(F32)
            mt = (lr.astype(BF).astype(F32) == lj).astype(BF)
            gg = _dot(mt, dk_ref[...])
            gg = gg[:, 0:DP] + gg[:, DP:2 * DP]
            rr = pl.ds(pl.multiple_of(i * 128, 128), 128)
            g1 = gg * lj[:, 0:1]
            for c5 in range(5):
                gp_ref[0, c5, rr, :] = gg[:, c5 * 128:(c5 + 1) * 128]
                gp_ref[1, c5, rr, :] = g1[:, c5 * 128:(c5 + 1) * 128]
            return c
        _loop('seg', 0, NJ // 128, seg)

    pl.run_scoped(s4_bwd, pltpu.VMEM((PB, 2 * CB, D), BF),
                  pltpu.VMEM((L, 2 * DP), BF), pltpu.VMEM((1, D), F32), pltpu.VMEM((CB, D), F32),
                  pltpu.VMEM((CB, D), F32), pltpu.VMEM((CB, D), F32))

    def ssm_bwd(ddt_ref):
        ddt_ref[...] = jnp.zeros(ddt_ref.shape, F32)

        def chunk(c, cc):
            ns = pl.ds(pl.multiple_of((c % 4) * 32, 32), 32)
            ds_ = pl.ds(pl.multiple_of((c // 4) * 128, 128), 128)
            pr = jnp.ones((32, 128), F32)
            z = jnp.zeros((32, 128), F32)
            st = (pr, z, z, z, z, z)
            for (j0, j1, p) in SEGS:
                mr = mul_ref[p, 0, ns, ds_]
                mi = mul_ref[p, 1, ns, ds_]

                def step(j, carry):
                    pr, pi_, s0r, s0i, s1r, s1i = carry
                    js = pl.ds(pl.multiple_of(j * 8, 8), 8)
                    g0t = gp_ref[0, c // 4, js, :]
                    g1t = gp_ref[1, c // 4, js, :]
                    for t in range(8):
                        g0 = g0t[t:t + 1, :]
                        g1 = g1t[t:t + 1, :]
                        s0r, s0i = s0r + g0 * pr, s0i + g0 * pi_
                        s1r, s1i = s1r + g1 * pr, s1i + g1 * pi_
                        pr, pi_ = pr * mr - pi_ * mi, pr * mi + pi_ * mr
                    return (pr, pi_, s0r, s0i, s1r, s1i)
                st = lax.fori_loop(j0, j1, step, st)
            _, _, s0r, s0i, s1r, s1i = st
            dtc = jnp.exp(ldt_ref[:, ds_].astype(F32)).astype(BF).astype(F32)
            ar, ai = are_ref[ns, ds_].astype(F32), aim_ref[ns, ds_].astype(F32)
            b_r, b_i = bre_ref[ns, ds_].astype(F32), bim_ref[ns, ds_].astype(F32)
            cr, ci = cre_ref[ns, ds_].astype(F32), cim_ref[ns, ds_].astype(F32)
            br, bi = dtc * b_r, dtc * b_i
            dcre_ref[ns, ds_] = (s0r * br - s0i * bi).astype(BF)
            dcim_ref[ns, ds_] = (-(s0r * bi + s0i * br)).astype(BF)
            dbr = cr * s0r - ci * s0i
            dbi = -(cr * s0i + ci * s0r)
            dbre_ref[ns, ds_] = (dtc * dbr).astype(BF)
            dbim_ref[ns, ds_] = (dtc * dbi).astype(BF)
            wr = cr * br - ci * bi
            wi = cr * bi + ci * br
            dlr = wr * s1r - wi * s1i
            dli = -(wr * s1i + wi * s1r)
            dare_ref[ns, ds_] = (dtc * dlr).astype(BF)
            daim_ref[ns, ds_] = (dtc * dli).astype(BF)
            ddt_ref[:, ds_] += jnp.sum(dlr * ar + dli * ai + dbr * b_r + dbi * b_i, axis=0, keepdims=True)
            return cc
        _loop('chunk', 0, 20, chunk)
        dldt_ref[...] = (ddt_ref[...] * dt).astype(BF)
    pl.run_scoped(ssm_bwd, pltpu.VMEM((1, DP), F32))
    for cp in cout:
        cp.wait()


@jax.jit
def pallas_sequential_preLN__ssm_conv_s4__mixer_gmlp__prompt_kernel(
    A_u: jax.Array,
    A_A_re: jax.Array,
    A_A_im: jax.Array,
    A_B_re: jax.Array,
    A_B_im: jax.Array,
    A_C_re: jax.Array,
    A_C_im: jax.Array,
    A_log_dt: jax.Array,
    A_Dskip: jax.Array,
    B_x: jax.Array,
    B_w_in: jax.Array,
    B_w_sp: jax.Array,
    B_b_sp: jax.Array,
    B_w_out: jax.Array,
    grad_out: jax.Array,
):
    tp = lambda a: jnp.pad(a.T, ((0, 0), (0, DP - D)))
    args = (A_u[0].T, grad_out[0].T, tp(A_A_re), tp(A_A_im), tp(A_B_re), tp(A_B_im), tp(A_C_re), tp(A_C_im),
            jnp.pad(A_log_dt[None, :], ((0, 0), (0, DP - D))), A_Dskip[None, :],
            B_w_in, B_w_sp, B_b_sp[:, None], B_w_out.T)
    sds = lambda *s: jax.ShapeDtypeStruct(s, BF)
    out_shape = (sds(D, L), sds(D, L), sds(N, DP), sds(N, DP), sds(N, DP), sds(N, DP), sds(N, DP), sds(N, DP),
                 sds(1, DP), sds(1, D), sds(D, FF), sds(L, L), sds(L, 1), sds(D, FH))
    vm = pl.BlockSpec(memory_space=pltpu.VMEM)
    an = pl.BlockSpec(memory_space=pl.ANY)
    res = pl.pallas_call(
        _kernel,
        in_specs=[an, an] + [vm] * 8 + [an, an, vm, an],
        out_specs=(an, an) + (vm,) * 8 + (an, an, vm, an),
        out_shape=out_shape,
        scratch_shapes=[pltpu.VMEM((PB, 2 * CB, D), BF), pltpu.VMEM((PB, 2 * CB, D), BF), pltpu.VMEM((L, D), F32),
                        pltpu.VMEM((4, 2, N, DP), F32), pltpu.VMEM((2, 5, NJ, 128), F32),
                        pltpu.VMEM((D, FF), BF),
                        pltpu.VMEM((L, L), BF), pltpu.VMEM((D, FH), BF),
                        pltpu.VMEM((D, L), BF), pltpu.VMEM((D, L), BF), pltpu.VMEM((D, FF), BF),
                        pltpu.VMEM((L, L), BF), pltpu.VMEM((D, FH), BF),
                        pltpu.VMEM((L, D), BF), pltpu.VMEM((L, D), BF), pltpu.VMEM((L, D), BF),
                        pltpu.SemaphoreType.DMA((10,))],
        compiler_params=pltpu.CompilerParams(vmem_limit_bytes=120 * 1024 * 1024),
    )(*args)
    (out, dx, dare, daim, dbre, dbim, dcre, dcim, dldt, ddsk, dwin, dwsp, dbsp, dwout) = res
    ut = lambda a: a[:, :D].T
    return (out.T[None], dx.T[None], ut(dare), ut(daim), ut(dbre), ut(dbim), ut(dcre), ut(dcim),
            dldt[0, :D], ddsk[0], dwin, dwsp, dbsp[:, 0], dwout.T)
```

```python
import functools
import math

import jax
import jax.numpy as jnp
from jax import lax
import jax.experimental.pallas as pl
import jax.experimental.pallas.tpu as pltpu

F32 = jnp.float32
BF = jnp.bfloat16
L = 2048
D = 576
DP = 640
N = 128
FH = 2304
FF = 4608
NJ = 768
TM = 256
NT = L // TM
GC = math.sqrt(2.0 / math.pi)


def _dot(a, b):
    return jnp.dot(a, b, preferred_element_type=F32)


def _dot_nt(a, b):
    return lax.dot_general(a, b, (((1,), (1,)), ((), ())), preferred_element_type=F32)


def _dot_tn(a, b):
    return lax.dot_general(a, b, (((0,), (0,)), ((), ())), preferred_element_type=F32)


def _ln(x):
    m = jnp.mean(x, axis=-1, keepdims=True)
    c = x - m
    v = jnp.mean(c * c, axis=-1, keepdims=True)
    r = lax.rsqrt(v + 1e-5)
    return c * r, r


def _lnb(dy, y, r):
    return r * (dy - jnp.mean(dy, axis=-1, keepdims=True)
                - y * jnp.mean(dy * y, axis=-1, keepdims=True))


def _gelu(a):
    t = jnp.tanh(GC * (a + 0.044715 * a * a * a))
    return 0.5 * a * (1.0 + t)


def _dgelu(a):
    t = jnp.tanh(GC * (a + 0.044715 * a * a * a))
    return 0.5 * (1.0 + t) + 0.5 * a * (1.0 - t * t) * GC * (1.0 + 3 * 0.044715 * a * a)


def _loop(name, lo, hi, body):
    with jax.named_scope(name):
        lax.fori_loop(lo, hi, body, 0)


def _rows(i, t=TM):
    return pl.ds(pl.multiple_of(i * t, t), t)


CB = 256
PB = L // CB


def _dft_mats():
    k = lax.broadcasted_iota(jnp.int32, (CB, CB), 0)
    t = lax.broadcasted_iota(jnp.int32, (CB, CB), 1)
    ang = (((2 * k + 1) * t) & (4 * CB - 1)).astype(F32) * (math.pi / (2 * CB))
    ff = jnp.concatenate([jnp.cos(ang), -jnp.sin(ang)], 0).astype(BF)
    t = lax.broadcasted_iota(jnp.int32, (2 * CB, CB), 0)
    k = lax.broadcasted_iota(jnp.int32, (2 * CB, CB), 1)
    ang = (((2 * k + 1) * t) & (4 * CB - 1)).astype(F32) * (math.pi / (2 * CB))
    fi = jnp.concatenate([jnp.cos(ang), -jnp.sin(ang)], 1).astype(BF)
    return ff, fi


def _lval(j):
    return jnp.where(j <= 256, j,
                     jnp.where(j <= 384, 256 + 2 * (j - 256),
                               jnp.where(j <= 512, 512 + 4 * (j - 384),
                                         jnp.where(j <= 640, 1024 + 8 * (j - 512), -1)))).astype(F32)


SEGS = ((0, 32, 0), (32, 48, 1), (48, 64, 2), (64, 81, 3))


def _kernel(x_hbm, do_hbm, are_ref, aim_ref, bre_ref, bim_ref, cre_ref, cim_ref,
            ldt_ref, dsk_ref, win_hbm, wsp_hbm, bsp_ref, wout_hbm,
            out_hbm, dx_hbm, dare_ref, daim_ref, dbre_ref, dbim_ref, dcre_ref, dcim_ref,
            dldt_ref, ddsk_ref, dwin_hbm, dwsp_hbm, dbsp_ref, dwout_hbm,
            uf_ref, kf_ref, h_ref, mul_ref, gp_ref,
            win_ref, wsp_ref, wout_ref,
            out_ref, dx_ref, dwout_ref, x_ref, do_ref, u_ref, a_ref, z2_ref, g_ref, sems):
    dwin_ref, dwsp_ref = win_ref, wsp_ref
    xt_ref, dot_ref = out_ref, dx_ref
    cin = [pltpu.make_async_copy(a, b, sems.at[i]) for i, (a, b) in enumerate(
        ((x_hbm, xt_ref), (win_hbm, win_ref), (wsp_hbm, wsp_ref), (wout_hbm, wout_ref), (do_hbm, dot_ref)))]
    cout = [pltpu.make_async_copy(a, b, sems.at[5 + i]) for i, (a, b) in enumerate(
        ((out_ref, out_hbm), (dwsp_ref, dwsp_hbm), (dwout_ref, dwout_hbm), (dwin_ref, dwin_hbm),
         (dx_ref, dx_hbm)))]
    for cp in cin:
        cp.start()
    dsk = dsk_ref[...].astype(F32)
    dt = jnp.exp(ldt_ref[...].astype(F32)).astype(BF).astype(F32)
    lar = dt * are_ref[...].astype(F32)
    lai = dt * aim_ref[...].astype(F32)
    for p in range(4):
        e = jnp.exp(lar * (2.0 ** p))
        mul_ref[p, 0] = e * jnp.cos(lai * (2.0 ** p))
        mul_ref[p, 1] = e * jnp.sin(lai * (2.0 ** p))

    cin[0].wait()
    def ln_x(i, c):
        r = _rows(i)
        x = xt_ref[:, r].astype(F32).T
        x_ref[r, :] = x.astype(BF)
        u, _ = _ln(x)
        u_ref[r, :] = u.astype(BF)
        return c
    _loop('ln_x', 0, NT, ln_x)

    def s4_fwd(kp_ref, zr_ref, zi_ref, car_ref):
        ff, fi = _dft_mats()
        kp_ref[...] = jnp.zeros(kp_ref.shape, F32)

        def chunk(c, cc):
            ns = pl.ds(pl.multiple_of((c % 2) * 64, 64), 64)
            ds_ = pl.ds(pl.multiple_of((c // 2) * 128, 128), 128)
            dtc = jnp.exp(ldt_ref[:, ds_].astype(F32)).astype(BF).astype(F32)
            br = dtc * bre_ref[ns, ds_].astype(F32)
            bi = dtc * bim_ref[ns, ds_].astype(F32)
            cr = cre_ref[ns, ds_].astype(F32)
            ci = cim_ref[ns, ds_].astype(F32)
            pr = cr * br - ci * bi
            pi_ = cr * bi + ci * br
            for (j0, j1, p) in SEGS:
                mr = mul_ref[p, 0, ns, ds_]
                mi = mul_ref[p, 1, ns, ds_]

                def step(j, carry):
                    pr, pi_ = carry
                    rows = []
                    for _ in range(8):
                        rows.append(jnp.sum(pr, axis=0, keepdims=True))
                        pr, pi_ = pr * mr - pi_ * mi, pr * mi + pi_ * mr
                    js = pl.ds(pl.multiple_of(j * 8, 8), 8)
                    kp_ref[c // 2, js, :] = kp_ref[c // 2, js, :] + jnp.concatenate(rows, 0)
                    return pr, pi_
                pr, pi_ = lax.fori_loop(j0, j1, step, (pr, pi_))
            return cc
        _loop('chunk', 0, 10, chunk)

        kpb = jnp.concatenate([kp_ref[c] for c in range(5)], 1)[:, :D].astype(BF)
        lj = _lval(lax.broadcasted_iota(jnp.int32, (CB, NJ), 1))

        def fwd_dft(i, c):
            lr = (lax.broadcasted_iota(jnp.int32, (CB, NJ), 0) + i * CB).astype(F32)
            m = (lr.astype(BF).astype(F32) == lj).astype(BF)
            kf_ref[i] = _dot(ff, _dot(m, kpb).astype(BF)).astype(BF)
            uf_ref[i] = _dot(ff, u_ref[_rows(i, CB), :]).astype(BF)
            return c
        _loop('fwd_dft', 0, PB, fwd_dft)
        car_ref[...] = jnp.zeros(car_ref.shape, F32)

        def inv(i, c):
            zr_ref[...] = jnp.zeros(zr_ref.shape, F32)
            zi_ref[...] = jnp.zeros(zi_ref.shape, F32)

            def mac(j, cc):
                ur, ui = uf_ref[i - j, 0:CB, :].astype(F32), uf_ref[i - j, CB:2 * CB, :].astype(F32)
                kr, ki = kf_ref[j, 0:CB, :].astype(F32), kf_ref[j, CB:2 * CB, :].astype(F32)
                zr_ref[...] += ur * kr - ui * ki
                zi_ref[...] += ur * ki + ui * kr
                return cc
            lax.fori_loop(0, i + 1, mac, 0)
            z = jnp.concatenate([zr_ref[...].astype(BF), zi_ref[...].astype(BF)], 0)
            yy = _dot(fi, z) * (1.0 / CB)
            r = _rows(i, CB)
            h_ref[r, :] = (x_ref[r, :].astype(F32) + yy[0:CB] + car_ref[...]
                           + u_ref[r, :].astype(F32) * dsk)
            car_ref[...] = yy[CB:2 * CB]
            return c
        _loop('inv', 0, PB, inv)

    pl.run_scoped(s4_fwd, pltpu.VMEM((5, NJ, 128), F32), pltpu.VMEM((CB, D), F32),
                  pltpu.VMEM((CB, D), F32), pltpu.VMEM((CB, D), F32))

    def gmlp(r2_ref, acc_ref):
        for cp in cin[1:]:
            cp.wait()
        def f1(i, c):
            r = _rows(i)
            hn, _ = _ln(h_ref[r, :])
            a = _dot(hn.astype(BF), win_ref[...]).astype(BF)
            a_ref[r, :] = a
            z2n, rr = _ln(_gelu(a[:, FH:].astype(F32)).astype(BF).astype(F32))
            z2_ref[r, :] = z2n.astype(BF)
            r2_ref[r, :] = rr
            return c
        _loop('f1', 0, NT, f1)
        acc_ref[...] = jnp.zeros(acc_ref.shape, F32)

        def f2(i, c):
            r = _rows(i)
            g = (_dot(wsp_ref[r, :], z2_ref[...]) + bsp_ref[r, :].astype(F32)).astype(BF).astype(F32)
            a1 = a_ref[r, 0:FH].astype(F32)
            z1 = _gelu(a1).astype(BF).astype(F32)
            q = (z1 * g).astype(BF)
            out_ref[:, r] = (h_ref[r, :] + _dot_nt(q, wout_ref[...])).T.astype(BF)
            dot_ = dot_ref[:, r]
            do = dot_.astype(F32).T.astype(BF)
            do_ref[r, :] = do
            dq = _dot(do, wout_ref[...])
            acc_ref[...] += _dot(dot_, q)
            dg = (dq * z1).astype(BF)
            g_ref[r, :] = dg
            dbsp_ref[r, :] = jnp.sum(dg.astype(F32), axis=1, keepdims=True).astype(BF)
            a_ref[r, 0:FH] = (dq * g * _dgelu(a1)).astype(BF)
            return c
        _loop('f2', 0, NT, f2)
        dwout_ref[...] = acc_ref[...].astype(BF)
        cout[0].start()
        cout[2].start()

        def f3(i, c):
            r = _rows(i)
            dz2n = _dot_tn(wsp_ref[:, r], g_ref[...])
            dz2 = _lnb(dz2n, z2_ref[r, :].astype(F32), r2_ref[r, :])
            a_ref[r, FH:FF] = (dz2 * _dgelu(a_ref[r, FH:FF].astype(F32))).astype(BF)
            return c
        _loop('f3', 0, NT, f3)

        def f6(i, c):
            r = _rows(i)
            hn, rh = _ln(h_ref[r, :])
            dhn = _dot_nt(a_ref[r, :], win_ref[...])
            h_ref[r, :] = do_ref[r, :].astype(F32) + _lnb(dhn, hn.astype(BF).astype(F32), rh)
            do_ref[r, :] = hn.astype(BF)
            return c
        _loop('f6', 0, NT, f6)

    pl.run_scoped(gmlp, pltpu.VMEM((L, 1), F32), pltpu.VMEM((D, FH), F32))

    def s4_bwd(dyf_ref, dk_ref, dsum_ref, zr_ref, zi_ref, car_ref):
        ff, fi = _dft_mats()
        dsum_ref[...] = jnp.zeros(dsum_ref.shape, F32)

        def cast(i, c):
            r = _rows(i, CB)
            dh = h_ref[r, :]
            dyf_ref[i] = _dot(ff, dh.astype(BF)).astype(BF)
            dsum_ref[...] += jnp.sum(dh * u_ref[r, :].astype(F32), axis=0, keepdims=True)
            return c
        _loop('cast', 0, PB, cast)
        ddsk_ref[...] = dsum_ref[...].astype(BF)

        def corr(rr, ref):
            zr_ref[...] = jnp.zeros(zr_ref.shape, F32)
            zi_ref[...] = jnp.zeros(zi_ref.shape, F32)

            def mac(j, cc):
                yr, yi = dyf_ref[rr + j, 0:CB, :].astype(F32), dyf_ref[rr + j, CB:2 * CB, :].astype(F32)
                kr, ki = ref[j, 0:CB, :].astype(F32), ref[j, CB:2 * CB, :].astype(F32)
                zr_ref[...] += yr * kr + yi * ki
                zi_ref[...] += yi * kr - yr * ki
                return cc
            lax.fori_loop(0, PB - rr, mac, 0)
            z = jnp.concatenate([zr_ref[...].astype(BF), zi_ref[...].astype(BF)], 0)
            yy = _dot(fi, z) * (1.0 / CB)
            res = yy[0:CB] + car_ref[...]
            car_ref[...] = -yy[CB:2 * CB]
            return res

        def inv_dk(i, c):
            rr = PB - 1 - i
            r = _rows(rr, CB)
            dk = corr(rr, uf_ref)
            dkh = dk.astype(BF)
            dk_ref[r, 0:D] = dkh
            dk_ref[r, DP:DP + D] = (dk - dkh.astype(F32)).astype(BF)
            return c

        def inv_du(i, c):
            rr = PB - 1 - i
            r = _rows(rr, CB)
            dh = h_ref[r, :]
            du = corr(rr, kf_ref) + dh * dsk
            u, rx = _ln(x_ref[r, :].astype(F32))
            dx_ref[:, r] = (dh + _lnb(du, u.astype(BF).astype(F32), rx)).T.astype(BF)
            return c
        dk_ref[:, D:DP] = jnp.zeros((L, DP - D), BF)
        dk_ref[:, DP + D:2 * DP] = jnp.zeros((L, DP - D), BF)
        car_ref[...] = jnp.zeros(car_ref.shape, F32)
        _loop('inv_dk', 0, PB, inv_dk)
        car_ref[...] = jnp.zeros(car_ref.shape, F32)
        _loop('inv_du', 0, PB, inv_du)
        cout[4].start()

        def seg(i, c):
            lj = _lval(lax.broadcasted_iota(jnp.int32, (128, L), 0) + i * 128)
            lr = lax.broadcasted_iota(jnp.int32, (128, L), 1).astype(F32)
            mt = (lr.astype(BF).astype(F32) == lj).astype(BF)
            gg = _dot(mt, dk_ref[...])
            gg = gg[:, 0:DP] + gg[:, DP:2 * DP]
            rr = pl.ds(pl.multiple_of(i * 128, 128), 128)
            g1 = gg * lj[:, 0:1]
            for c5 in range(5):
                gp_ref[0, c5, rr, :] = gg[:, c5 * 128:(c5 + 1) * 128]
                gp_ref[1, c5, rr, :] = g1[:, c5 * 128:(c5 + 1) * 128]
            return c
        _loop('seg', 0, NJ // 128, seg)

    pl.run_scoped(s4_bwd, pltpu.VMEM((PB, 2 * CB, D), BF),
                  pltpu.VMEM((L, 2 * DP), BF), pltpu.VMEM((1, D), F32), pltpu.VMEM((CB, D), F32),
                  pltpu.VMEM((CB, D), F32), pltpu.VMEM((CB, D), F32))

    def ssm_bwd(ddt_ref):
        ddt_ref[...] = jnp.zeros(ddt_ref.shape, F32)

        def piece_wsp(pc):
            pc = jnp.minimum(pc, 63)
            rt, ct = _rows(pc // 8), _rows(pc % 8)
            dwsp_ref[rt, ct] = _dot_nt(g_ref[rt, :], z2_ref[ct, :]).astype(BF)

        def piece_win(pc):
            cs = _rows(pc, 128)
            dwin_ref[:, cs] = _dot_tn(do_ref[...], a_ref[:, cs]).astype(BF)

        def chunk(c, cc, c0, piece):
            ns = pl.ds(pl.multiple_of((c % 4) * 32, 32), 32)
            ds_ = pl.ds(pl.multiple_of((c // 4) * 128, 128), 128)
            pr = jnp.ones((32, 128), F32)
            z = jnp.zeros((32, 128), F32)
            st = (pr, z, z, z, z, z)

            def step(j, carry, mr, mi):
                pr, pi_, s0r, s0i, s1r, s1i = carry
                js = pl.ds(pl.multiple_of(j * 8, 8), 8)
                g0t = gp_ref[0, c // 4, js, :]
                g1t = gp_ref[1, c // 4, js, :]
                for t in range(8):
                    g0 = g0t[t:t + 1, :]
                    g1 = g1t[t:t + 1, :]
                    s0r, s0i = s0r + g0 * pr, s0i + g0 * pi_
                    s1r, s1i = s1r + g1 * pr, s1i + g1 * pi_
                    pr, pi_ = pr * mr - pi_ * mi, pr * mi + pi_ * mr
                return (pr, pi_, s0r, s0i, s1r, s1i)

            def body(b, st):
                p = jnp.maximum(b - 1, 0)
                mr = mul_ref[p, 0, ns, ds_]
                mi = mul_ref[p, 1, ns, ds_]
                piece((c - c0) * 5 + b)
                for s16 in range(16):
                    st = step(b * 16 + s16, st, mr, mi)
                return st
            st = lax.fori_loop(0, 5, body, st)
            st = step(80, st, mul_ref[3, 0, ns, ds_], mul_ref[3, 1, ns, ds_])
            _, _, s0r, s0i, s1r, s1i = st
            dtc = jnp.exp(ldt_ref[:, ds_].astype(F32)).astype(BF).astype(F32)
            ar, ai = are_ref[ns, ds_].astype(F32), aim_ref[ns, ds_].astype(F32)
            b_r, b_i = bre_ref[ns, ds_].astype(F32), bim_ref[ns, ds_].astype(F32)
            cr, ci = cre_ref[ns, ds_].astype(F32), cim_ref[ns, ds_].astype(F32)
            br, bi = dtc * b_r, dtc * b_i
            dcre_ref[ns, ds_] = (s0r * br - s0i * bi).astype(BF)
            dcim_ref[ns, ds_] = (-(s0r * bi + s0i * br)).astype(BF)
            dbr = cr * s0r - ci * s0i
            dbi = -(cr * s0i + ci * s0r)
            dbre_ref[ns, ds_] = (dtc * dbr).astype(BF)
            dbim_ref[ns, ds_] = (dtc * dbi).astype(BF)
            wr = cr * br - ci * bi
            wi = cr * bi + ci * br
            dlr = wr * s1r - wi * s1i
            dli = -(wr * s1i + wi * s1r)
            dare_ref[ns, ds_] = (dtc * dlr).astype(BF)
            daim_ref[ns, ds_] = (dtc * dli).astype(BF)
            ddt_ref[:, ds_] += jnp.sum(dlr * ar + dli * ai + dbr * b_r + dbi * b_i, axis=0, keepdims=True)
            return cc
        _loop('chunk_wsp', 0, 13, functools.partial(chunk, c0=0, piece=piece_wsp))
        cout[1].start()
        piece_win(35)
        _loop('chunk_win', 13, 20, functools.partial(chunk, c0=13, piece=piece_win))
        cout[3].start()
        dldt_ref[...] = (ddt_ref[...] * dt).astype(BF)
    pl.run_scoped(ssm_bwd, pltpu.VMEM((1, DP), F32))
    for cp in cout:
        cp.wait()


@jax.jit
def pallas_sequential_preLN__ssm_conv_s4__mixer_gmlp__prompt_kernel(
    A_u: jax.Array,
    A_A_re: jax.Array,
    A_A_im: jax.Array,
    A_B_re: jax.Array,
    A_B_im: jax.Array,
    A_C_re: jax.Array,
    A_C_im: jax.Array,
    A_log_dt: jax.Array,
    A_Dskip: jax.Array,
    B_x: jax.Array,
    B_w_in: jax.Array,
    B_w_sp: jax.Array,
    B_b_sp: jax.Array,
    B_w_out: jax.Array,
    grad_out: jax.Array,
):
    tp = lambda a: jnp.pad(a.T, ((0, 0), (0, DP - D)))
    args = (A_u[0].T, grad_out[0].T, tp(A_A_re), tp(A_A_im), tp(A_B_re), tp(A_B_im), tp(A_C_re), tp(A_C_im),
            jnp.pad(A_log_dt[None, :], ((0, 0), (0, DP - D))), A_Dskip[None, :],
            B_w_in, B_w_sp, B_b_sp[:, None], B_w_out.T)
    sds = lambda *s: jax.ShapeDtypeStruct(s, BF)
    out_shape = (sds(D, L), sds(D, L), sds(N, DP), sds(N, DP), sds(N, DP), sds(N, DP), sds(N, DP), sds(N, DP),
                 sds(1, DP), sds(1, D), sds(D, FF), sds(L, L), sds(L, 1), sds(D, FH))
    vm = pl.BlockSpec(memory_space=pltpu.VMEM)
    an = pl.BlockSpec(memory_space=pl.ANY)
    res = pl.pallas_call(
        _kernel,
        in_specs=[an, an] + [vm] * 8 + [an, an, vm, an],
        out_specs=(an, an) + (vm,) * 8 + (an, an, vm, an),
        out_shape=out_shape,
        scratch_shapes=[pltpu.VMEM((PB, 2 * CB, D), BF), pltpu.VMEM((PB, 2 * CB, D), BF), pltpu.VMEM((L, D), F32),
                        pltpu.VMEM((4, 2, N, DP), F32), pltpu.VMEM((2, 5, NJ, 128), F32),
                        pltpu.VMEM((D, FF), BF),
                        pltpu.VMEM((L, L), BF), pltpu.VMEM((D, FH), BF),
                        pltpu.VMEM((D, L), BF), pltpu.VMEM((D, L), BF), pltpu.VMEM((D, FH), BF),
                        pltpu.VMEM((L, D), BF), pltpu.VMEM((L, D), BF), pltpu.VMEM((L, D), BF),
                        pltpu.VMEM((L, FF), BF), pltpu.VMEM((L, FH), BF), pltpu.VMEM((L, FH), BF),
                        pltpu.SemaphoreType.DMA((10,))],
        compiler_params=pltpu.CompilerParams(vmem_limit_bytes=120 * 1024 * 1024),
    )(*args)
    (out, dx, dare, daim, dbre, dbim, dcre, dcim, dldt, ddsk, dwin, dwsp, dbsp, dwout) = res
    ut = lambda a: a[:, :D].T
    return (out.T[None], dx.T[None], ut(dare), ut(daim), ut(dbre), ut(dbim), ut(dcre), ut(dcim),
            dldt[0, :D], ddsk[0], dwin, dwsp, dbsp[:, 0], dwout.T)
```

```python
import functools
import math

import jax
import jax.numpy as jnp
from jax import lax
import jax.experimental.pallas as pl
import jax.experimental.pallas.tpu as pltpu

F32 = jnp.float32
BF = jnp.bfloat16
L = 2048
D = 576
DP = 640
N = 128
FH = 2304
FF = 4608
NJ = 768
TM = 256
NT = L // TM
GC = math.sqrt(2.0 / math.pi)


def _dot(a, b):
    return jnp.dot(a, b, preferred_element_type=F32)


def _dot_nt(a, b):
    return lax.dot_general(a, b, (((1,), (1,)), ((), ())), preferred_element_type=F32)


def _dot_tn(a, b):
    return lax.dot_general(a, b, (((0,), (0,)), ((), ())), preferred_element_type=F32)


def _ln(x):
    m = jnp.mean(x, axis=-1, keepdims=True)
    c = x - m
    v = jnp.mean(c * c, axis=-1, keepdims=True)
    r = lax.rsqrt(v + 1e-5)
    return c * r, r


def _lnb(dy, y, r):
    return r * (dy - jnp.mean(dy, axis=-1, keepdims=True)
                - y * jnp.mean(dy * y, axis=-1, keepdims=True))


def _gelu(a):
    t = jnp.tanh(GC * (a + 0.044715 * a * a * a))
    return 0.5 * a * (1.0 + t)


def _dgelu(a):
    t = jnp.tanh(GC * (a + 0.044715 * a * a * a))
    return 0.5 * (1.0 + t) + 0.5 * a * (1.0 - t * t) * GC * (1.0 + 3 * 0.044715 * a * a)


def _loop(name, lo, hi, body):
    with jax.named_scope(name):
        lax.fori_loop(lo, hi, body, 0)


def _rows(i, t=TM):
    return pl.ds(pl.multiple_of(i * t, t), t)


CB = 256
PB = L // CB


def _dft_mats():
    k = lax.broadcasted_iota(jnp.int32, (CB, CB), 0)
    t = lax.broadcasted_iota(jnp.int32, (CB, CB), 1)
    ang = (((2 * k + 1) * t) & (4 * CB - 1)).astype(F32) * (math.pi / (2 * CB))
    ff = jnp.concatenate([jnp.cos(ang), -jnp.sin(ang)], 0).astype(BF)
    t = lax.broadcasted_iota(jnp.int32, (2 * CB, CB), 0)
    k = lax.broadcasted_iota(jnp.int32, (2 * CB, CB), 1)
    ang = (((2 * k + 1) * t) & (4 * CB - 1)).astype(F32) * (math.pi / (2 * CB))
    fi = jnp.concatenate([jnp.cos(ang), -jnp.sin(ang)], 1).astype(BF)
    return ff, fi


def _lval(j):
    return jnp.where(j <= 256, j,
                     jnp.where(j <= 384, 256 + 2 * (j - 256),
                               jnp.where(j <= 512, 512 + 4 * (j - 384),
                                         jnp.where(j <= 640, 1024 + 8 * (j - 512), -1)))).astype(F32)


SEGS = ((0, 32, 0), (32, 48, 1), (48, 64, 2), (64, 81, 3))


def _kernel(x_hbm, do_hbm, are_ref, aim_ref, bre_ref, bim_ref, cre_ref, cim_ref,
            ldt_ref, dsk_ref, win_hbm, wsp_hbm, bsp_ref, wout_hbm,
            out_hbm, dx_hbm, dare_ref, daim_ref, dbre_ref, dbim_ref, dcre_ref, dcim_ref,
            dldt_ref, ddsk_ref, dwin_hbm, dwsp_hbm, dbsp_ref, dwout_hbm,
            uf_ref, kf_ref, h_ref, mul_ref, gp_ref,
            win_ref, wsp_ref, wout_ref,
            out_ref, dx_ref, dwout_ref, x_ref, do_ref, u_ref, a_ref, z2_ref, g_ref, sems):
    dwin_ref, dwsp_ref = win_ref, wsp_ref
    xt_ref, dot_ref = out_ref, dx_ref
    cin = [pltpu.make_async_copy(a, b, sems.at[i]) for i, (a, b) in enumerate(
        ((x_hbm, xt_ref), (win_hbm, win_ref), (wsp_hbm, wsp_ref), (wout_hbm, wout_ref), (do_hbm, dot_ref)))]
    cout = [pltpu.make_async_copy(a, b, sems.at[5 + i]) for i, (a, b) in enumerate(
        ((out_ref, out_hbm), (dwsp_ref, dwsp_hbm), (dwout_ref, dwout_hbm), (dwin_ref, dwin_hbm),
         (dx_ref, dx_hbm)))]
    for cp in cin:
        cp.start()
    dsk = dsk_ref[...].astype(F32)
    dt = jnp.exp(ldt_ref[...].astype(F32)).astype(BF).astype(F32)
    lar = dt * are_ref[...].astype(F32)
    lai = dt * aim_ref[...].astype(F32)
    for p in range(4):
        e = jnp.exp(lar * (2.0 ** p))
        mul_ref[p, 0] = e * jnp.cos(lai * (2.0 ** p))
        mul_ref[p, 1] = e * jnp.sin(lai * (2.0 ** p))

    cin[0].wait()
    def ln_x(i, c):
        r = _rows(i)
        x = xt_ref[:, r].astype(F32).T
        x_ref[r, :] = x.astype(BF)
        u, _ = _ln(x)
        u_ref[r, :] = u.astype(BF)
        return c
    _loop('ln_x', 0, NT, ln_x)

    def s4_fwd(kp_ref, zr_ref, zi_ref, car_ref):
        ff, fi = _dft_mats()
        kp_ref[...] = jnp.zeros(kp_ref.shape, F32)

        def chunk(c, cc):
            ns = pl.ds(pl.multiple_of((c % 2) * 64, 64), 64)
            ds_ = pl.ds(pl.multiple_of((c // 2) * 128, 128), 128)
            dtc = jnp.exp(ldt_ref[:, ds_].astype(F32)).astype(BF).astype(F32)
            br = dtc * bre_ref[ns, ds_].astype(F32)
            bi = dtc * bim_ref[ns, ds_].astype(F32)
            cr = cre_ref[ns, ds_].astype(F32)
            ci = cim_ref[ns, ds_].astype(F32)
            pr = cr * br - ci * bi
            pi_ = cr * bi + ci * br
            for (j0, j1, p) in SEGS:
                mr = mul_ref[p, 0, ns, ds_]
                mi = mul_ref[p, 1, ns, ds_]

                def step(j, carry):
                    pr, pi_ = carry
                    rows = []
                    for _ in range(8):
                        rows.append(jnp.sum(pr, axis=0, keepdims=True))
                        pr, pi_ = pr * mr - pi_ * mi, pr * mi + pi_ * mr
                    js = pl.ds(pl.multiple_of(j * 8, 8), 8)
                    kp_ref[c // 2, js, :] = kp_ref[c // 2, js, :] + jnp.concatenate(rows, 0)
                    return pr, pi_
                pr, pi_ = lax.fori_loop(j0, j1, step, (pr, pi_))
            return cc
        _loop('chunk', 0, 10, chunk)

        kpb = jnp.concatenate([kp_ref[c] for c in range(5)], 1)[:, :D].astype(BF)
        lj = _lval(lax.broadcasted_iota(jnp.int32, (CB, NJ), 1))

        def fwd_dft(i, c):
            lr = (lax.broadcasted_iota(jnp.int32, (CB, NJ), 0) + i * CB).astype(F32)
            m = (lr.astype(BF).astype(F32) == lj).astype(BF)
            kf_ref[i] = _dot(ff, _dot(m, kpb).astype(BF)).astype(BF)
            uf_ref[i] = _dot(ff, u_ref[_rows(i, CB), :]).astype(BF)
            return c
        _loop('fwd_dft', 0, PB, fwd_dft)
        car_ref[...] = jnp.zeros(car_ref.shape, F32)

        def inv(i, c):
            zr_ref[...] = jnp.zeros(zr_ref.shape, F32)
            zi_ref[...] = jnp.zeros(zi_ref.shape, F32)

            def mac(j, cc):
                ur, ui = uf_ref[i - j, 0:CB, :].astype(F32), uf_ref[i - j, CB:2 * CB, :].astype(F32)
                kr, ki = kf_ref[j, 0:CB, :].astype(F32), kf_ref[j, CB:2 * CB, :].astype(F32)
                zr_ref[...] += ur * kr - ui * ki
                zi_ref[...] += ur * ki + ui * kr
                return cc
            lax.fori_loop(0, i + 1, mac, 0)
            z = jnp.concatenate([zr_ref[...].astype(BF), zi_ref[...].astype(BF)], 0)
            yy = _dot(fi, z) * (1.0 / CB)
            r = _rows(i, CB)
            h_ref[r, :] = (x_ref[r, :].astype(F32) + yy[0:CB] + car_ref[...]
                           + u_ref[r, :].astype(F32) * dsk)
            car_ref[...] = yy[CB:2 * CB]
            return c
        _loop('inv', 0, PB, inv)

    pl.run_scoped(s4_fwd, pltpu.VMEM((5, NJ, 128), F32), pltpu.VMEM((CB, D), F32),
                  pltpu.VMEM((CB, D), F32), pltpu.VMEM((CB, D), F32))

    def gmlp(r2_ref, acc_ref):
        for cp in cin[1:]:
            cp.wait()
        def f1(i, c):
            r = _rows(i)
            hn, _ = _ln(h_ref[r, :])
            a = _dot(hn.astype(BF), win_ref[...]).astype(BF)
            a_ref[r, :] = a
            z2n, rr = _ln(_gelu(a[:, FH:].astype(F32)).astype(BF).astype(F32))
            z2_ref[r, :] = z2n.astype(BF)
            r2_ref[r, :] = rr
            return c
        _loop('f1', 0, NT, f1)
        acc_ref[...] = jnp.zeros(acc_ref.shape, F32)

        def f2(i, c):
            r = _rows(i)
            g = (_dot(wsp_ref[r, :], z2_ref[...]) + bsp_ref[r, :].astype(F32)).astype(BF).astype(F32)
            a1 = a_ref[r, 0:FH].astype(F32)
            z1 = _gelu(a1).astype(BF).astype(F32)
            q = (z1 * g).astype(BF)
            out_ref[:, r] = (h_ref[r, :] + _dot_nt(q, wout_ref[...])).T.astype(BF)
            dot_ = dot_ref[:, r]
            do = dot_.astype(F32).T.astype(BF)
            do_ref[r, :] = do
            dq = _dot(do, wout_ref[...])
            acc_ref[...] += _dot(dot_, q)
            dg = (dq * z1).astype(BF)
            g_ref[r, :] = dg
            dbsp_ref[r, :] = jnp.sum(dg.astype(F32), axis=1, keepdims=True).astype(BF)
            a_ref[r, 0:FH] = (dq * g * _dgelu(a1)).astype(BF)
            return c
        _loop('f2', 0, NT, f2)
        dwout_ref[...] = acc_ref[...].astype(BF)
        cout[0].start()
        cout[2].start()

        def f3(i, c):
            r = _rows(i)
            dz2n = _dot_tn(wsp_ref[:, r], g_ref[...])
            dz2 = _lnb(dz2n, z2_ref[r, :].astype(F32), r2_ref[r, :])
            a_ref[r, FH:FF] = (dz2 * _dgelu(a_ref[r, FH:FF].astype(F32))).astype(BF)
            return c
        _loop('f3', 0, NT, f3)

        def f6(i, c):
            r = _rows(i)
            hn, rh = _ln(h_ref[r, :])
            dhn = _dot_nt(a_ref[r, :], win_ref[...])
            h_ref[r, :] = do_ref[r, :].astype(F32) + _lnb(dhn, hn.astype(BF).astype(F32), rh)
            do_ref[r, :] = hn.astype(BF)
            return c
        _loop('f6', 0, NT, f6)

    pl.run_scoped(gmlp, pltpu.VMEM((L, 1), F32), pltpu.VMEM((D, FH), F32))

    def s4_bwd(dyf_ref, dk_ref, dsum_ref, zr_ref, zi_ref, car_ref):
        ff, fi = _dft_mats()
        dsum_ref[...] = jnp.zeros(dsum_ref.shape, F32)

        def cast(i, c):
            r = _rows(i, CB)
            dh = h_ref[r, :]
            dyf_ref[i] = _dot(ff, dh.astype(BF)).astype(BF)
            dsum_ref[...] += jnp.sum(dh * u_ref[r, :].astype(F32), axis=0, keepdims=True)
            return c
        _loop('cast', 0, PB, cast)
        ddsk_ref[...] = dsum_ref[...].astype(BF)

        def corr(rr, ref):
            zr_ref[...] = jnp.zeros(zr_ref.shape, F32)
            zi_ref[...] = jnp.zeros(zi_ref.shape, F32)

            def mac(j, cc):
                yr, yi = dyf_ref[rr + j, 0:CB, :].astype(F32), dyf_ref[rr + j, CB:2 * CB, :].astype(F32)
                kr, ki = ref[j, 0:CB, :].astype(F32), ref[j, CB:2 * CB, :].astype(F32)
                zr_ref[...] += yr * kr + yi * ki
                zi_ref[...] += yi * kr - yr * ki
                return cc
            lax.fori_loop(0, PB - rr, mac, 0)
            z = jnp.concatenate([zr_ref[...].astype(BF), zi_ref[...].astype(BF)], 0)
            yy = _dot(fi, z) * (1.0 / CB)
            res = yy[0:CB] + car_ref[...]
            car_ref[...] = -yy[CB:2 * CB]
            return res

        def inv_dk(i, c):
            rr = PB - 1 - i
            r = _rows(rr, CB)
            dk = corr(rr, uf_ref)
            dkh = dk.astype(BF)
            dk_ref[r, 0:D] = dkh
            dk_ref[r, DP:DP + D] = (dk - dkh.astype(F32)).astype(BF)
            return c

        def inv_du(i, c):
            rr = PB - 1 - i
            r = _rows(rr, CB)
            dh = h_ref[r, :]
            du = corr(rr, kf_ref) + dh * dsk
            u, rx = _ln(x_ref[r, :].astype(F32))
            dx_ref[:, r] = (dh + _lnb(du, u.astype(BF).astype(F32), rx)).T.astype(BF)
            return c
        dk_ref[:, D:DP] = jnp.zeros((L, DP - D), BF)
        dk_ref[:, DP + D:2 * DP] = jnp.zeros((L, DP - D), BF)
        car_ref[...] = jnp.zeros(car_ref.shape, F32)
        _loop('inv_dk', 0, PB, inv_dk)
        car_ref[...] = jnp.zeros(car_ref.shape, F32)
        _loop('inv_du', 0, PB, inv_du)
        cout[4].start()

        def seg(i, c):
            lj = _lval(lax.broadcasted_iota(jnp.int32, (128, L), 0) + i * 128)
            lr = lax.broadcasted_iota(jnp.int32, (128, L), 1).astype(F32)
            mt = (lr.astype(BF).astype(F32) == lj).astype(BF)
            gg = _dot(mt, dk_ref[...])
            gg = gg[:, 0:DP] + gg[:, DP:2 * DP]
            rr = pl.ds(pl.multiple_of(i * 128, 128), 128)
            g1 = gg * lj[:, 0:1]
            for c5 in range(5):
                gp_ref[0, c5, rr, :] = gg[:, c5 * 128:(c5 + 1) * 128]
                gp_ref[1, c5, rr, :] = g1[:, c5 * 128:(c5 + 1) * 128]
            return c
        _loop('seg', 0, NJ // 128, seg)

    pl.run_scoped(s4_bwd, pltpu.VMEM((PB, 2 * CB, D), BF),
                  pltpu.VMEM((L, 2 * DP), BF), pltpu.VMEM((1, D), F32), pltpu.VMEM((CB, D), F32),
                  pltpu.VMEM((CB, D), F32), pltpu.VMEM((CB, D), F32))

    def ssm_bwd(ddt_ref):
        ddt_ref[...] = jnp.zeros(ddt_ref.shape, F32)

        def piece_wsp(pc, k, acc):
            pc = jnp.minimum(pc, 63)
            rt, ct = _rows(pc // 8), _rows(pc % 8)
            ks = [k] if k < 15 else [15, 16, 17]
            for kk in ks:
                part = _dot_nt(g_ref[rt, kk * 128:(kk + 1) * 128], z2_ref[ct, kk * 128:(kk + 1) * 128])
                acc = part if acc is None else acc + part
            if k == 15:
                dwsp_ref[rt, ct] = acc.astype(BF)
            return acc

        def piece_win(pc, k, acc):
            cs = _rows(pc, 128)
            part = _dot_tn(do_ref[k * 128:(k + 1) * 128, :], a_ref[k * 128:(k + 1) * 128, cs])
            acc = part if acc is None else acc + part
            if k == 15:
                dwin_ref[:, cs] = acc.astype(BF)
            return acc

        def chunk(c, cc, c0, piece):
            ns = pl.ds(pl.multiple_of((c % 4) * 32, 32), 32)
            ds_ = pl.ds(pl.multiple_of((c // 4) * 128, 128), 128)
            pr = jnp.ones((32, 128), F32)
            z = jnp.zeros((32, 128), F32)
            st = (pr, z, z, z, z, z)

            def step(j, carry, mr, mi):
                pr, pi_, s0r, s0i, s1r, s1i = carry
                js = pl.ds(pl.multiple_of(j * 8, 8), 8)
                g0t = gp_ref[0, c // 4, js, :]
                g1t = gp_ref[1, c // 4, js, :]
                for t in range(8):
                    g0 = g0t[t:t + 1, :]
                    g1 = g1t[t:t + 1, :]
                    s0r, s0i = s0r + g0 * pr, s0i + g0 * pi_
                    s1r, s1i = s1r + g1 * pr, s1i + g1 * pi_
                    pr, pi_ = pr * mr - pi_ * mi, pr * mi + pi_ * mr
                return (pr, pi_, s0r, s0i, s1r, s1i)

            def body(b, st):
                p = jnp.maximum(b - 1, 0)
                mr = mul_ref[p, 0, ns, ds_]
                mi = mul_ref[p, 1, ns, ds_]
                acc = None
                for s16 in range(16):
                    acc = piece((c - c0) * 5 + b, s16, acc)
                    st = step(b * 16 + s16, st, mr, mi)
                return st
            st = lax.fori_loop(0, 5, body, st)
            st = step(80, st, mul_ref[3, 0, ns, ds_], mul_ref[3, 1, ns, ds_])
            _, _, s0r, s0i, s1r, s1i = st
            dtc = jnp.exp(ldt_ref[:, ds_].astype(F32)).astype(BF).astype(F32)
            ar, ai = are_ref[ns, ds_].astype(F32), aim_ref[ns, ds_].astype(F32)
            b_r, b_i = bre_ref[ns, ds_].astype(F32), bim_ref[ns, ds_].astype(F32)
            cr, ci = cre_ref[ns, ds_].astype(F32), cim_ref[ns, ds_].astype(F32)
            br, bi = dtc * b_r, dtc * b_i
            dcre_ref[ns, ds_] = (s0r * br - s0i * bi).astype(BF)
            dcim_ref[ns, ds_] = (-(s0r * bi + s0i * br)).astype(BF)
            dbr = cr * s0r - ci * s0i
            dbi = -(cr * s0i + ci * s0r)
            dbre_ref[ns, ds_] = (dtc * dbr).astype(BF)
            dbim_ref[ns, ds_] = (dtc * dbi).astype(BF)
            wr = cr * br - ci * bi
            wi = cr * bi + ci * br
            dlr = wr * s1r - wi * s1i
            dli = -(wr * s1i + wi * s1r)
            dare_ref[ns, ds_] = (dtc * dlr).astype(BF)
            daim_ref[ns, ds_] = (dtc * dli).astype(BF)
            ddt_ref[:, ds_] += jnp.sum(dlr * ar + dli * ai + dbr * b_r + dbi * b_i, axis=0, keepdims=True)
            return cc
        _loop('chunk_wsp', 0, 13, functools.partial(chunk, c0=0, piece=piece_wsp))
        cout[1].start()
        acc = None
        for k in range(16):
            acc = piece_win(35, k, acc)
        _loop('chunk_win', 13, 20, functools.partial(chunk, c0=13, piece=piece_win))
        cout[3].start()
        dldt_ref[...] = (ddt_ref[...] * dt).astype(BF)
    pl.run_scoped(ssm_bwd, pltpu.VMEM((1, DP), F32))
    for cp in cout:
        cp.wait()


@jax.jit
def pallas_sequential_preLN__ssm_conv_s4__mixer_gmlp__prompt_kernel(
    A_u: jax.Array,
    A_A_re: jax.Array,
    A_A_im: jax.Array,
    A_B_re: jax.Array,
    A_B_im: jax.Array,
    A_C_re: jax.Array,
    A_C_im: jax.Array,
    A_log_dt: jax.Array,
    A_Dskip: jax.Array,
    B_x: jax.Array,
    B_w_in: jax.Array,
    B_w_sp: jax.Array,
    B_b_sp: jax.Array,
    B_w_out: jax.Array,
    grad_out: jax.Array,
):
    tp = lambda a: jnp.pad(a.T, ((0, 0), (0, DP - D)))
    args = (A_u[0].T, grad_out[0].T, tp(A_A_re), tp(A_A_im), tp(A_B_re), tp(A_B_im), tp(A_C_re), tp(A_C_im),
            jnp.pad(A_log_dt[None, :], ((0, 0), (0, DP - D))), A_Dskip[None, :],
            B_w_in, B_w_sp, B_b_sp[:, None], B_w_out.T)
    sds = lambda *s: jax.ShapeDtypeStruct(s, BF)
    out_shape = (sds(D, L), sds(D, L), sds(N, DP), sds(N, DP), sds(N, DP), sds(N, DP), sds(N, DP), sds(N, DP),
                 sds(1, DP), sds(1, D), sds(D, FF), sds(L, L), sds(L, 1), sds(D, FH))
    vm = pl.BlockSpec(memory_space=pltpu.VMEM)
    an = pl.BlockSpec(memory_space=pl.ANY)
    res = pl.pallas_call(
        _kernel,
        in_specs=[an, an] + [vm] * 8 + [an, an, vm, an],
        out_specs=(an, an) + (vm,) * 8 + (an, an, vm, an),
        out_shape=out_shape,
        scratch_shapes=[pltpu.VMEM((PB, 2 * CB, D), BF), pltpu.VMEM((PB, 2 * CB, D), BF), pltpu.VMEM((L, D), F32),
                        pltpu.VMEM((4, 2, N, DP), F32), pltpu.VMEM((2, 5, NJ, 128), F32),
                        pltpu.VMEM((D, FF), BF),
                        pltpu.VMEM((L, L), BF), pltpu.VMEM((D, FH), BF),
                        pltpu.VMEM((D, L), BF), pltpu.VMEM((D, L), BF), pltpu.VMEM((D, FH), BF),
                        pltpu.VMEM((L, D), BF), pltpu.VMEM((L, D), BF), pltpu.VMEM((L, D), BF),
                        pltpu.VMEM((L, FF), BF), pltpu.VMEM((L, FH), BF), pltpu.VMEM((L, FH), BF),
                        pltpu.SemaphoreType.DMA((10,))],
        compiler_params=pltpu.CompilerParams(vmem_limit_bytes=120 * 1024 * 1024),
    )(*args)
    (out, dx, dare, daim, dbre, dbim, dcre, dcim, dldt, ddsk, dwin, dwsp, dbsp, dwout) = res
    ut = lambda a: a[:, :D].T
    return (out.T[None], dx.T[None], ut(dare), ut(daim), ut(dbre), ut(dbim), ut(dcre), ut(dcim),
            dldt[0, :D], ddsk[0], dwin, dwsp, dbsp[:, 0], dwout.T)
```

```python
import functools
import math

import jax
import jax.numpy as jnp
from jax import lax
import jax.experimental.pallas as pl
import jax.experimental.pallas.tpu as pltpu

F32 = jnp.float32
BF = jnp.bfloat16
L = 2048
D = 576
DP = 640
N = 128
FH = 2304
FF = 4608
NJ = 768
TM = 256
NT = L // TM
GC = math.sqrt(2.0 / math.pi)


def _dot(a, b):
    return jnp.dot(a, b, preferred_element_type=F32)


def _dot_nt(a, b):
    return lax.dot_general(a, b, (((1,), (1,)), ((), ())), preferred_element_type=F32)


def _dot_tn(a, b):
    return lax.dot_general(a, b, (((0,), (0,)), ((), ())), preferred_element_type=F32)


def _ln(x):
    m = jnp.mean(x, axis=-1, keepdims=True)
    c = x - m
    v = jnp.mean(c * c, axis=-1, keepdims=True)
    r = lax.rsqrt(v + 1e-5)
    return c * r, r


def _lnb(dy, y, r):
    return r * (dy - jnp.mean(dy, axis=-1, keepdims=True)
                - y * jnp.mean(dy * y, axis=-1, keepdims=True))


def _gelu(a):
    t = jnp.tanh(GC * (a + 0.044715 * a * a * a))
    return 0.5 * a * (1.0 + t)


def _dgelu(a):
    t = jnp.tanh(GC * (a + 0.044715 * a * a * a))
    return 0.5 * (1.0 + t) + 0.5 * a * (1.0 - t * t) * GC * (1.0 + 3 * 0.044715 * a * a)


def _loop(name, lo, hi, body):
    with jax.named_scope(name):
        lax.fori_loop(lo, hi, body, 0)


def _rows(i, t=TM):
    return pl.ds(pl.multiple_of(i * t, t), t)


CB = 256
PB = L // CB


def _dft_mats():
    k = lax.broadcasted_iota(jnp.int32, (CB, CB), 0)
    t = lax.broadcasted_iota(jnp.int32, (CB, CB), 1)
    ang = (((2 * k + 1) * t) & (4 * CB - 1)).astype(F32) * (math.pi / (2 * CB))
    ff = jnp.concatenate([jnp.cos(ang), -jnp.sin(ang)], 0).astype(BF)
    t = lax.broadcasted_iota(jnp.int32, (2 * CB, CB), 0)
    k = lax.broadcasted_iota(jnp.int32, (2 * CB, CB), 1)
    ang = (((2 * k + 1) * t) & (4 * CB - 1)).astype(F32) * (math.pi / (2 * CB))
    fi = jnp.concatenate([jnp.cos(ang), -jnp.sin(ang)], 1).astype(BF)
    return ff, fi


def _lval(j):
    return jnp.where(j <= 256, j,
                     jnp.where(j <= 384, 256 + 2 * (j - 256),
                               jnp.where(j <= 512, 512 + 4 * (j - 384),
                                         jnp.where(j <= 640, 1024 + 8 * (j - 512), -1)))).astype(F32)


SEGS = ((0, 16, 0), (16, 24, 1), (24, 32, 2), (32, 41, 3))


def _kernel(x_hbm, do_hbm, are_ref, aim_ref, bre_ref, bim_ref, cre_ref, cim_ref,
            ldt_ref, dsk_ref, win_hbm, wsp_hbm, bsp_ref, wout_hbm,
            out_hbm, dx_hbm, dare_ref, daim_ref, dbre_ref, dbim_ref, dcre_ref, dcim_ref,
            dldt_ref, ddsk_ref, dwin_hbm, dwsp_hbm, dbsp_ref, dwout_hbm,
            uf_ref, kf_ref, h_ref, mul_ref, gp_ref,
            win_ref, wsp_ref, wout_ref,
            out_ref, dx_ref, dwout_ref, x_ref, do_ref, u_ref, a_ref, z2_ref, g_ref, sems):
    dwin_ref, dwsp_ref = win_ref, wsp_ref
    xt_ref, dot_ref = out_ref, dx_ref
    cin = [pltpu.make_async_copy(a, b, sems.at[i]) for i, (a, b) in enumerate(
        ((x_hbm, xt_ref), (win_hbm, win_ref), (wsp_hbm, wsp_ref), (wout_hbm, wout_ref), (do_hbm, dot_ref)))]
    cout = [pltpu.make_async_copy(a, b, sems.at[5 + i]) for i, (a, b) in enumerate(
        ((out_ref, out_hbm), (dwsp_ref, dwsp_hbm), (dwout_ref, dwout_hbm), (dwin_ref, dwin_hbm),
         (dx_ref, dx_hbm)))]
    for cp in cin:
        cp.start()
    dsk = dsk_ref[...].astype(F32)
    dt = jnp.exp(ldt_ref[...].astype(F32)).astype(BF).astype(F32)
    lar = dt * are_ref[...].astype(F32)
    lai = dt * aim_ref[...].astype(F32)
    for p in range(4):
        e = jnp.exp(lar * (2.0 ** p))
        mul_ref[p, 0] = e * jnp.cos(lai * (2.0 ** p))
        mul_ref[p, 1] = e * jnp.sin(lai * (2.0 ** p))

    cin[0].wait()
    def ln_x(i, c):
        r = _rows(i)
        x = xt_ref[:, r].astype(F32).T
        x_ref[r, :] = x.astype(BF)
        u, _ = _ln(x)
        u_ref[r, :] = u.astype(BF)
        return c
    _loop('ln_x', 0, NT, ln_x)

    def s4_fwd(kp_ref, zr_ref, zi_ref, car_ref, yt_ref):
        ff, fi = _dft_mats()
        kp_ref[...] = jnp.zeros(kp_ref.shape, F32)

        def chunk(c, cc):
            ns = pl.ds(pl.multiple_of((c % 2) * 64, 64), 64)
            ds_ = pl.ds(pl.multiple_of((c // 2) * 128, 128), 128)
            dtc = jnp.exp(ldt_ref[:, ds_].astype(F32)).astype(BF).astype(F32)
            br = dtc * bre_ref[ns, ds_].astype(F32)
            bi = dtc * bim_ref[ns, ds_].astype(F32)
            cr = cre_ref[ns, ds_].astype(F32)
            ci = cim_ref[ns, ds_].astype(F32)
            pr = cr * br - ci * bi
            pi_ = cr * bi + ci * br
            for (j0, j1, p) in SEGS:
                mr = mul_ref[p, 0, ns, ds_]
                mi = mul_ref[p, 1, ns, ds_]
                yr, yi = jnp.ones((64, 128), F32), jnp.zeros((64, 128), F32)
                for o in range(16):
                    yt_ref[0, o] = yr
                    yt_ref[1, o] = yi
                    yr, yi = yr * mr - yi * mi, yr * mi + yi * mr

                def step(j, carry, yr=yr, yi=yi):
                    pr, pi_ = carry
                    rows = []
                    for o in range(16):
                        rows.append(jnp.sum(pr * yt_ref[0, o] - pi_ * yt_ref[1, o], axis=0, keepdims=True))
                    js = pl.ds(pl.multiple_of(j * 16, 16), 16)
                    kp_ref[c // 2, js, :] = kp_ref[c // 2, js, :] + jnp.concatenate(rows, 0)
                    return pr * yr - pi_ * yi, pr * yi + pi_ * yr
                pr, pi_ = lax.fori_loop(j0, j1, step, (pr, pi_))
            return cc
        _loop('chunk', 0, 10, chunk)

        kpb = jnp.concatenate([kp_ref[c] for c in range(5)], 1)[:, :D].astype(BF)
        lj = _lval(lax.broadcasted_iota(jnp.int32, (CB, NJ), 1))

        def fwd_dft(i, c):
            lr = (lax.broadcasted_iota(jnp.int32, (CB, NJ), 0) + i * CB).astype(F32)
            m = (lr.astype(BF).astype(F32) == lj).astype(BF)
            kf_ref[i] = _dot(ff, _dot(m, kpb).astype(BF)).astype(BF)
            uf_ref[i] = _dot(ff, u_ref[_rows(i, CB), :]).astype(BF)
            return c
        _loop('fwd_dft', 0, PB, fwd_dft)
        car_ref[...] = jnp.zeros(car_ref.shape, F32)

        def inv(i, c):
            zr_ref[...] = jnp.zeros(zr_ref.shape, F32)
            zi_ref[...] = jnp.zeros(zi_ref.shape, F32)

            def mac(j, cc):
                ur, ui = uf_ref[i - j, 0:CB, :].astype(F32), uf_ref[i - j, CB:2 * CB, :].astype(F32)
                kr, ki = kf_ref[j, 0:CB, :].astype(F32), kf_ref[j, CB:2 * CB, :].astype(F32)
                zr_ref[...] += ur * kr - ui * ki
                zi_ref[...] += ur * ki + ui * kr
                return cc
            lax.fori_loop(0, i + 1, mac, 0)
            z = jnp.concatenate([zr_ref[...].astype(BF), zi_ref[...].astype(BF)], 0)
            yy = _dot(fi, z) * (1.0 / CB)
            r = _rows(i, CB)
            h_ref[r, :] = (x_ref[r, :].astype(F32) + yy[0:CB] + car_ref[...]
                           + u_ref[r, :].astype(F32) * dsk)
            car_ref[...] = yy[CB:2 * CB]
            return c
        _loop('inv', 0, PB, inv)

    pl.run_scoped(s4_fwd, pltpu.VMEM((5, NJ, 128), F32), pltpu.VMEM((CB, D), F32),
                  pltpu.VMEM((CB, D), F32), pltpu.VMEM((CB, D), F32), pltpu.VMEM((2, 16, 64, 128), F32))

    def gmlp(r2_ref, acc_ref):
        for cp in cin[1:]:
            cp.wait()
        def f1(i, c):
            r = _rows(i)
            hn, _ = _ln(h_ref[r, :])
            a = _dot(hn.astype(BF), win_ref[...]).astype(BF)
            a_ref[r, :] = a
            z2n, rr = _ln(_gelu(a[:, FH:].astype(F32)).astype(BF).astype(F32))
            z2_ref[r, :] = z2n.astype(BF)
            r2_ref[r, :] = rr
            return c
        _loop('f1', 0, NT, f1)
        acc_ref[...] = jnp.zeros(acc_ref.shape, F32)

        def f2(i, c):
            r = _rows(i)
            g = (_dot(wsp_ref[r, :], z2_ref[...]) + bsp_ref[r, :].astype(F32)).astype(BF).astype(F32)
            a1 = a_ref[r, 0:FH].astype(F32)
            z1 = _gelu(a1).astype(BF).astype(F32)
            q = (z1 * g).astype(BF)
            out_ref[:, r] = (h_ref[r, :] + _dot_nt(q, wout_ref[...])).T.astype(BF)
            dot_ = dot_ref[:, r]
            do = dot_.astype(F32).T.astype(BF)
            do_ref[r, :] = do
            dq = _dot(do, wout_ref[...])
            acc_ref[...] += _dot(dot_, q)
            dg = (dq * z1).astype(BF)
            g_ref[r, :] = dg
            dbsp_ref[r, :] = jnp.sum(dg.astype(F32), axis=1, keepdims=True).astype(BF)
            a_ref[r, 0:FH] = (dq * g * _dgelu(a1)).astype(BF)
            return c
        _loop('f2', 0, NT, f2)
        dwout_ref[...] = acc_ref[...].astype(BF)
        cout[0].start()
        cout[2].start()

        def f3(i, c):
            r = _rows(i)
            dz2n = _dot_tn(wsp_ref[:, r], g_ref[...])
            dz2 = _lnb(dz2n, z2_ref[r, :].astype(F32), r2_ref[r, :])
            a_ref[r, FH:FF] = (dz2 * _dgelu(a_ref[r, FH:FF].astype(F32))).astype(BF)
            return c
        _loop('f3', 0, NT, f3)

        def f6(i, c):
            r = _rows(i)
            hn, rh = _ln(h_ref[r, :])
            dhn = _dot_nt(a_ref[r, :], win_ref[...])
            h_ref[r, :] = do_ref[r, :].astype(F32) + _lnb(dhn, hn.astype(BF).astype(F32), rh)
            do_ref[r, :] = hn.astype(BF)
            return c
        _loop('f6', 0, NT, f6)

        def dwsp(i, c):
            r = _rows(i)
            dwsp_ref[r, :] = _dot_nt(g_ref[r, :], z2_ref[...]).astype(BF)
            return c
        _loop('dwsp', 0, NT, dwsp)
        cout[1].start()

        def dwin(i, c):
            cs = pl.ds(pl.multiple_of(i * 512, 512), 512)
            dwin_ref[:, cs] = _dot_tn(do_ref[...], a_ref[:, cs]).astype(BF)
            return c
        _loop('dwin', 0, FF // 512, dwin)
        cout[3].start()

    pl.run_scoped(gmlp, pltpu.VMEM((L, 1), F32), pltpu.VMEM((D, FH), F32))

    def s4_bwd(dyf_ref, dk_ref, dsum_ref, zr_ref, zi_ref, car_ref):
        ff, fi = _dft_mats()
        dsum_ref[...] = jnp.zeros(dsum_ref.shape, F32)

        def cast(i, c):
            r = _rows(i, CB)
            dh = h_ref[r, :]
            dyf_ref[i] = _dot(ff, dh.astype(BF)).astype(BF)
            dsum_ref[...] += jnp.sum(dh * u_ref[r, :].astype(F32), axis=0, keepdims=True)
            return c
        _loop('cast', 0, PB, cast)
        ddsk_ref[...] = dsum_ref[...].astype(BF)

        def corr(rr, ref):
            zr_ref[...] = jnp.zeros(zr_ref.shape, F32)
            zi_ref[...] = jnp.zeros(zi_ref.shape, F32)

            def mac(j, cc):
                yr, yi = dyf_ref[rr + j, 0:CB, :].astype(F32), dyf_ref[rr + j, CB:2 * CB, :].astype(F32)
                kr, ki = ref[j, 0:CB, :].astype(F32), ref[j, CB:2 * CB, :].astype(F32)
                zr_ref[...] += yr * kr + yi * ki
                zi_ref[...] += yi * kr - yr * ki
                return cc
            lax.fori_loop(0, PB - rr, mac, 0)
            z = jnp.concatenate([zr_ref[...].astype(BF), zi_ref[...].astype(BF)], 0)
            yy = _dot(fi, z) * (1.0 / CB)
            res = yy[0:CB] + car_ref[...]
            car_ref[...] = -yy[CB:2 * CB]
            return res

        def inv_dk(i, c):
            rr = PB - 1 - i
            r = _rows(rr, CB)
            dk = corr(rr, uf_ref)
            dkh = dk.astype(BF)
            dk_ref[r, 0:D] = dkh
            dk_ref[r, DP:DP + D] = (dk - dkh.astype(F32)).astype(BF)
            return c

        def inv_du(i, c):
            rr = PB - 1 - i
            r = _rows(rr, CB)
            dh = h_ref[r, :]
            du = corr(rr, kf_ref) + dh * dsk
            u, rx = _ln(x_ref[r, :].astype(F32))
            dx_ref[:, r] = (dh + _lnb(du, u.astype(BF).astype(F32), rx)).T.astype(BF)
            return c
        dk_ref[:, D:DP] = jnp.zeros((L, DP - D), BF)
        dk_ref[:, DP + D:2 * DP] = jnp.zeros((L, DP - D), BF)
        car_ref[...] = jnp.zeros(car_ref.shape, F32)
        _loop('inv_dk', 0, PB, inv_dk)
        car_ref[...] = jnp.zeros(car_ref.shape, F32)
        _loop('inv_du', 0, PB, inv_du)
        cout[4].start()

        def seg(i, c):
            lj = _lval(lax.broadcasted_iota(jnp.int32, (128, L), 0) + i * 128)
            lr = lax.broadcasted_iota(jnp.int32, (128, L), 1).astype(F32)
            mt = (lr.astype(BF).astype(F32) == lj).astype(BF)
            gg = _dot(mt, dk_ref[...])
            gg = gg[:, 0:DP] + gg[:, DP:2 * DP]
            rr = pl.ds(pl.multiple_of(i * 128, 128), 128)
            g1 = gg * lj[:, 0:1]
            for c5 in range(5):
                gp_ref[0, c5, rr, :] = gg[:, c5 * 128:(c5 + 1) * 128]
                gp_ref[1, c5, rr, :] = g1[:, c5 * 128:(c5 + 1) * 128]
            return c
        _loop('seg', 0, NJ // 128, seg)

    pl.run_scoped(s4_bwd, pltpu.VMEM((PB, 2 * CB, D), BF),
                  pltpu.VMEM((L, 2 * DP), BF), pltpu.VMEM((1, D), F32), pltpu.VMEM((CB, D), F32),
                  pltpu.VMEM((CB, D), F32), pltpu.VMEM((CB, D), F32))

    def ssm_bwd(ddt_ref, yt_ref):
        ddt_ref[...] = jnp.zeros(ddt_ref.shape, F32)

        def chunk(c, cc):
            ns = pl.ds(pl.multiple_of((c % 4) * 32, 32), 32)
            ds_ = pl.ds(pl.multiple_of((c // 4) * 128, 128), 128)
            pr = jnp.ones((32, 128), F32)
            z = jnp.zeros((32, 128), F32)
            st = (pr, z, z, z, z, z)
            for (j0, j1, p) in SEGS:
                mr = mul_ref[p, 0, ns, ds_]
                mi = mul_ref[p, 1, ns, ds_]
                yr, yi = jnp.ones((32, 128), F32), jnp.zeros((32, 128), F32)
                for o in range(16):
                    yt_ref[0, o] = yr
                    yt_ref[1, o] = yi
                    yr, yi = yr * mr - yi * mi, yr * mi + yi * mr

                def step(j, carry, yr=yr, yi=yi):
                    pr, pi_, s0r, s0i, s1r, s1i = carry
                    js = pl.ds(pl.multiple_of(j * 16, 16), 16)
                    g0t = gp_ref[0, c // 4, js, :]
                    g1t = gp_ref[1, c // 4, js, :]
                    t0r = t0i = t1r = t1i = None
                    for o in range(16):
                        g0 = g0t[o:o + 1, :]
                        g1 = g1t[o:o + 1, :]
                        a_, b_ = yt_ref[0, o], yt_ref[1, o]
                        if o == 0:
                            t0r, t0i, t1r, t1i = g0 * a_, g0 * b_, g1 * a_, g1 * b_
                        else:
                            t0r, t0i = t0r + g0 * a_, t0i + g0 * b_
                            t1r, t1i = t1r + g1 * a_, t1i + g1 * b_
                    return (pr * yr - pi_ * yi, pr * yi + pi_ * yr,
                            s0r + pr * t0r - pi_ * t0i, s0i + pr * t0i + pi_ * t0r,
                            s1r + pr * t1r - pi_ * t1i, s1i + pr * t1i + pi_ * t1r)
                st = lax.fori_loop(j0, j1, step, st)
            _, _, s0r, s0i, s1r, s1i = st
            dtc = jnp.exp(ldt_ref[:, ds_].astype(F32)).astype(BF).astype(F32)
            ar, ai = are_ref[ns, ds_].astype(F32), aim_ref[ns, ds_].astype(F32)
            b_r, b_i = bre_ref[ns, ds_].astype(F32), bim_ref[ns, ds_].astype(F32)
            cr, ci = cre_ref[ns, ds_].astype(F32), cim_ref[ns, ds_].astype(F32)
            br, bi = dtc * b_r, dtc * b_i
            dcre_ref[ns, ds_] = (s0r * br - s0i * bi).astype(BF)
            dcim_ref[ns, ds_] = (-(s0r * bi + s0i * br)).astype(BF)
            dbr = cr * s0r - ci * s0i
            dbi = -(cr * s0i + ci * s0r)
            dbre_ref[ns, ds_] = (dtc * dbr).astype(BF)
            dbim_ref[ns, ds_] = (dtc * dbi).astype(BF)
            wr = cr * br - ci * bi
            wi = cr * bi + ci * br
            dlr = wr * s1r - wi * s1i
            dli = -(wr * s1i + wi * s1r)
            dare_ref[ns, ds_] = (dtc * dlr).astype(BF)
            daim_ref[ns, ds_] = (dtc * dli).astype(BF)
            ddt_ref[:, ds_] += jnp.sum(dlr * ar + dli * ai + dbr * b_r + dbi * b_i, axis=0, keepdims=True)
            return cc
        _loop('chunkb', 0, 20, chunk)
        dldt_ref[...] = (ddt_ref[...] * dt).astype(BF)
    pl.run_scoped(ssm_bwd, pltpu.VMEM((1, DP), F32), pltpu.VMEM((2, 16, 32, 128), F32))
    for cp in cout:
        cp.wait()


@jax.jit
def pallas_sequential_preLN__ssm_conv_s4__mixer_gmlp__prompt_kernel(
    A_u: jax.Array,
    A_A_re: jax.Array,
    A_A_im: jax.Array,
    A_B_re: jax.Array,
    A_B_im: jax.Array,
    A_C_re: jax.Array,
    A_C_im: jax.Array,
    A_log_dt: jax.Array,
    A_Dskip: jax.Array,
    B_x: jax.Array,
    B_w_in: jax.Array,
    B_w_sp: jax.Array,
    B_b_sp: jax.Array,
    B_w_out: jax.Array,
    grad_out: jax.Array,
):
    tp = lambda a: jnp.pad(a.T, ((0, 0), (0, DP - D)))
    args = (A_u[0].T, grad_out[0].T, tp(A_A_re), tp(A_A_im), tp(A_B_re), tp(A_B_im), tp(A_C_re), tp(A_C_im),
            jnp.pad(A_log_dt[None, :], ((0, 0), (0, DP - D))), A_Dskip[None, :],
            B_w_in, B_w_sp, B_b_sp[:, None], B_w_out.T)
    sds = lambda *s: jax.ShapeDtypeStruct(s, BF)
    out_shape = (sds(D, L), sds(D, L), sds(N, DP), sds(N, DP), sds(N, DP), sds(N, DP), sds(N, DP), sds(N, DP),
                 sds(1, DP), sds(1, D), sds(D, FF), sds(L, L), sds(L, 1), sds(D, FH))
    vm = pl.BlockSpec(memory_space=pltpu.VMEM)
    an = pl.BlockSpec(memory_space=pl.ANY)
    res = pl.pallas_call(
        _kernel,
        in_specs=[an, an] + [vm] * 8 + [an, an, vm, an],
        out_specs=(an, an) + (vm,) * 8 + (an, an, vm, an),
        out_shape=out_shape,
        scratch_shapes=[pltpu.VMEM((PB, 2 * CB, D), BF), pltpu.VMEM((PB, 2 * CB, D), BF), pltpu.VMEM((L, D), F32),
                        pltpu.VMEM((4, 2, N, DP), F32), pltpu.VMEM((2, 5, NJ, 128), F32),
                        pltpu.VMEM((D, FF), BF),
                        pltpu.VMEM((L, L), BF), pltpu.VMEM((D, FH), BF),
                        pltpu.VMEM((D, L), BF), pltpu.VMEM((D, L), BF), pltpu.VMEM((D, FH), BF),
                        pltpu.VMEM((L, D), BF), pltpu.VMEM((L, D), BF), pltpu.VMEM((L, D), BF),
                        pltpu.VMEM((L, FF), BF), pltpu.VMEM((L, FH), BF), pltpu.VMEM((L, FH), BF),
                        pltpu.SemaphoreType.DMA((10,))],
        compiler_params=pltpu.CompilerParams(vmem_limit_bytes=120 * 1024 * 1024),
    )(*args)
    (out, dx, dare, daim, dbre, dbim, dcre, dcim, dldt, ddsk, dwin, dwsp, dbsp, dwout) = res
    ut = lambda a: a[:, :D].T
    return (out.T[None], dx.T[None], ut(dare), ut(daim), ut(dbre), ut(dbim), ut(dcre), ut(dcim),
            dldt[0, :D], ddsk[0], dwin, dwsp, dbsp[:, 0], dwout.T)
```

```python
import functools
import math

import jax
import jax.numpy as jnp
from jax import lax
import jax.experimental.pallas as pl
import jax.experimental.pallas.tpu as pltpu

F32 = jnp.float32
BF = jnp.bfloat16
L = 2048
D = 576
DP = 640
N = 128
FH = 2304
FF = 4608
NJ = 768
TM = 256
NT = L // TM
GC = math.sqrt(2.0 / math.pi)


def _dot(a, b):
    return jnp.dot(a, b, preferred_element_type=F32)


def _dot_nt(a, b):
    return lax.dot_general(a, b, (((1,), (1,)), ((), ())), preferred_element_type=F32)


def _dot_tn(a, b):
    return lax.dot_general(a, b, (((0,), (0,)), ((), ())), preferred_element_type=F32)


def _ln(x):
    m = jnp.mean(x, axis=-1, keepdims=True)
    c = x - m
    v = jnp.mean(c * c, axis=-1, keepdims=True)
    r = lax.rsqrt(v + 1e-5)
    return c * r, r


def _lnb(dy, y, r):
    return r * (dy - jnp.mean(dy, axis=-1, keepdims=True)
                - y * jnp.mean(dy * y, axis=-1, keepdims=True))


def _gelu(a):
    t = jnp.tanh(GC * (a + 0.044715 * a * a * a))
    return 0.5 * a * (1.0 + t)


def _dgelu(a):
    t = jnp.tanh(GC * (a + 0.044715 * a * a * a))
    return 0.5 * (1.0 + t) + 0.5 * a * (1.0 - t * t) * GC * (1.0 + 3 * 0.044715 * a * a)


def _loop(name, lo, hi, body):
    with jax.named_scope(name):
        lax.fori_loop(lo, hi, body, 0)


def _rows(i, t=TM):
    return pl.ds(pl.multiple_of(i * t, t), t)


CB = 256
PB = L // CB


def _dft_mats():
    k = lax.broadcasted_iota(jnp.int32, (CB, CB), 0)
    t = lax.broadcasted_iota(jnp.int32, (CB, CB), 1)
    ang = (((2 * k + 1) * t) & (4 * CB - 1)).astype(F32) * (math.pi / (2 * CB))
    ff = jnp.concatenate([jnp.cos(ang), -jnp.sin(ang)], 0).astype(BF)
    t = lax.broadcasted_iota(jnp.int32, (2 * CB, CB), 0)
    k = lax.broadcasted_iota(jnp.int32, (2 * CB, CB), 1)
    ang = (((2 * k + 1) * t) & (4 * CB - 1)).astype(F32) * (math.pi / (2 * CB))
    fi = jnp.concatenate([jnp.cos(ang), -jnp.sin(ang)], 1).astype(BF)
    return ff, fi


def _lval(j):
    return jnp.where(j <= 256, j,
                     jnp.where(j <= 384, 256 + 2 * (j - 256),
                               jnp.where(j <= 512, 512 + 4 * (j - 384),
                                         jnp.where(j <= 640, 1024 + 8 * (j - 512), -1)))).astype(F32)


SEGS = ((0, 16, 0), (16, 24, 1), (24, 32, 2), (32, 41, 3))


def _kernel(x_hbm, do_hbm, are_ref, aim_ref, bre_ref, bim_ref, cre_ref, cim_ref,
            ldt_ref, dsk_ref, win_hbm, wsp_hbm, bsp_ref, wout_hbm,
            out_hbm, dx_hbm, dare_ref, daim_ref, dbre_ref, dbim_ref, dcre_ref, dcim_ref,
            dldt_ref, ddsk_ref, dwin_hbm, dwsp_hbm, dbsp_ref, dwout_hbm,
            uf_ref, kf_ref, h_ref, mul_ref, gp_ref,
            win_ref, wsp_ref, wout_ref,
            out_ref, dx_ref, dwout_ref, x_ref, do_ref, u_ref, a_ref, z2_ref, g_ref, sems):
    dwin_ref, dwsp_ref = win_ref, wsp_ref
    xt_ref, dot_ref = out_ref, dx_ref
    cin = [pltpu.make_async_copy(a, b, sems.at[i]) for i, (a, b) in enumerate(
        ((x_hbm, xt_ref), (win_hbm, win_ref), (wsp_hbm, wsp_ref), (wout_hbm, wout_ref), (do_hbm, dot_ref)))]
    cout = [pltpu.make_async_copy(a, b, sems.at[5 + i]) for i, (a, b) in enumerate(
        ((out_ref, out_hbm), (dwsp_ref, dwsp_hbm), (dwout_ref, dwout_hbm), (dwin_ref, dwin_hbm),
         (dx_ref, dx_hbm)))]
    for cp in cin:
        cp.start()
    dsk = dsk_ref[...].astype(F32)
    dt = jnp.exp(ldt_ref[...].astype(F32)).astype(BF).astype(F32)
    lar = dt * are_ref[...].astype(F32)
    lai = dt * aim_ref[...].astype(F32)
    for p in range(4):
        e = jnp.exp(lar * (2.0 ** p))
        mul_ref[p, 0] = e * jnp.cos(lai * (2.0 ** p))
        mul_ref[p, 1] = e * jnp.sin(lai * (2.0 ** p))

    cin[0].wait()
    def ln_x(i, c):
        r = _rows(i)
        x = xt_ref[:, r].astype(F32).T
        x_ref[r, :] = x.astype(BF)
        u, _ = _ln(x)
        u_ref[r, :] = u.astype(BF)
        return c
    _loop('ln_x', 0, NT, ln_x)

    def s4_fwd(kp_ref, zr_ref, zi_ref, car_ref, yt_ref, kpb_ref):
        ff, fi = _dft_mats()
        kp_ref[...] = jnp.zeros(kp_ref.shape, F32)

        def chunk(c, cc):
            ns = pl.ds(pl.multiple_of((c % 2) * 64, 64), 64)
            ds_ = pl.ds(pl.multiple_of((c // 2) * 128, 128), 128)
            dtc = jnp.exp(ldt_ref[:, ds_].astype(F32)).astype(BF).astype(F32)
            br = dtc * bre_ref[ns, ds_].astype(F32)
            bi = dtc * bim_ref[ns, ds_].astype(F32)
            cr = cre_ref[ns, ds_].astype(F32)
            ci = cim_ref[ns, ds_].astype(F32)
            pr = cr * br - ci * bi
            pi_ = cr * bi + ci * br
            for (j0, j1, p) in SEGS:
                mr = mul_ref[p, 0, ns, ds_]
                mi = mul_ref[p, 1, ns, ds_]
                yr, yi = jnp.ones((64, 128), F32), jnp.zeros((64, 128), F32)
                for o in range(16):
                    yt_ref[0, o] = yr
                    yt_ref[1, o] = yi
                    yr, yi = yr * mr - yi * mi, yr * mi + yi * mr

                def step(j, carry, yr=yr, yi=yi):
                    pr, pi_ = carry
                    rows = []
                    for o in range(16):
                        rows.append(jnp.sum(pr * yt_ref[0, o] - pi_ * yt_ref[1, o], axis=0, keepdims=True))
                    js = pl.ds(pl.multiple_of(j * 16, 16), 16)
                    kp_ref[c // 2, js, :] = kp_ref[c // 2, js, :] + jnp.concatenate(rows, 0)
                    return pr * yr - pi_ * yi, pr * yi + pi_ * yr
                pr, pi_ = lax.fori_loop(j0, j1, step, (pr, pi_))
            return cc
        _loop('chunk', 0, 10, chunk)

        kpb = jnp.concatenate([kp_ref[c] for c in range(5)], 1)[:, :D].astype(BF)
        kpb_ref[...] = kpb

        def fwd_dft(i, c):
            j0 = jnp.where(i == 0, 0, jnp.where(i == 1, 256, jnp.where(i < 4, 384, 512)))
            j0 = pl.multiple_of(j0, 128)
            lj = _lval(lax.broadcasted_iota(jnp.int32, (CB, 256), 1) + j0)
            lr = (lax.broadcasted_iota(jnp.int32, (CB, 256), 0) + i * CB).astype(F32)
            m = (lr.astype(BF).astype(F32) == lj).astype(BF)
            kf_ref[i] = _dot(ff, _dot(m, kpb_ref[pl.ds(j0, 256), :]).astype(BF)).astype(BF)
            uf_ref[i] = _dot(ff, u_ref[_rows(i, CB), :]).astype(BF)
            return c
        _loop('fwd_dft', 0, PB, fwd_dft)
        car_ref[...] = jnp.zeros(car_ref.shape, F32)

        def inv(i, c):
            zr_ref[...] = jnp.zeros(zr_ref.shape, F32)
            zi_ref[...] = jnp.zeros(zi_ref.shape, F32)

            def mac(j, cc):
                ur, ui = uf_ref[i - j, 0:CB, :].astype(F32), uf_ref[i - j, CB:2 * CB, :].astype(F32)
                kr, ki = kf_ref[j, 0:CB, :].astype(F32), kf_ref[j, CB:2 * CB, :].astype(F32)
                zr_ref[...] += ur * kr - ui * ki
                zi_ref[...] += ur * ki + ui * kr
                return cc
            lax.fori_loop(0, i + 1, mac, 0)
            z = jnp.concatenate([zr_ref[...].astype(BF), zi_ref[...].astype(BF)], 0)
            yy = _dot(fi, z) * (1.0 / CB)
            r = _rows(i, CB)
            h_ref[r, :] = (x_ref[r, :].astype(F32) + yy[0:CB] + car_ref[...]
                           + u_ref[r, :].astype(F32) * dsk)
            car_ref[...] = yy[CB:2 * CB]
            return c
        _loop('inv', 0, PB, inv)

    pl.run_scoped(s4_fwd, pltpu.VMEM((5, NJ, 128), F32), pltpu.VMEM((CB, D), F32),
                  pltpu.VMEM((CB, D), F32), pltpu.VMEM((CB, D), F32), pltpu.VMEM((2, 16, 64, 128), F32),
                  pltpu.VMEM((NJ, D), BF))

    def gmlp(r2_ref, acc_ref):
        for cp in cin[1:]:
            cp.wait()
        def f1(i, c):
            r = _rows(i)
            hn, _ = _ln(h_ref[r, :])
            a = _dot(hn.astype(BF), win_ref[...]).astype(BF)
            a_ref[r, :] = a
            z2n, rr = _ln(_gelu(a[:, FH:].astype(F32)).astype(BF).astype(F32))
            z2_ref[r, :] = z2n.astype(BF)
            r2_ref[r, :] = rr
            return c
        _loop('f1', 0, NT, f1)
        acc_ref[...] = jnp.zeros(acc_ref.shape, F32)

        def f2(i, c):
            r = _rows(i)
            g = (_dot(wsp_ref[r, :], z2_ref[...]) + bsp_ref[r, :].astype(F32)).astype(BF).astype(F32)
            a1 = a_ref[r, 0:FH].astype(F32)
            z1 = _gelu(a1).astype(BF).astype(F32)
            q = (z1 * g).astype(BF)
            out_ref[:, r] = (h_ref[r, :] + _dot_nt(q, wout_ref[...])).T.astype(BF)
            dot_ = dot_ref[:, r]
            do = dot_.astype(F32).T.astype(BF)
            do_ref[r, :] = do
            dq = _dot(do, wout_ref[...])
            acc_ref[...] += _dot(dot_, q)
            dg = (dq * z1).astype(BF)
            g_ref[r, :] = dg
            dbsp_ref[r, :] = jnp.sum(dg.astype(F32), axis=1, keepdims=True).astype(BF)
            a_ref[r, 0:FH] = (dq * g * _dgelu(a1)).astype(BF)
            return c
        _loop('f2', 0, NT, f2)
        dwout_ref[...] = acc_ref[...].astype(BF)
        cout[0].start()
        cout[2].start()

        def f3(i, c):
            r = _rows(i)
            dz2n = _dot_tn(wsp_ref[:, r], g_ref[...])
            dz2 = _lnb(dz2n, z2_ref[r, :].astype(F32), r2_ref[r, :])
            a_ref[r, FH:FF] = (dz2 * _dgelu(a_ref[r, FH:FF].astype(F32))).astype(BF)
            return c
        _loop('f3', 0, NT, f3)

        def f6(i, c):
            r = _rows(i)
            hn, rh = _ln(h_ref[r, :])
            dhn = _dot_nt(a_ref[r, :], win_ref[...])
            h_ref[r, :] = do_ref[r, :].astype(F32) + _lnb(dhn, hn.astype(BF).astype(F32), rh)
            do_ref[r, :] = hn.astype(BF)
            return c
        _loop('f6', 0, NT, f6)

        def dwsp(i, c):
            r = _rows(i)
            dwsp_ref[r, :] = _dot_nt(g_ref[r, :], z2_ref[...]).astype(BF)
            return c
        _loop('dwsp', 0, NT, dwsp)
        cout[1].start()

        def dwin(i, c):
            cs = pl.ds(pl.multiple_of(i * 512, 512), 512)
            dwin_ref[:, cs] = _dot_tn(do_ref[...], a_ref[:, cs]).astype(BF)
            return c
        _loop('dwin', 0, FF // 512, dwin)
        cout[3].start()

    pl.run_scoped(gmlp, pltpu.VMEM((L, 1), F32), pltpu.VMEM((D, FH), F32))

    def s4_bwd(dyf_ref, dk_ref, dsum_ref, zr_ref, zi_ref, car_ref):
        ff, fi = _dft_mats()
        dsum_ref[...] = jnp.zeros(dsum_ref.shape, F32)

        def cast(i, c):
            r = _rows(i, CB)
            dh = h_ref[r, :]
            dyf_ref[i] = _dot(ff, dh.astype(BF)).astype(BF)
            dsum_ref[...] += jnp.sum(dh * u_ref[r, :].astype(F32), axis=0, keepdims=True)
            return c
        _loop('cast', 0, PB, cast)
        ddsk_ref[...] = dsum_ref[...].astype(BF)

        def corr(rr, ref):
            zr_ref[...] = jnp.zeros(zr_ref.shape, F32)
            zi_ref[...] = jnp.zeros(zi_ref.shape, F32)

            def mac(j, cc):
                yr, yi = dyf_ref[rr + j, 0:CB, :].astype(F32), dyf_ref[rr + j, CB:2 * CB, :].astype(F32)
                kr, ki = ref[j, 0:CB, :].astype(F32), ref[j, CB:2 * CB, :].astype(F32)
                zr_ref[...] += yr * kr + yi * ki
                zi_ref[...] += yi * kr - yr * ki
                return cc
            lax.fori_loop(0, PB - rr, mac, 0)
            z = jnp.concatenate([zr_ref[...].astype(BF), zi_ref[...].astype(BF)], 0)
            yy = _dot(fi, z) * (1.0 / CB)
            res = yy[0:CB] + car_ref[...]
            car_ref[...] = -yy[CB:2 * CB]
            return res

        def inv_dk(i, c):
            rr = PB - 1 - i
            r = _rows(rr, CB)
            dk = corr(rr, uf_ref)
            dkh = dk.astype(BF)
            dk_ref[r, 0:D] = dkh
            dk_ref[r, DP:DP + D] = (dk - dkh.astype(F32)).astype(BF)
            return c

        def inv_du(i, c):
            rr = PB - 1 - i
            r = _rows(rr, CB)
            dh = h_ref[r, :]
            du = corr(rr, kf_ref) + dh * dsk
            u, rx = _ln(x_ref[r, :].astype(F32))
            dx_ref[:, r] = (dh + _lnb(du, u.astype(BF).astype(F32), rx)).T.astype(BF)
            return c
        dk_ref[:, D:DP] = jnp.zeros((L, DP - D), BF)
        dk_ref[:, DP + D:2 * DP] = jnp.zeros((L, DP - D), BF)
        car_ref[...] = jnp.zeros(car_ref.shape, F32)
        _loop('inv_dk', 0, PB, inv_dk)
        car_ref[...] = jnp.zeros(car_ref.shape, F32)
        _loop('inv_du', 0, PB, inv_du)
        cout[4].start()

        for i, (l0, l1) in enumerate(((0, 128), (128, 256), (256, 512), (384, 1024), (896, 2048), (1920, 2048))):
            w = l1 - l0
            lj = _lval(lax.broadcasted_iota(jnp.int32, (128, w), 0) + i * 128)
            lr = (lax.broadcasted_iota(jnp.int32, (128, w), 1) + l0).astype(F32)
            mt = (lr.astype(BF).astype(F32) == lj).astype(BF)
            gg = _dot(mt, dk_ref[l0:l1, :])
            gg = gg[:, 0:DP] + gg[:, DP:2 * DP]
            g1 = gg * lj[:, 0:1]
            for c5 in range(5):
                gp_ref[0, c5, i * 128:(i + 1) * 128, :] = gg[:, c5 * 128:(c5 + 1) * 128]
                gp_ref[1, c5, i * 128:(i + 1) * 128, :] = g1[:, c5 * 128:(c5 + 1) * 128]

    pl.run_scoped(s4_bwd, pltpu.VMEM((PB, 2 * CB, D), BF),
                  pltpu.VMEM((L, 2 * DP), BF), pltpu.VMEM((1, D), F32), pltpu.VMEM((CB, D), F32),
                  pltpu.VMEM((CB, D), F32), pltpu.VMEM((CB, D), F32))

    def ssm_bwd(ddt_ref, yt_ref):
        ddt_ref[...] = jnp.zeros(ddt_ref.shape, F32)

        def chunk(c, cc):
            ns = pl.ds(pl.multiple_of((c % 4) * 32, 32), 32)
            ds_ = pl.ds(pl.multiple_of((c // 4) * 128, 128), 128)
            pr = jnp.ones((32, 128), F32)
            z = jnp.zeros((32, 128), F32)
            st = (pr, z, z, z, z, z)
            for (j0, j1, p) in SEGS:
                mr = mul_ref[p, 0, ns, ds_]
                mi = mul_ref[p, 1, ns, ds_]
                yr, yi = jnp.ones((32, 128), F32), jnp.zeros((32, 128), F32)
                for o in range(16):
                    yt_ref[0, o] = yr
                    yt_ref[1, o] = yi
                    yr, yi = yr * mr - yi * mi, yr * mi + yi * mr

                def step(j, carry, yr=yr, yi=yi):
                    pr, pi_, s0r, s0i, s1r, s1i = carry
                    js = pl.ds(pl.multiple_of(j * 16, 16), 16)
                    g0t = gp_ref[0, c // 4, js, :]
                    g1t = gp_ref[1, c // 4, js, :]
                    t0r = t0i = t1r = t1i = None
                    for o in range(16):
                        g0 = g0t[o:o + 1, :]
                        g1 = g1t[o:o + 1, :]
                        a_, b_ = yt_ref[0, o], yt_ref[1, o]
                        if o == 0:
                            t0r, t0i, t1r, t1i = g0 * a_, g0 * b_, g1 * a_, g1 * b_
                        else:
                            t0r, t0i = t0r + g0 * a_, t0i + g0 * b_
                            t1r, t1i = t1r + g1 * a_, t1i + g1 * b_
                    return (pr * yr - pi_ * yi, pr * yi + pi_ * yr,
                            s0r + pr * t0r - pi_ * t0i, s0i + pr * t0i + pi_ * t0r,
                            s1r + pr * t1r - pi_ * t1i, s1i + pr * t1i + pi_ * t1r)
                st = lax.fori_loop(j0, j1, step, st)
            _, _, s0r, s0i, s1r, s1i = st
            dtc = jnp.exp(ldt_ref[:, ds_].astype(F32)).astype(BF).astype(F32)
            ar, ai = are_ref[ns, ds_].astype(F32), aim_ref[ns, ds_].astype(F32)
            b_r, b_i = bre_ref[ns, ds_].astype(F32), bim_ref[ns, ds_].astype(F32)
            cr, ci = cre_ref[ns, ds_].astype(F32), cim_ref[ns, ds_].astype(F32)
            br, bi = dtc * b_r, dtc * b_i
            dcre_ref[ns, ds_] = (s0r * br - s0i * bi).astype(BF)
            dcim_ref[ns, ds_] = (-(s0r * bi + s0i * br)).astype(BF)
            dbr = cr * s0r - ci * s0i
            dbi = -(cr * s0i + ci * s0r)
            dbre_ref[ns, ds_] = (dtc * dbr).astype(BF)
            dbim_ref[ns, ds_] = (dtc * dbi).astype(BF)
            wr = cr * br - ci * bi
            wi = cr * bi + ci * br
            dlr = wr * s1r - wi * s1i
            dli = -(wr * s1i + wi * s1r)
            dare_ref[ns, ds_] = (dtc * dlr).astype(BF)
            daim_ref[ns, ds_] = (dtc * dli).astype(BF)
            ddt_ref[:, ds_] += jnp.sum(dlr * ar + dli * ai + dbr * b_r + dbi * b_i, axis=0, keepdims=True)
            return cc
        _loop('chunkb', 0, 20, chunk)
        dldt_ref[...] = (ddt_ref[...] * dt).astype(BF)
    pl.run_scoped(ssm_bwd, pltpu.VMEM((1, DP), F32), pltpu.VMEM((2, 16, 32, 128), F32))
    for cp in cout:
        cp.wait()


@jax.jit
def pallas_sequential_preLN__ssm_conv_s4__mixer_gmlp__prompt_kernel(
    A_u: jax.Array,
    A_A_re: jax.Array,
    A_A_im: jax.Array,
    A_B_re: jax.Array,
    A_B_im: jax.Array,
    A_C_re: jax.Array,
    A_C_im: jax.Array,
    A_log_dt: jax.Array,
    A_Dskip: jax.Array,
    B_x: jax.Array,
    B_w_in: jax.Array,
    B_w_sp: jax.Array,
    B_b_sp: jax.Array,
    B_w_out: jax.Array,
    grad_out: jax.Array,
):
    tp = lambda a: jnp.pad(a.T, ((0, 0), (0, DP - D)))
    args = (A_u[0].T, grad_out[0].T, tp(A_A_re), tp(A_A_im), tp(A_B_re), tp(A_B_im), tp(A_C_re), tp(A_C_im),
            jnp.pad(A_log_dt[None, :], ((0, 0), (0, DP - D))), A_Dskip[None, :],
            B_w_in, B_w_sp, B_b_sp[:, None], B_w_out.T)
    sds = lambda *s: jax.ShapeDtypeStruct(s, BF)
    out_shape = (sds(D, L), sds(D, L), sds(N, DP), sds(N, DP), sds(N, DP), sds(N, DP), sds(N, DP), sds(N, DP),
                 sds(1, DP), sds(1, D), sds(D, FF), sds(L, L), sds(L, 1), sds(D, FH))
    vm = pl.BlockSpec(memory_space=pltpu.VMEM)
    an = pl.BlockSpec(memory_space=pl.ANY)
    res = pl.pallas_call(
        _kernel,
        in_specs=[an, an] + [vm] * 8 + [an, an, vm, an],
        out_specs=(an, an) + (vm,) * 8 + (an, an, vm, an),
        out_shape=out_shape,
        scratch_shapes=[pltpu.VMEM((PB, 2 * CB, D), BF), pltpu.VMEM((PB, 2 * CB, D), BF), pltpu.VMEM((L, D), F32),
                        pltpu.VMEM((4, 2, N, DP), F32), pltpu.VMEM((2, 5, NJ, 128), F32),
                        pltpu.VMEM((D, FF), BF),
                        pltpu.VMEM((L, L), BF), pltpu.VMEM((D, FH), BF),
                        pltpu.VMEM((D, L), BF), pltpu.VMEM((D, L), BF), pltpu.VMEM((D, FH), BF),
                        pltpu.VMEM((L, D), BF), pltpu.VMEM((L, D), BF), pltpu.VMEM((L, D), BF),
                        pltpu.VMEM((L, FF), BF), pltpu.VMEM((L, FH), BF), pltpu.VMEM((L, FH), BF),
                        pltpu.SemaphoreType.DMA((10,))],
        compiler_params=pltpu.CompilerParams(vmem_limit_bytes=120 * 1024 * 1024),
    )(*args)
    (out, dx, dare, daim, dbre, dbim, dcre, dcim, dldt, ddsk, dwin, dwsp, dbsp, dwout) = res
    ut = lambda a: a[:, :D].T
    return (out.T[None], dx.T[None], ut(dare), ut(daim), ut(dbre), ut(dbim), ut(dcre), ut(dcim),
            dldt[0, :D], ddsk[0], dwin, dwsp, dbsp[:, 0], dwout.T)
```

```python
import functools
import math

import jax
import jax.numpy as jnp
from jax import lax
import jax.experimental.pallas as pl
import jax.experimental.pallas.tpu as pltpu

F32 = jnp.float32
BF = jnp.bfloat16
L = 2048
D = 576
DP = 640
N = 128
FH = 2304
FF = 4608
NJ = 768
TM = 256
NT = L // TM
GC = math.sqrt(2.0 / math.pi)


def _dot(a, b):
    return jnp.dot(a, b, preferred_element_type=F32)


def _dot_nt(a, b):
    return lax.dot_general(a, b, (((1,), (1,)), ((), ())), preferred_element_type=F32)


def _dot_tn(a, b):
    return lax.dot_general(a, b, (((0,), (0,)), ((), ())), preferred_element_type=F32)


def _ln(x):
    m = jnp.mean(x, axis=-1, keepdims=True)
    c = x - m
    v = jnp.mean(c * c, axis=-1, keepdims=True)
    r = lax.rsqrt(v + 1e-5)
    return c * r, r


def _lnb(dy, y, r):
    return r * (dy - jnp.mean(dy, axis=-1, keepdims=True)
                - y * jnp.mean(dy * y, axis=-1, keepdims=True))


def _gelu(a):
    t = jnp.tanh(GC * (a + 0.044715 * a * a * a))
    return 0.5 * a * (1.0 + t)


def _dgelu(a):
    t = jnp.tanh(GC * (a + 0.044715 * a * a * a))
    return 0.5 * (1.0 + t) + 0.5 * a * (1.0 - t * t) * GC * (1.0 + 3 * 0.044715 * a * a)


def _loop(name, lo, hi, body):
    with jax.named_scope(name):
        lax.fori_loop(lo, hi, body, 0)


def _rows(i, t=TM):
    return pl.ds(pl.multiple_of(i * t, t), t)


CB = 256
PB = L // CB


def _dft_mats():
    k = lax.broadcasted_iota(jnp.int32, (CB, CB), 0)
    t = lax.broadcasted_iota(jnp.int32, (CB, CB), 1)
    ang = (((2 * k + 1) * t) & (4 * CB - 1)).astype(F32) * (math.pi / (2 * CB))
    ff = jnp.concatenate([jnp.cos(ang), -jnp.sin(ang)], 0).astype(BF)
    t = lax.broadcasted_iota(jnp.int32, (2 * CB, CB), 0)
    k = lax.broadcasted_iota(jnp.int32, (2 * CB, CB), 1)
    ang = (((2 * k + 1) * t) & (4 * CB - 1)).astype(F32) * (math.pi / (2 * CB))
    fi = jnp.concatenate([jnp.cos(ang), -jnp.sin(ang)], 1).astype(BF)
    return ff, fi


def _lval(j):
    return jnp.where(j <= 256, j,
                     jnp.where(j <= 384, 256 + 2 * (j - 256),
                               jnp.where(j <= 512, 512 + 4 * (j - 384),
                                         jnp.where(j <= 640, 1024 + 8 * (j - 512), -1)))).astype(F32)


SEGS = ((0, 16, 0), (16, 24, 1), (24, 32, 2), (32, 41, 3))


def _kernel(x_hbm, do_hbm, are_in, aim_in, bre_in, bim_in, cre_in, cim_in,
            ldt_ref, dsk_ref, win_hbm, wsp_hbm, bsp_ref, wout_hbm,
            out_hbm, dx_hbm, dare_o, daim_o, dbre_o, dbim_o, dcre_o, dcim_o,
            dldt_ref, ddsk_ref, dwin_hbm, dwsp_hbm, dbsp_ref, dwout_hbm,
            uf_ref, kf_ref, h_ref, mul_ref, gp_ref,
            win_ref, wsp_ref, wout_ref,
            out_ref, dx_ref, dwout_ref, x_ref, do_ref, u_ref, a_ref, z2_ref, g_ref, prm_ref, gsc_ref, sems):
    dwin_ref, dwsp_ref = win_ref, wsp_ref
    xt_ref, dot_ref = out_ref, dx_ref
    cin = [pltpu.make_async_copy(a, b, sems.at[i]) for i, (a, b) in enumerate(
        ((x_hbm, xt_ref), (win_hbm, win_ref), (wsp_hbm, wsp_ref), (wout_hbm, wout_ref), (do_hbm, dot_ref)))]
    cout = [pltpu.make_async_copy(a, b, sems.at[5 + i]) for i, (a, b) in enumerate(
        ((out_ref, out_hbm), (dwsp_ref, dwsp_hbm), (dwout_ref, dwout_hbm), (dwin_ref, dwin_hbm),
         (dx_ref, dx_hbm)))]
    for cp in cin:
        cp.start()
    for i, ref in enumerate((are_in, aim_in, bre_in, bim_in, cre_in, cim_in)):
        prm_ref[i, :, 0:D] = ref[...].astype(F32).T
        prm_ref[i, :, D:DP] = jnp.zeros((N, DP - D), F32)
    are_ref, aim_ref, bre_ref, bim_ref, cre_ref, cim_ref = [prm_ref.at[i] for i in range(6)]
    dare_ref, daim_ref, dbre_ref, dbim_ref, dcre_ref, dcim_ref = [gsc_ref.at[i] for i in range(6)]
    dsk = dsk_ref[...].astype(F32)
    dt = jnp.exp(ldt_ref[...].astype(F32)).astype(BF).astype(F32)
    lar = dt * are_ref[...].astype(F32)
    lai = dt * aim_ref[...].astype(F32)
    for p in range(4):
        e = jnp.exp(lar * (2.0 ** p))
        mul_ref[p, 0] = e * jnp.cos(lai * (2.0 ** p))
        mul_ref[p, 1] = e * jnp.sin(lai * (2.0 ** p))

    cin[0].wait()
    def ln_x(i, c):
        r = _rows(i)
        x = xt_ref[:, r].astype(F32).T
        x_ref[r, :] = x.astype(BF)
        u, _ = _ln(x)
        u_ref[r, :] = u.astype(BF)
        return c
    _loop('ln_x', 0, NT, ln_x)

    def s4_fwd(kp_ref, zr_ref, zi_ref, car_ref, yt_ref, kpb_ref):
        ff, fi = _dft_mats()
        kp_ref[...] = jnp.zeros(kp_ref.shape, F32)

        def chunk(c, cc):
            ns = pl.ds(pl.multiple_of((c % 2) * 64, 64), 64)
            ds_ = pl.ds(pl.multiple_of((c // 2) * 128, 128), 128)
            dtc = jnp.exp(ldt_ref[:, ds_].astype(F32)).astype(BF).astype(F32)
            br = dtc * bre_ref[ns, ds_].astype(F32)
            bi = dtc * bim_ref[ns, ds_].astype(F32)
            cr = cre_ref[ns, ds_].astype(F32)
            ci = cim_ref[ns, ds_].astype(F32)
            pr = cr * br - ci * bi
            pi_ = cr * bi + ci * br
            for (j0, j1, p) in SEGS:
                mr = mul_ref[p, 0, ns, ds_]
                mi = mul_ref[p, 1, ns, ds_]
                yr, yi = jnp.ones((64, 128), F32), jnp.zeros((64, 128), F32)
                for o in range(16):
                    yt_ref[0, o] = yr
                    yt_ref[1, o] = yi
                    yr, yi = yr * mr - yi * mi, yr * mi + yi * mr

                def step(j, carry, yr=yr, yi=yi):
                    pr, pi_ = carry
                    rows = []
                    for o in range(16):
                        rows.append(jnp.sum(pr * yt_ref[0, o] - pi_ * yt_ref[1, o], axis=0, keepdims=True))
                    js = pl.ds(pl.multiple_of(j * 16, 16), 16)
                    kp_ref[c // 2, js, :] = kp_ref[c // 2, js, :] + jnp.concatenate(rows, 0)
                    return pr * yr - pi_ * yi, pr * yi + pi_ * yr
                pr, pi_ = lax.fori_loop(j0, j1, step, (pr, pi_))
            return cc
        _loop('chunk', 0, 10, chunk)

        kpb = jnp.concatenate([kp_ref[c] for c in range(5)], 1)[:, :D].astype(BF)
        kpb_ref[...] = kpb

        def fwd_dft(i, c):
            j0 = jnp.where(i == 0, 0, jnp.where(i == 1, 256, jnp.where(i < 4, 384, 512)))
            j0 = pl.multiple_of(j0, 128)
            lj = _lval(lax.broadcasted_iota(jnp.int32, (CB, 256), 1) + j0)
            lr = (lax.broadcasted_iota(jnp.int32, (CB, 256), 0) + i * CB).astype(F32)
            m = (lr.astype(BF).astype(F32) == lj).astype(BF)
            kf_ref[i] = _dot(ff, _dot(m, kpb_ref[pl.ds(j0, 256), :]).astype(BF)).astype(BF)
            uf_ref[i] = _dot(ff, u_ref[_rows(i, CB), :]).astype(BF)
            return c
        _loop('fwd_dft', 0, PB, fwd_dft)
        car_ref[...] = jnp.zeros(car_ref.shape, F32)

        def inv(i, c):
            zr_ref[...] = jnp.zeros(zr_ref.shape, F32)
            zi_ref[...] = jnp.zeros(zi_ref.shape, F32)

            def mac(j, cc):
                ur, ui = uf_ref[i - j, 0:CB, :].astype(F32), uf_ref[i - j, CB:2 * CB, :].astype(F32)
                kr, ki = kf_ref[j, 0:CB, :].astype(F32), kf_ref[j, CB:2 * CB, :].astype(F32)
                zr_ref[...] += ur * kr - ui * ki
                zi_ref[...] += ur * ki + ui * kr
                return cc
            lax.fori_loop(0, i + 1, mac, 0)
            z = jnp.concatenate([zr_ref[...].astype(BF), zi_ref[...].astype(BF)], 0)
            yy = _dot(fi, z) * (1.0 / CB)
            r = _rows(i, CB)
            h_ref[r, :] = (x_ref[r, :].astype(F32) + yy[0:CB] + car_ref[...]
                           + u_ref[r, :].astype(F32) * dsk)
            car_ref[...] = yy[CB:2 * CB]
            return c
        _loop('inv', 0, PB, inv)

    pl.run_scoped(s4_fwd, pltpu.VMEM((5, NJ, 128), F32), pltpu.VMEM((CB, D), F32),
                  pltpu.VMEM((CB, D), F32), pltpu.VMEM((CB, D), F32), pltpu.VMEM((2, 16, 64, 128), F32),
                  pltpu.VMEM((NJ, D), BF))

    def gmlp(r2_ref, acc_ref):
        for cp in cin[1:]:
            cp.wait()
        def f1(i, c):
            r = _rows(i)
            hn, _ = _ln(h_ref[r, :])
            a = _dot(hn.astype(BF), win_ref[...]).astype(BF)
            a_ref[r, :] = a
            z2n, rr = _ln(_gelu(a[:, FH:].astype(F32)).astype(BF).astype(F32))
            z2_ref[r, :] = z2n.astype(BF)
            r2_ref[r, :] = rr
            return c
        _loop('f1', 0, NT, f1)
        acc_ref[...] = jnp.zeros(acc_ref.shape, F32)

        def f2(i, c):
            r = _rows(i, 128)
            g = (_dot(wsp_ref[r, :], z2_ref[...]) + bsp_ref[r, :].astype(F32)).astype(BF).astype(F32)
            a1 = a_ref[r, 0:FH].astype(F32)
            z1 = _gelu(a1).astype(BF).astype(F32)
            q = (z1 * g).astype(BF)
            out_ref[:, r] = (h_ref[r, :] + _dot_nt(q, wout_ref[...])).T.astype(BF)
            dot_ = dot_ref[:, r]
            do = dot_.astype(F32).T.astype(BF)
            do_ref[r, :] = do
            dq = _dot(do, wout_ref[...])
            acc_ref[...] += _dot(dot_, q)
            dg = (dq * z1).astype(BF)
            g_ref[r, :] = dg
            dbsp_ref[r, :] = jnp.sum(dg.astype(F32), axis=1, keepdims=True).astype(BF)
            a_ref[r, 0:FH] = (dq * g * _dgelu(a1)).astype(BF)
            return c
        _loop('f2', 0, L // 128, f2)
        dwout_ref[...] = acc_ref[...].astype(BF)
        cout[0].start()
        cout[2].start()

        def f3(i, c):
            r = _rows(i)
            dz2n = _dot(wsp_ref[:, r].astype(F32).T.astype(BF), g_ref[...])
            dz2 = _lnb(dz2n, z2_ref[r, :].astype(F32), r2_ref[r, :])
            a_ref[r, FH:FF] = (dz2 * _dgelu(a_ref[r, FH:FF].astype(F32))).astype(BF)
            return c
        _loop('f3', 0, NT, f3)

        def f6(i, c):
            r = _rows(i)
            hn, rh = _ln(h_ref[r, :])
            dhn = _dot_nt(a_ref[r, :], win_ref[...])
            h_ref[r, :] = do_ref[r, :].astype(F32) + _lnb(dhn, hn.astype(BF).astype(F32), rh)
            do_ref[r, :] = hn.astype(BF)
            return c
        _loop('f6', 0, NT, f6)

        def dwsp(i, c):
            r = _rows(i)
            dwsp_ref[r, :] = _dot_nt(g_ref[r, :], z2_ref[...]).astype(BF)
            return c
        _loop('dwsp', 0, NT, dwsp)
        cout[1].start()

        def dwin(i, c):
            cs = pl.ds(pl.multiple_of(i * 512, 512), 512)
            dwin_ref[:, cs] = _dot_tn(do_ref[...], a_ref[:, cs]).astype(BF)
            return c
        _loop('dwin', 0, FF // 512, dwin)
        cout[3].start()

    pl.run_scoped(gmlp, pltpu.VMEM((L, 1), F32), pltpu.VMEM((D, FH), F32))

    def s4_bwd(dyf_ref, dk_ref, dsum_ref, zr_ref, zi_ref, car_ref):
        ff, fi = _dft_mats()
        dsum_ref[...] = jnp.zeros(dsum_ref.shape, F32)

        def cast(i, c):
            r = _rows(i, CB)
            dh = h_ref[r, :]
            dyf_ref[i] = _dot(ff, dh.astype(BF)).astype(BF)
            dsum_ref[...] += jnp.sum(dh * u_ref[r, :].astype(F32), axis=0, keepdims=True)
            return c
        _loop('cast', 0, PB, cast)
        ddsk_ref[...] = dsum_ref[...].astype(BF)

        def corr(rr, ref):
            zr_ref[...] = jnp.zeros(zr_ref.shape, F32)
            zi_ref[...] = jnp.zeros(zi_ref.shape, F32)

            def mac(j, cc):
                yr, yi = dyf_ref[rr + j, 0:CB, :].astype(F32), dyf_ref[rr + j, CB:2 * CB, :].astype(F32)
                kr, ki = ref[j, 0:CB, :].astype(F32), ref[j, CB:2 * CB, :].astype(F32)
                zr_ref[...] += yr * kr + yi * ki
                zi_ref[...] += yi * kr - yr * ki
                return cc
            lax.fori_loop(0, PB - rr, mac, 0)
            z = jnp.concatenate([zr_ref[...].astype(BF), zi_ref[...].astype(BF)], 0)
            yy = _dot(fi, z) * (1.0 / CB)
            res = yy[0:CB] + car_ref[...]
            car_ref[...] = -yy[CB:2 * CB]
            return res

        def inv_dk(i, c):
            rr = PB - 1 - i
            r = _rows(rr, CB)
            dk = corr(rr, uf_ref)
            dkh = dk.astype(BF)
            dk_ref[r, 0:D] = dkh
            dk_ref[r, DP:DP + D] = (dk - dkh.astype(F32)).astype(BF)
            return c

        def inv_du(i, c):
            rr = PB - 1 - i
            r = _rows(rr, CB)
            dh = h_ref[r, :]
            du = corr(rr, kf_ref) + dh * dsk
            u, rx = _ln(x_ref[r, :].astype(F32))
            dx_ref[:, r] = (dh + _lnb(du, u.astype(BF).astype(F32), rx)).T.astype(BF)
            return c
        dk_ref[:, D:DP] = jnp.zeros((L, DP - D), BF)
        dk_ref[:, DP + D:2 * DP] = jnp.zeros((L, DP - D), BF)
        car_ref[...] = jnp.zeros(car_ref.shape, F32)
        _loop('inv_dk', 0, PB, inv_dk)
        car_ref[...] = jnp.zeros(car_ref.shape, F32)
        _loop('inv_du', 0, PB, inv_du)
        cout[4].start()

        for i, (l0, l1) in enumerate(((0, 128), (128, 256), (256, 512), (384, 1024), (896, 2048), (1920, 2048))):
            w = l1 - l0
            lj = _lval(lax.broadcasted_iota(jnp.int32, (128, w), 0) + i * 128)
            lr = (lax.broadcasted_iota(jnp.int32, (128, w), 1) + l0).astype(F32)
            mt = (lr.astype(BF).astype(F32) == lj).astype(BF)
            gg = _dot(mt, dk_ref[l0:l1, :])
            gg = gg[:, 0:DP] + gg[:, DP:2 * DP]
            g1 = gg * lj[:, 0:1]
            for c5 in range(5):
                gp_ref[0, c5, i * 128:(i + 1) * 128, :] = gg[:, c5 * 128:(c5 + 1) * 128]
                gp_ref[1, c5, i * 128:(i + 1) * 128, :] = g1[:, c5 * 128:(c5 + 1) * 128]

    pl.run_scoped(s4_bwd, pltpu.VMEM((PB, 2 * CB, D), BF),
                  pltpu.VMEM((L, 2 * DP), BF), pltpu.VMEM((1, D), F32), pltpu.VMEM((CB, D), F32),
                  pltpu.VMEM((CB, D), F32), pltpu.VMEM((CB, D), F32))

    def ssm_bwd(ddt_ref, yt_ref):
        ddt_ref[...] = jnp.zeros(ddt_ref.shape, F32)

        def chunk(c, cc):
            ns = pl.ds(pl.multiple_of((c % 4) * 32, 32), 32)
            ds_ = pl.ds(pl.multiple_of((c // 4) * 128, 128), 128)
            pr = jnp.ones((32, 128), F32)
            z = jnp.zeros((32, 128), F32)
            st = (pr, z, z, z, z, z)
            for (j0, j1, p) in SEGS:
                mr = mul_ref[p, 0, ns, ds_]
                mi = mul_ref[p, 1, ns, ds_]
                yr, yi = jnp.ones((32, 128), F32), jnp.zeros((32, 128), F32)
                for o in range(16):
                    yt_ref[0, o] = yr
                    yt_ref[1, o] = yi
                    yr, yi = yr * mr - yi * mi, yr * mi + yi * mr

                def step(j, carry, yr=yr, yi=yi):
                    pr, pi_, s0r, s0i, s1r, s1i = carry
                    js = pl.ds(pl.multiple_of(j * 16, 16), 16)
                    g0t = gp_ref[0, c // 4, js, :]
                    g1t = gp_ref[1, c // 4, js, :]
                    t0r = t0i = t1r = t1i = None
                    for o in range(16):
                        g0 = g0t[o:o + 1, :]
                        g1 = g1t[o:o + 1, :]
                        a_, b_ = yt_ref[0, o], yt_ref[1, o]
                        if o == 0:
                            t0r, t0i, t1r, t1i = g0 * a_, g0 * b_, g1 * a_, g1 * b_
                        else:
                            t0r, t0i = t0r + g0 * a_, t0i + g0 * b_
                            t1r, t1i = t1r + g1 * a_, t1i + g1 * b_
                    return (pr * yr - pi_ * yi, pr * yi + pi_ * yr,
                            s0r + pr * t0r - pi_ * t0i, s0i + pr * t0i + pi_ * t0r,
                            s1r + pr * t1r - pi_ * t1i, s1i + pr * t1i + pi_ * t1r)
                st = lax.fori_loop(j0, j1, step, st)
            _, _, s0r, s0i, s1r, s1i = st
            dtc = jnp.exp(ldt_ref[:, ds_].astype(F32)).astype(BF).astype(F32)
            ar, ai = are_ref[ns, ds_].astype(F32), aim_ref[ns, ds_].astype(F32)
            b_r, b_i = bre_ref[ns, ds_].astype(F32), bim_ref[ns, ds_].astype(F32)
            cr, ci = cre_ref[ns, ds_].astype(F32), cim_ref[ns, ds_].astype(F32)
            br, bi = dtc * b_r, dtc * b_i
            dcre_ref[ns, ds_] = (s0r * br - s0i * bi)
            dcim_ref[ns, ds_] = (-(s0r * bi + s0i * br))
            dbr = cr * s0r - ci * s0i
            dbi = -(cr * s0i + ci * s0r)
            dbre_ref[ns, ds_] = (dtc * dbr)
            dbim_ref[ns, ds_] = (dtc * dbi)
            wr = cr * br - ci * bi
            wi = cr * bi + ci * br
            dlr = wr * s1r - wi * s1i
            dli = -(wr * s1i + wi * s1r)
            dare_ref[ns, ds_] = (dtc * dlr)
            daim_ref[ns, ds_] = (dtc * dli)
            ddt_ref[:, ds_] += jnp.sum(dlr * ar + dli * ai + dbr * b_r + dbi * b_i, axis=0, keepdims=True)
            return cc
        _loop('chunkb', 0, 20, chunk)
        dldt_ref[...] = (ddt_ref[...] * dt).astype(BF)
        for i, ref in enumerate((dare_o, daim_o, dbre_o, dbim_o, dcre_o, dcim_o)):
            ref[...] = gsc_ref[i, :, 0:D].T.astype(BF)
    pl.run_scoped(ssm_bwd, pltpu.VMEM((1, DP), F32), pltpu.VMEM((2, 16, 32, 128), F32))
    for cp in cout:
        cp.wait()


@jax.jit
def pallas_sequential_preLN__ssm_conv_s4__mixer_gmlp__prompt_kernel(
    A_u: jax.Array,
    A_A_re: jax.Array,
    A_A_im: jax.Array,
    A_B_re: jax.Array,
    A_B_im: jax.Array,
    A_C_re: jax.Array,
    A_C_im: jax.Array,
    A_log_dt: jax.Array,
    A_Dskip: jax.Array,
    B_x: jax.Array,
    B_w_in: jax.Array,
    B_w_sp: jax.Array,
    B_b_sp: jax.Array,
    B_w_out: jax.Array,
    grad_out: jax.Array,
):
    args = (A_u[0].T, grad_out[0].T, A_A_re, A_A_im, A_B_re, A_B_im, A_C_re, A_C_im,
            jnp.pad(A_log_dt[None, :], ((0, 0), (0, DP - D))), A_Dskip[None, :],
            B_w_in, B_w_sp, B_b_sp[:, None], B_w_out.T)
    sds = lambda *s: jax.ShapeDtypeStruct(s, BF)
    out_shape = (sds(D, L), sds(D, L), sds(D, N), sds(D, N), sds(D, N), sds(D, N), sds(D, N), sds(D, N),
                 sds(1, DP), sds(1, D), sds(D, FF), sds(L, L), sds(L, 1), sds(D, FH))
    vm = pl.BlockSpec(memory_space=pltpu.VMEM)
    an = pl.BlockSpec(memory_space=pl.ANY)
    res = pl.pallas_call(
        _kernel,
        in_specs=[an, an] + [vm] * 8 + [an, an, vm, an],
        out_specs=(an, an) + (vm,) * 8 + (an, an, vm, an),
        out_shape=out_shape,
        scratch_shapes=[pltpu.VMEM((PB, 2 * CB, D), BF), pltpu.VMEM((PB, 2 * CB, D), BF), pltpu.VMEM((L, D), F32),
                        pltpu.VMEM((4, 2, N, DP), F32), pltpu.VMEM((2, 5, NJ, 128), F32),
                        pltpu.VMEM((D, FF), BF),
                        pltpu.VMEM((L, L), BF), pltpu.VMEM((D, FH), BF),
                        pltpu.VMEM((D, L), BF), pltpu.VMEM((D, L), BF), pltpu.VMEM((D, FH), BF),
                        pltpu.VMEM((L, D), BF), pltpu.VMEM((L, D), BF), pltpu.VMEM((L, D), BF),
                        pltpu.VMEM((L, FF), BF), pltpu.VMEM((L, FH), BF), pltpu.VMEM((L, FH), BF),
                        pltpu.VMEM((6, N, DP), F32), pltpu.VMEM((6, N, DP), F32),
                        pltpu.SemaphoreType.DMA((10,))],
        compiler_params=pltpu.CompilerParams(vmem_limit_bytes=120 * 1024 * 1024),
    )(*args)
    (out, dx, dare, daim, dbre, dbim, dcre, dcim, dldt, ddsk, dwin, dwsp, dbsp, dwout) = res
    return (out.T[None], dx.T[None], dare, daim, dbre, dbim, dcre, dcim,
            dldt[0, :D], ddsk[0], dwin, dwsp, dbsp[:, 0], dwout.T)
```

```python
import functools
import math

import jax
import jax.numpy as jnp
from jax import lax
import jax.experimental.pallas as pl
import jax.experimental.pallas.tpu as pltpu

F32 = jnp.float32
BF = jnp.bfloat16
L = 2048
D = 576
DP = 640
N = 128
FH = 2304
FF = 4608
NJ = 768
TM = 256
NT = L // TM
GC = math.sqrt(2.0 / math.pi)


def _dot(a, b):
    return jnp.dot(a, b, preferred_element_type=F32)


def _dot_nt(a, b):
    return lax.dot_general(a, b, (((1,), (1,)), ((), ())), preferred_element_type=F32)


def _dot_tn(a, b):
    return lax.dot_general(a, b, (((0,), (0,)), ((), ())), preferred_element_type=F32)


def _ln(x):
    m = jnp.mean(x, axis=-1, keepdims=True)
    c = x - m
    v = jnp.mean(c * c, axis=-1, keepdims=True)
    r = lax.rsqrt(v + 1e-5)
    return c * r, r


def _lnb(dy, y, r):
    return r * (dy - jnp.mean(dy, axis=-1, keepdims=True)
                - y * jnp.mean(dy * y, axis=-1, keepdims=True))


def _gelu(a):
    t = jnp.tanh(GC * (a + 0.044715 * a * a * a))
    return 0.5 * a * (1.0 + t)


def _dgelu(a):
    t = jnp.tanh(GC * (a + 0.044715 * a * a * a))
    return 0.5 * (1.0 + t) + 0.5 * a * (1.0 - t * t) * GC * (1.0 + 3 * 0.044715 * a * a)


def _loop(name, lo, hi, body):
    with jax.named_scope(name):
        lax.fori_loop(lo, hi, body, 0)


def _rows(i, t=TM):
    return pl.ds(pl.multiple_of(i * t, t), t)


CB = 256
PB = L // CB


def _dft_mats():
    k = lax.broadcasted_iota(jnp.int32, (CB, CB), 0)
    t = lax.broadcasted_iota(jnp.int32, (CB, CB), 1)
    ang = (((2 * k + 1) * t) & (4 * CB - 1)).astype(F32) * (math.pi / (2 * CB))
    ff = jnp.concatenate([jnp.cos(ang), -jnp.sin(ang)], 0).astype(BF)
    t = lax.broadcasted_iota(jnp.int32, (2 * CB, CB), 0)
    k = lax.broadcasted_iota(jnp.int32, (2 * CB, CB), 1)
    ang = (((2 * k + 1) * t) & (4 * CB - 1)).astype(F32) * (math.pi / (2 * CB))
    fi = jnp.concatenate([jnp.cos(ang), -jnp.sin(ang)], 1).astype(BF)
    return ff, fi


def _spec_mac(a_ref, ia, b_ref, n, conj, z_ref):
    SB = 32

    def sub(t, c):
        r1 = pl.ds(pl.multiple_of(t * SB, SB), SB)
        r2 = pl.ds(pl.multiple_of(CB + t * SB, SB), SB)

        def mac(j, carry):
            zr, zi = carry
            ar, ai = a_ref[ia(j), r1, :].astype(F32), a_ref[ia(j), r2, :].astype(F32)
            br, bi = b_ref[j, r1, :].astype(F32), b_ref[j, r2, :].astype(F32)
            if conj:
                return zr + ar * br + ai * bi, zi + ai * br - ar * bi
            return zr + ar * br - ai * bi, zi + ar * bi + ai * br
        z0 = jnp.zeros((SB, D), F32)
        zr, zi = lax.fori_loop(0, n, mac, (z0, z0))
        z_ref[r1, :] = zr.astype(BF)
        z_ref[r2, :] = zi.astype(BF)
        return c
    lax.fori_loop(0, CB // SB, sub, 0)


def _lval(j):
    return jnp.where(j <= 256, j,
                     jnp.where(j <= 384, 256 + 2 * (j - 256),
                               jnp.where(j <= 512, 512 + 4 * (j - 384),
                                         jnp.where(j <= 640, 1024 + 8 * (j - 512), -1)))).astype(F32)


SEGS = ((0, 16, 0), (16, 24, 1), (24, 32, 2), (32, 41, 3))


def _kernel(x_hbm, do_hbm, are_in, aim_in, bre_in, bim_in, cre_in, cim_in,
            ldt_ref, dsk_ref, win_hbm, wsp_hbm, bsp_ref, wout_hbm,
            out_hbm, dx_hbm, dare_o, daim_o, dbre_o, dbim_o, dcre_o, dcim_o,
            dldt_ref, ddsk_ref, dwin_hbm, dwsp_hbm, dbsp_ref, dwout_hbm,
            uf_ref, kf_ref, h_ref, mul_ref, gp_ref,
            win_ref, wsp_ref, wout_ref,
            out_ref, dx_ref, dwout_ref, x_ref, do_ref, u_ref, a_ref, z2_ref, g_ref, prm_ref, gsc_ref, sems):
    dwin_ref, dwsp_ref = win_ref, wsp_ref
    xt_ref, dot_ref = out_ref, dx_ref
    cin = [pltpu.make_async_copy(a, b, sems.at[i]) for i, (a, b) in enumerate(
        ((x_hbm, xt_ref), (win_hbm, win_ref), (wsp_hbm, wsp_ref), (wout_hbm, wout_ref), (do_hbm, dot_ref)))]
    cout = [pltpu.make_async_copy(a, b, sems.at[5 + i]) for i, (a, b) in enumerate(
        ((out_ref, out_hbm), (dwsp_ref, dwsp_hbm), (dwout_ref, dwout_hbm), (dwin_ref, dwin_hbm),
         (dx_ref, dx_hbm)))]
    for cp in cin:
        cp.start()
    for i, ref in enumerate((are_in, aim_in, bre_in, bim_in, cre_in, cim_in)):
        prm_ref[i, :, 0:D] = ref[...].astype(F32).T
        prm_ref[i, :, D:DP] = jnp.zeros((N, DP - D), F32)
    are_ref, aim_ref, bre_ref, bim_ref, cre_ref, cim_ref = [prm_ref.at[i] for i in range(6)]
    dare_ref, daim_ref, dbre_ref, dbim_ref, dcre_ref, dcim_ref = [gsc_ref.at[i] for i in range(6)]
    dsk = dsk_ref[...].astype(F32)
    dt = jnp.exp(ldt_ref[...].astype(F32)).astype(BF).astype(F32)
    lar = dt * are_ref[...].astype(F32)
    lai = dt * aim_ref[...].astype(F32)
    for p in range(4):
        e = jnp.exp(lar * (2.0 ** p))
        mul_ref[p, 0] = e * jnp.cos(lai * (2.0 ** p))
        mul_ref[p, 1] = e * jnp.sin(lai * (2.0 ** p))

    cin[0].wait()
    def ln_x(i, c):
        r = _rows(i)
        x = xt_ref[:, r].astype(F32).T
        x_ref[r, :] = x.astype(BF)
        u, _ = _ln(x)
        u_ref[r, :] = u.astype(BF)
        return c
    _loop('ln_x', 0, NT, ln_x)

    def s4_fwd(kp_ref, zr_ref, zi_ref, car_ref, yt_ref, kpb_ref):
        ff, fi = _dft_mats()
        kp_ref[...] = jnp.zeros(kp_ref.shape, F32)

        def chunk(c, cc):
            ns = pl.ds(pl.multiple_of((c % 2) * 64, 64), 64)
            ds_ = pl.ds(pl.multiple_of((c // 2) * 128, 128), 128)
            dtc = jnp.exp(ldt_ref[:, ds_].astype(F32)).astype(BF).astype(F32)
            br = dtc * bre_ref[ns, ds_].astype(F32)
            bi = dtc * bim_ref[ns, ds_].astype(F32)
            cr = cre_ref[ns, ds_].astype(F32)
            ci = cim_ref[ns, ds_].astype(F32)
            pr = cr * br - ci * bi
            pi_ = cr * bi + ci * br
            for (j0, j1, p) in SEGS:
                mr = mul_ref[p, 0, ns, ds_]
                mi = mul_ref[p, 1, ns, ds_]
                yr, yi = jnp.ones((64, 128), F32), jnp.zeros((64, 128), F32)
                for o in range(16):
                    yt_ref[0, o] = yr
                    yt_ref[1, o] = yi
                    yr, yi = yr * mr - yi * mi, yr * mi + yi * mr

                def step(j, carry, yr=yr, yi=yi):
                    pr, pi_ = carry
                    rows = []
                    for o in range(16):
                        rows.append(jnp.sum(pr * yt_ref[0, o] - pi_ * yt_ref[1, o], axis=0, keepdims=True))
                    js = pl.ds(pl.multiple_of(j * 16, 16), 16)
                    kp_ref[c // 2, js, :] = kp_ref[c // 2, js, :] + jnp.concatenate(rows, 0)
                    return pr * yr - pi_ * yi, pr * yi + pi_ * yr
                pr, pi_ = lax.fori_loop(j0, j1, step, (pr, pi_))
            return cc
        _loop('chunk', 0, 10, chunk)

        kpb = jnp.concatenate([kp_ref[c] for c in range(5)], 1)[:, :D].astype(BF)
        kpb_ref[...] = kpb

        def fwd_dft(i, c):
            j0 = jnp.where(i == 0, 0, jnp.where(i == 1, 256, jnp.where(i < 4, 384, 512)))
            j0 = pl.multiple_of(j0, 128)
            lj = _lval(lax.broadcasted_iota(jnp.int32, (CB, 256), 1) + j0)
            lr = (lax.broadcasted_iota(jnp.int32, (CB, 256), 0) + i * CB).astype(F32)
            m = (lr.astype(BF).astype(F32) == lj).astype(BF)
            kf_ref[i] = _dot(ff, _dot(m, kpb_ref[pl.ds(j0, 256), :]).astype(BF)).astype(BF)
            uf_ref[i] = _dot(ff, u_ref[_rows(i, CB), :]).astype(BF)
            return c
        _loop('fwd_dft', 0, PB, fwd_dft)
        car_ref[...] = jnp.zeros(car_ref.shape, F32)

        def inv(i, c):
            _spec_mac(uf_ref, lambda j: i - j, kf_ref, i + 1, False, zr_ref)
            z = zr_ref[...]
            yy = _dot(fi, z) * (1.0 / CB)
            r = _rows(i, CB)
            h_ref[r, :] = (x_ref[r, :].astype(F32) + yy[0:CB] + car_ref[...]
                           + u_ref[r, :].astype(F32) * dsk)
            car_ref[...] = yy[CB:2 * CB]
            return c
        _loop('inv', 0, PB, inv)

    pl.run_scoped(s4_fwd, pltpu.VMEM((5, NJ, 128), F32), pltpu.VMEM((2 * CB, D), BF),
                  pltpu.VMEM((CB, D), F32), pltpu.VMEM((CB, D), F32), pltpu.VMEM((2, 16, 64, 128), F32),
                  pltpu.VMEM((NJ, D), BF))

    def gmlp(r2_ref, acc_ref):
        for cp in cin[1:]:
            cp.wait()
        def f1(i, c):
            r = _rows(i)
            hn, _ = _ln(h_ref[r, :])
            a = _dot(hn.astype(BF), win_ref[...]).astype(BF)
            a_ref[r, :] = a
            z2n, rr = _ln(_gelu(a[:, FH:].astype(F32)).astype(BF).astype(F32))
            z2_ref[r, :] = z2n.astype(BF)
            r2_ref[r, :] = rr
            return c
        _loop('f1', 0, NT, f1)
        acc_ref[...] = jnp.zeros(acc_ref.shape, F32)

        def f2(i, c):
            r = _rows(i, 128)
            g = (_dot(wsp_ref[r, :], z2_ref[...]) + bsp_ref[r, :].astype(F32)).astype(BF).astype(F32)
            a1 = a_ref[r, 0:FH].astype(F32)
            z1 = _gelu(a1).astype(BF).astype(F32)
            q = (z1 * g).astype(BF)
            out_ref[:, r] = (h_ref[r, :] + _dot_nt(q, wout_ref[...])).T.astype(BF)
            dot_ = dot_ref[:, r]
            do = dot_.astype(F32).T.astype(BF)
            do_ref[r, :] = do
            dq = _dot(do, wout_ref[...])
            acc_ref[...] += _dot(dot_, q)
            dg = (dq * z1).astype(BF)
            g_ref[r, :] = dg
            dbsp_ref[r, :] = jnp.sum(dg.astype(F32), axis=1, keepdims=True).astype(BF)
            a_ref[r, 0:FH] = (dq * g * _dgelu(a1)).astype(BF)
            return c
        _loop('f2', 0, L // 128, f2)
        dwout_ref[...] = acc_ref[...].astype(BF)
        cout[0].start()
        cout[2].start()

        def f3(i, c):
            r = _rows(i)
            dz2n = _dot(wsp_ref[:, r].astype(F32).T.astype(BF), g_ref[...])
            dz2 = _lnb(dz2n, z2_ref[r, :].astype(F32), r2_ref[r, :])
            a_ref[r, FH:FF] = (dz2 * _dgelu(a_ref[r, FH:FF].astype(F32))).astype(BF)
            return c
        _loop('f3', 0, NT, f3)

        def f6(i, c):
            r = _rows(i)
            hn, rh = _ln(h_ref[r, :])
            dhn = _dot_nt(a_ref[r, :], win_ref[...])
            h_ref[r, :] = do_ref[r, :].astype(F32) + _lnb(dhn, hn.astype(BF).astype(F32), rh)
            do_ref[r, :] = hn.astype(BF)
            return c
        _loop('f6', 0, NT, f6)

        def dwsp(i, c):
            r = _rows(i)
            dwsp_ref[r, :] = _dot_nt(g_ref[r, :], z2_ref[...]).astype(BF)
            return c
        _loop('dwsp', 0, NT, dwsp)
        cout[1].start()

        def dwin(i, c):
            cs = pl.ds(pl.multiple_of(i * 512, 512), 512)
            dwin_ref[:, cs] = _dot_tn(do_ref[...], a_ref[:, cs]).astype(BF)
            return c
        _loop('dwin', 0, FF // 512, dwin)
        cout[3].start()

    pl.run_scoped(gmlp, pltpu.VMEM((L, 1), F32), pltpu.VMEM((D, FH), F32))

    def s4_bwd(dyf_ref, dk_ref, dsum_ref, zr_ref, zi_ref, car_ref):
        ff, fi = _dft_mats()
        dsum_ref[...] = jnp.zeros(dsum_ref.shape, F32)

        def cast(i, c):
            r = _rows(i, CB)
            dh = h_ref[r, :]
            dyf_ref[i] = _dot(ff, dh.astype(BF)).astype(BF)
            dsum_ref[...] += jnp.sum(dh * u_ref[r, :].astype(F32), axis=0, keepdims=True)
            return c
        _loop('cast', 0, PB, cast)
        ddsk_ref[...] = dsum_ref[...].astype(BF)

        def corr(rr, ref):
            _spec_mac(dyf_ref, lambda j: rr + j, ref, PB - rr, True, zr_ref)
            z = zr_ref[...]
            yy = _dot(fi, z) * (1.0 / CB)
            res = yy[0:CB] + car_ref[...]
            car_ref[...] = -yy[CB:2 * CB]
            return res

        def inv_dk(i, c):
            rr = PB - 1 - i
            r = _rows(rr, CB)
            dk = corr(rr, uf_ref)
            dkh = dk.astype(BF)
            dk_ref[r, 0:D] = dkh
            dk_ref[r, DP:DP + D] = (dk - dkh.astype(F32)).astype(BF)
            return c

        def inv_du(i, c):
            rr = PB - 1 - i
            r = _rows(rr, CB)
            dh = h_ref[r, :]
            du = corr(rr, kf_ref) + dh * dsk
            u, rx = _ln(x_ref[r, :].astype(F32))
            dx_ref[:, r] = (dh + _lnb(du, u.astype(BF).astype(F32), rx)).T.astype(BF)
            return c
        dk_ref[:, D:DP] = jnp.zeros((L, DP - D), BF)
        dk_ref[:, DP + D:2 * DP] = jnp.zeros((L, DP - D), BF)
        car_ref[...] = jnp.zeros(car_ref.shape, F32)
        _loop('inv_dk', 0, PB, inv_dk)
        car_ref[...] = jnp.zeros(car_ref.shape, F32)
        _loop('inv_du', 0, PB, inv_du)
        cout[4].start()

        for i, (l0, l1) in enumerate(((0, 128), (128, 256), (256, 512), (384, 1024), (896, 2048), (1920, 2048))):
            w = l1 - l0
            lj = _lval(lax.broadcasted_iota(jnp.int32, (128, w), 0) + i * 128)
            lr = (lax.broadcasted_iota(jnp.int32, (128, w), 1) + l0).astype(F32)
            mt = (lr.astype(BF).astype(F32) == lj).astype(BF)
            gg = _dot(mt, dk_ref[l0:l1, :])
            gg = gg[:, 0:DP] + gg[:, DP:2 * DP]
            g1 = gg * lj[:, 0:1]
            for c5 in range(5):
                gp_ref[0, c5, i * 128:(i + 1) * 128, :] = gg[:, c5 * 128:(c5 + 1) * 128]
                gp_ref[1, c5, i * 128:(i + 1) * 128, :] = g1[:, c5 * 128:(c5 + 1) * 128]

    pl.run_scoped(s4_bwd, pltpu.VMEM((PB, 2 * CB, D), BF),
                  pltpu.VMEM((L, 2 * DP), BF), pltpu.VMEM((1, D), F32), pltpu.VMEM((2 * CB, D), BF),
                  pltpu.VMEM((CB, D), F32), pltpu.VMEM((CB, D), F32))

    def ssm_bwd(ddt_ref, yt_ref):
        ddt_ref[...] = jnp.zeros(ddt_ref.shape, F32)

        def chunk(c, cc):
            ns = pl.ds(pl.multiple_of((c % 4) * 32, 32), 32)
            ds_ = pl.ds(pl.multiple_of((c // 4) * 128, 128), 128)
            pr = jnp.ones((32, 128), F32)
            z = jnp.zeros((32, 128), F32)
            st = (pr, z, z, z, z, z)
            for (j0, j1, p) in SEGS:
                mr = mul_ref[p, 0, ns, ds_]
                mi = mul_ref[p, 1, ns, ds_]
                yr, yi = jnp.ones((32, 128), F32), jnp.zeros((32, 128), F32)
                for o in range(16):
                    yt_ref[0, o] = yr
                    yt_ref[1, o] = yi
                    yr, yi = yr * mr - yi * mi, yr * mi + yi * mr

                def step(j, carry, yr=yr, yi=yi):
                    pr, pi_, s0r, s0i, s1r, s1i = carry
                    js = pl.ds(pl.multiple_of(j * 16, 16), 16)
                    g0t = gp_ref[0, c // 4, js, :]
                    g1t = gp_ref[1, c // 4, js, :]
                    t0r = t0i = t1r = t1i = None
                    for o in range(16):
                        g0 = g0t[o:o + 1, :]
                        g1 = g1t[o:o + 1, :]
                        a_, b_ = yt_ref[0, o], yt_ref[1, o]
                        if o == 0:
                            t0r, t0i, t1r, t1i = g0 * a_, g0 * b_, g1 * a_, g1 * b_
                        else:
                            t0r, t0i = t0r + g0 * a_, t0i + g0 * b_
                            t1r, t1i = t1r + g1 * a_, t1i + g1 * b_
                    return (pr * yr - pi_ * yi, pr * yi + pi_ * yr,
                            s0r + pr * t0r - pi_ * t0i, s0i + pr * t0i + pi_ * t0r,
                            s1r + pr * t1r - pi_ * t1i, s1i + pr * t1i + pi_ * t1r)
                st = lax.fori_loop(j0, j1, step, st)
            _, _, s0r, s0i, s1r, s1i = st
            dtc = jnp.exp(ldt_ref[:, ds_].astype(F32)).astype(BF).astype(F32)
            ar, ai = are_ref[ns, ds_].astype(F32), aim_ref[ns, ds_].astype(F32)
            b_r, b_i = bre_ref[ns, ds_].astype(F32), bim_ref[ns, ds_].astype(F32)
            cr, ci = cre_ref[ns, ds_].astype(F32), cim_ref[ns, ds_].astype(F32)
            br, bi = dtc * b_r, dtc * b_i
            dcre_ref[ns, ds_] = (s0r * br - s0i * bi)
            dcim_ref[ns, ds_] = (-(s0r * bi + s0i * br))
            dbr = cr * s0r - ci * s0i
            dbi = -(cr * s0i + ci * s0r)
            dbre_ref[ns, ds_] = (dtc * dbr)
            dbim_ref[ns, ds_] = (dtc * dbi)
            wr = cr * br - ci * bi
            wi = cr * bi + ci * br
            dlr = wr * s1r - wi * s1i
            dli = -(wr * s1i + wi * s1r)
            dare_ref[ns, ds_] = (dtc * dlr)
            daim_ref[ns, ds_] = (dtc * dli)
            ddt_ref[:, ds_] += jnp.sum(dlr * ar + dli * ai + dbr * b_r + dbi * b_i, axis=0, keepdims=True)
            return cc
        _loop('chunkb', 0, 20, chunk)
        dldt_ref[...] = (ddt_ref[...] * dt).astype(BF)
        for i, ref in enumerate((dare_o, daim_o, dbre_o, dbim_o, dcre_o, dcim_o)):
            ref[...] = gsc_ref[i, :, 0:D].T.astype(BF)
    pl.run_scoped(ssm_bwd, pltpu.VMEM((1, DP), F32), pltpu.VMEM((2, 16, 32, 128), F32))
    for cp in cout:
        cp.wait()


@jax.jit
def pallas_sequential_preLN__ssm_conv_s4__mixer_gmlp__prompt_kernel(
    A_u: jax.Array,
    A_A_re: jax.Array,
    A_A_im: jax.Array,
    A_B_re: jax.Array,
    A_B_im: jax.Array,
    A_C_re: jax.Array,
    A_C_im: jax.Array,
    A_log_dt: jax.Array,
    A_Dskip: jax.Array,
    B_x: jax.Array,
    B_w_in: jax.Array,
    B_w_sp: jax.Array,
    B_b_sp: jax.Array,
    B_w_out: jax.Array,
    grad_out: jax.Array,
):
    args = (A_u[0].T, grad_out[0].T, A_A_re, A_A_im, A_B_re, A_B_im, A_C_re, A_C_im,
            jnp.pad(A_log_dt[None, :], ((0, 0), (0, DP - D))), A_Dskip[None, :],
            B_w_in, B_w_sp, B_b_sp[:, None], B_w_out.T)
    sds = lambda *s: jax.ShapeDtypeStruct(s, BF)
    out_shape = (sds(D, L), sds(D, L), sds(D, N), sds(D, N), sds(D, N), sds(D, N), sds(D, N), sds(D, N),
                 sds(1, DP), sds(1, D), sds(D, FF), sds(L, L), sds(L, 1), sds(D, FH))
    vm = pl.BlockSpec(memory_space=pltpu.VMEM)
    an = pl.BlockSpec(memory_space=pl.ANY)
    res = pl.pallas_call(
        _kernel,
        in_specs=[an, an] + [vm] * 8 + [an, an, vm, an],
        out_specs=(an, an) + (vm,) * 8 + (an, an, vm, an),
        out_shape=out_shape,
        scratch_shapes=[pltpu.VMEM((PB, 2 * CB, D), BF), pltpu.VMEM((PB, 2 * CB, D), BF), pltpu.VMEM((L, D), F32),
                        pltpu.VMEM((4, 2, N, DP), F32), pltpu.VMEM((2, 5, NJ, 128), F32),
                        pltpu.VMEM((D, FF), BF),
                        pltpu.VMEM((L, L), BF), pltpu.VMEM((D, FH), BF),
                        pltpu.VMEM((D, L), BF), pltpu.VMEM((D, L), BF), pltpu.VMEM((D, FH), BF),
                        pltpu.VMEM((L, D), BF), pltpu.VMEM((L, D), BF), pltpu.VMEM((L, D), BF),
                        pltpu.VMEM((L, FF), BF), pltpu.VMEM((L, FH), BF), pltpu.VMEM((L, FH), BF),
                        pltpu.VMEM((6, N, DP), F32), pltpu.VMEM((6, N, DP), F32),
                        pltpu.SemaphoreType.DMA((10,))],
        compiler_params=pltpu.CompilerParams(vmem_limit_bytes=120 * 1024 * 1024),
    )(*args)
    (out, dx, dare, daim, dbre, dbim, dcre, dcim, dldt, ddsk, dwin, dwsp, dbsp, dwout) = res
    return (out.T[None], dx.T[None], dare, daim, dbre, dbim, dcre, dcim,
            dldt[0, :D], ddsk[0], dwin, dwsp, dbsp[:, 0], dwout.T)
```

```python
import math

import jax
import jax.numpy as jnp
from jax import lax
import jax.experimental.pallas as pl
import jax.experimental.pallas.tpu as pltpu

F32 = jnp.float32
BF = jnp.bfloat16
L = 2048
D = 576
DP = 640
N = 128
FH = 2304
FF = 4608
NJ = 768
TM = 256
NT = L // TM
GC = math.sqrt(2.0 / math.pi)


def _dot(a, b):
    return jnp.dot(a, b, preferred_element_type=F32)


def _dot_nt(a, b):
    return lax.dot_general(a, b, (((1,), (1,)), ((), ())), preferred_element_type=F32)


def _dot_tn(a, b):
    return lax.dot_general(a, b, (((0,), (0,)), ((), ())), preferred_element_type=F32)


def _ln(x):
    m = jnp.mean(x, axis=-1, keepdims=True)
    c = x - m
    v = jnp.mean(c * c, axis=-1, keepdims=True)
    r = lax.rsqrt(v + 1e-5)
    return c * r, r


def _lnb(dy, y, r):
    return r * (dy - jnp.mean(dy, axis=-1, keepdims=True)
                - y * jnp.mean(dy * y, axis=-1, keepdims=True))


def _gelu(a):
    t = jnp.tanh(GC * (a + 0.044715 * a * a * a))
    return 0.5 * a * (1.0 + t)


def _dgelu(a):
    t = jnp.tanh(GC * (a + 0.044715 * a * a * a))
    return 0.5 * (1.0 + t) + 0.5 * a * (1.0 - t * t) * GC * (1.0 + 3 * 0.044715 * a * a)


def _loop(name, lo, hi, body):
    with jax.named_scope(name):
        lax.fori_loop(lo, hi, body, 0)


def _rows(i, t=TM):
    return pl.ds(pl.multiple_of(i * t, t), t)


CB = 256
PB = L // CB


def _dft_mats():
    k = lax.broadcasted_iota(jnp.int32, (CB, CB), 0)
    t = lax.broadcasted_iota(jnp.int32, (CB, CB), 1)
    ang = (((2 * k + 1) * t) & (4 * CB - 1)).astype(F32) * (math.pi / (2 * CB))
    ff = jnp.concatenate([jnp.cos(ang), -jnp.sin(ang)], 0).astype(BF)
    t = lax.broadcasted_iota(jnp.int32, (2 * CB, CB), 0)
    k = lax.broadcasted_iota(jnp.int32, (2 * CB, CB), 1)
    ang = (((2 * k + 1) * t) & (4 * CB - 1)).astype(F32) * (math.pi / (2 * CB))
    fi = jnp.concatenate([jnp.cos(ang), -jnp.sin(ang)], 1).astype(BF)
    return ff, fi


def _lval(j):
    return jnp.where(j <= 256, j,
                     jnp.where(j <= 384, 256 + 2 * (j - 256),
                               jnp.where(j <= 512, 512 + 4 * (j - 384),
                                         jnp.where(j <= 640, 1024 + 8 * (j - 512), -1)))).astype(F32)


SEGS = ((0, 16, 0), (16, 24, 1), (24, 32, 2), (32, 41, 3))


def _kernel(x_hbm, do_hbm, are_in, aim_in, bre_in, bim_in, cre_in, cim_in,
            ldt_ref, dsk_ref, win_hbm, wsp_hbm, bsp_ref, wout_hbm,
            out_hbm, dx_hbm, dare_o, daim_o, dbre_o, dbim_o, dcre_o, dcim_o,
            dldt_ref, ddsk_ref, dwin_hbm, dwsp_hbm, dbsp_ref, dwout_hbm,
            uf_ref, kf_ref, h_ref, mul_ref, gp_ref,
            win_ref, wsp_ref, wout_ref,
            out_ref, dx_ref, dwout_ref, x_ref, do_ref, u_ref, a_ref, z2_ref, g_ref, prm_ref, gsc_ref, sems):
    dwin_ref, dwsp_ref = win_ref, wsp_ref
    xt_ref, dot_ref = out_ref, dx_ref
    cin = [pltpu.make_async_copy(a, b, sems.at[i]) for i, (a, b) in enumerate(
        ((x_hbm, xt_ref), (win_hbm, win_ref), (wsp_hbm, wsp_ref), (wout_hbm, wout_ref), (do_hbm, dot_ref)))]
    cout = [pltpu.make_async_copy(a, b, sems.at[5 + i]) for i, (a, b) in enumerate(
        ((out_ref, out_hbm), (dwsp_ref, dwsp_hbm), (dwout_ref, dwout_hbm), (dwin_ref, dwin_hbm),
         (dx_ref, dx_hbm)))]
    for cp in cin:
        cp.start()
    for i, ref in enumerate((are_in, aim_in, bre_in, bim_in, cre_in, cim_in)):
        prm_ref[i, :, 0:D] = ref[...].astype(F32).T
        prm_ref[i, :, D:DP] = jnp.zeros((N, DP - D), F32)
    are_ref, aim_ref, bre_ref, bim_ref, cre_ref, cim_ref = [prm_ref.at[i] for i in range(6)]
    dare_ref, daim_ref, dbre_ref, dbim_ref, dcre_ref, dcim_ref = [gsc_ref.at[i] for i in range(6)]
    dsk = dsk_ref[...].astype(F32)
    dt = jnp.exp(ldt_ref[...].astype(F32)).astype(BF).astype(F32)
    lar = dt * are_ref[...].astype(F32)
    lai = dt * aim_ref[...].astype(F32)
    for p in range(4):
        e = jnp.exp(lar * (2.0 ** p))
        mul_ref[p, 0] = e * jnp.cos(lai * (2.0 ** p))
        mul_ref[p, 1] = e * jnp.sin(lai * (2.0 ** p))

    cin[0].wait()
    def ln_x(i, c):
        r = _rows(i)
        x = xt_ref[:, r].astype(F32).T
        x_ref[r, :] = x.astype(BF)
        u, _ = _ln(x)
        u_ref[r, :] = u.astype(BF)
        return c
    _loop('ln_x', 0, NT, ln_x)

    def s4_fwd(kp_ref, zr_ref, zi_ref, car_ref, yt_ref, kpb_ref):
        ff, fi = _dft_mats()
        kp_ref[...] = jnp.zeros(kp_ref.shape, F32)

        def chunk(c, cc):
            ns = pl.ds(pl.multiple_of((c % 2) * 64, 64), 64)
            ds_ = pl.ds(pl.multiple_of((c // 2) * 128, 128), 128)
            dtc = jnp.exp(ldt_ref[:, ds_].astype(F32)).astype(BF).astype(F32)
            br = dtc * bre_ref[ns, ds_].astype(F32)
            bi = dtc * bim_ref[ns, ds_].astype(F32)
            cr = cre_ref[ns, ds_].astype(F32)
            ci = cim_ref[ns, ds_].astype(F32)
            pr = cr * br - ci * bi
            pi_ = cr * bi + ci * br
            for (j0, j1, p) in SEGS:
                mr = mul_ref[p, 0, ns, ds_]
                mi = mul_ref[p, 1, ns, ds_]
                yr, yi = jnp.ones((64, 128), F32), jnp.zeros((64, 128), F32)
                for o in range(16):
                    yt_ref[0, o] = yr
                    yt_ref[1, o] = yi
                    yr, yi = yr * mr - yi * mi, yr * mi + yi * mr

                def step(j, carry, yr=yr, yi=yi):
                    pr, pi_ = carry
                    rows = []
                    for o in range(16):
                        rows.append(jnp.sum(pr * yt_ref[0, o] - pi_ * yt_ref[1, o], axis=0, keepdims=True))
                    js = pl.ds(pl.multiple_of(j * 16, 16), 16)
                    kp_ref[c // 2, js, :] = kp_ref[c // 2, js, :] + jnp.concatenate(rows, 0)
                    return pr * yr - pi_ * yi, pr * yi + pi_ * yr
                pr, pi_ = lax.fori_loop(j0, j1, step, (pr, pi_))
            return cc
        _loop('chunk', 0, 10, chunk)

        kpb = jnp.concatenate([kp_ref[c] for c in range(5)], 1)[:, :D].astype(BF)
        kpb_ref[...] = jnp.where(lax.broadcasted_iota(jnp.int32, (NJ, D), 0) <= 640, kpb, jnp.zeros_like(kpb))

        def fwd_dft(i, c):
            j0 = jnp.where(i == 0, 0, jnp.where(i == 1, 256, jnp.where(i < 4, 384, 512)))
            j0 = pl.multiple_of(j0, 128)
            lj = _lval(lax.broadcasted_iota(jnp.int32, (CB, 256), 1) + j0)
            lr = (lax.broadcasted_iota(jnp.int32, (CB, 256), 0) + i * CB).astype(F32)
            m = (lr.astype(BF).astype(F32) == lj).astype(BF)
            kf_ref[i] = _dot(ff, _dot(m, kpb_ref[pl.ds(j0, 256), :]).astype(BF)).astype(BF)
            uf_ref[i] = _dot(ff, u_ref[_rows(i, CB), :]).astype(BF)
            return c
        _loop('fwd_dft', 0, PB, fwd_dft)
        car_ref[...] = jnp.zeros(car_ref.shape, F32)

        def inv(i, c):
            zr_ref[...] = jnp.zeros(zr_ref.shape, F32)
            zi_ref[...] = jnp.zeros(zi_ref.shape, F32)

            def mac(j, cc):
                ur, ui = uf_ref[i - j, 0:CB, :].astype(F32), uf_ref[i - j, CB:2 * CB, :].astype(F32)
                kr, ki = kf_ref[j, 0:CB, :].astype(F32), kf_ref[j, CB:2 * CB, :].astype(F32)
                zr_ref[...] += ur * kr - ui * ki
                zi_ref[...] += ur * ki + ui * kr
                return cc
            lax.fori_loop(0, i + 1, mac, 0)
            z = jnp.concatenate([zr_ref[...].astype(BF), zi_ref[...].astype(BF)], 0)
            yy = _dot(fi, z) * (1.0 / CB)
            r = _rows(i, CB)
            h_ref[r, :] = (x_ref[r, :].astype(F32) + yy[0:CB] + car_ref[...]
                           + u_ref[r, :].astype(F32) * dsk)
            car_ref[...] = yy[CB:2 * CB]
            return c
        _loop('inv', 0, PB, inv)

    pl.run_scoped(s4_fwd, pltpu.VMEM((5, NJ, 128), F32), pltpu.VMEM((CB, D), F32),
                  pltpu.VMEM((CB, D), F32), pltpu.VMEM((CB, D), F32), pltpu.VMEM((2, 16, 64, 128), F32),
                  pltpu.VMEM((NJ, D), BF))

    def gmlp(r2_ref, acc_ref):
        for cp in cin[1:]:
            cp.wait()
        def f1(i, c):
            r = _rows(i)
            hn, _ = _ln(h_ref[r, :])
            a = _dot(hn.astype(BF), win_ref[...]).astype(BF)
            a_ref[r, :] = a
            z2n, rr = _ln(_gelu(a[:, FH:].astype(F32)).astype(BF).astype(F32))
            z2_ref[r, :] = z2n.astype(BF)
            r2_ref[r, :] = rr
            return c
        _loop('f1', 0, NT, f1)
        acc_ref[...] = jnp.zeros(acc_ref.shape, F32)

        def f2(i, c):
            r = _rows(i, 128)
            g = (_dot(wsp_ref[r, :], z2_ref[...]) + bsp_ref[r, :].astype(F32)).astype(BF).astype(F32)
            a1 = a_ref[r, 0:FH].astype(F32)
            z1 = _gelu(a1).astype(BF).astype(F32)
            q = (z1 * g).astype(BF)
            out_ref[:, r] = (h_ref[r, :] + _dot_nt(q, wout_ref[...])).T.astype(BF)
            dot_ = dot_ref[:, r]
            do = dot_.astype(F32).T.astype(BF)
            do_ref[r, :] = do
            dq = _dot(do, wout_ref[...])
            acc_ref[...] += _dot(dot_, q)
            dg = (dq * z1).astype(BF)
            g_ref[r, :] = dg
            dbsp_ref[r, :] = jnp.sum(dg.astype(F32), axis=1, keepdims=True).astype(BF)
            a_ref[r, 0:FH] = (dq * g * _dgelu(a1)).astype(BF)
            return c
        _loop('f2', 0, L // 128, f2)
        dwout_ref[...] = acc_ref[...].astype(BF)
        cout[0].start()
        cout[2].start()

        def f3(i, c):
            r = _rows(i)
            dz2n = _dot(wsp_ref[:, r].astype(F32).T.astype(BF), g_ref[...])
            dz2 = _lnb(dz2n, z2_ref[r, :].astype(F32), r2_ref[r, :])
            a_ref[r, FH:FF] = (dz2 * _dgelu(a_ref[r, FH:FF].astype(F32))).astype(BF)
            return c
        _loop('f3', 0, NT, f3)

        def f6(i, c):
            r = _rows(i)
            hn, rh = _ln(h_ref[r, :])
            dhn = _dot_nt(a_ref[r, :], win_ref[...])
            h_ref[r, :] = do_ref[r, :].astype(F32) + _lnb(dhn, hn.astype(BF).astype(F32), rh)
            do_ref[r, :] = hn.astype(BF)
            return c
        _loop('f6', 0, NT, f6)

        def dwsp(i, c):
            r = _rows(i)
            dwsp_ref[r, :] = _dot_nt(g_ref[r, :], z2_ref[...]).astype(BF)
            return c
        _loop('dwsp', 0, NT, dwsp)
        cout[1].start()

        def dwin(i, c):
            cs = pl.ds(pl.multiple_of(i * 512, 512), 512)
            dwin_ref[:, cs] = _dot_tn(do_ref[...], a_ref[:, cs]).astype(BF)
            return c
        _loop('dwin', 0, FF // 512, dwin)
        cout[3].start()

    pl.run_scoped(gmlp, pltpu.VMEM((L, 1), F32), pltpu.VMEM((D, FH), F32))

    def s4_bwd(dyf_ref, dk_ref, dsum_ref, zr_ref, zi_ref, car_ref):
        ff, fi = _dft_mats()
        dsum_ref[...] = jnp.zeros(dsum_ref.shape, F32)

        def cast(i, c):
            r = _rows(i, CB)
            dh = h_ref[r, :]
            dyf_ref[i] = _dot(ff, dh.astype(BF)).astype(BF)
            dsum_ref[...] += jnp.sum(dh * u_ref[r, :].astype(F32), axis=0, keepdims=True)
            return c
        _loop('cast', 0, PB, cast)
        ddsk_ref[...] = dsum_ref[...].astype(BF)

        def corr(rr, ref):
            zr_ref[...] = jnp.zeros(zr_ref.shape, F32)
            zi_ref[...] = jnp.zeros(zi_ref.shape, F32)

            def mac(j, cc):
                yr, yi = dyf_ref[rr + j, 0:CB, :].astype(F32), dyf_ref[rr + j, CB:2 * CB, :].astype(F32)
                kr, ki = ref[j, 0:CB, :].astype(F32), ref[j, CB:2 * CB, :].astype(F32)
                zr_ref[...] += yr * kr + yi * ki
                zi_ref[...] += yi * kr - yr * ki
                return cc
            lax.fori_loop(0, PB - rr, mac, 0)
            z = jnp.concatenate([zr_ref[...].astype(BF), zi_ref[...].astype(BF)], 0)
            yy = _dot(fi, z) * (1.0 / CB)
            res = yy[0:CB] + car_ref[...]
            car_ref[...] = -yy[CB:2 * CB]
            return res

        def inv_dk(i, c):
            rr = PB - 1 - i
            r = _rows(rr, CB)
            dk = corr(rr, uf_ref)
            dkh = dk.astype(BF)
            dk_ref[r, 0:D] = dkh
            dk_ref[r, DP:DP + D] = (dk - dkh.astype(F32)).astype(BF)
            return c

        def inv_du(i, c):
            rr = PB - 1 - i
            r = _rows(rr, CB)
            dh = h_ref[r, :]
            du = corr(rr, kf_ref) + dh * dsk
            u, rx = _ln(x_ref[r, :].astype(F32))
            dx_ref[:, r] = (dh + _lnb(du, u.astype(BF).astype(F32), rx)).T.astype(BF)
            return c
        dk_ref[:, D:DP] = jnp.zeros((L, DP - D), BF)
        dk_ref[:, DP + D:2 * DP] = jnp.zeros((L, DP - D), BF)
        car_ref[...] = jnp.zeros(car_ref.shape, F32)
        _loop('inv_dk', 0, PB, inv_dk)
        car_ref[...] = jnp.zeros(car_ref.shape, F32)
        _loop('inv_du', 0, PB, inv_du)
        cout[4].start()

        for i, (l0, l1) in enumerate(((0, 128), (128, 256), (256, 512), (384, 1024), (896, 2048), (1920, 2048))):
            w = l1 - l0
            lj = _lval(lax.broadcasted_iota(jnp.int32, (128, w), 0) + i * 128)
            lr = (lax.broadcasted_iota(jnp.int32, (128, w), 1) + l0).astype(F32)
            mt = (lr.astype(BF).astype(F32) == lj).astype(BF)
            gg = _dot(mt, dk_ref[l0:l1, :])
            gg = gg[:, 0:DP] + gg[:, DP:2 * DP]
            g1 = gg * lj[:, 0:1]
            for c5 in range(5):
                gp_ref[0, c5, i * 128:(i + 1) * 128, :] = gg[:, c5 * 128:(c5 + 1) * 128]
                gp_ref[1, c5, i * 128:(i + 1) * 128, :] = g1[:, c5 * 128:(c5 + 1) * 128]

    pl.run_scoped(s4_bwd, pltpu.VMEM((PB, 2 * CB, D), BF),
                  pltpu.VMEM((L, 2 * DP), BF), pltpu.VMEM((1, D), F32), pltpu.VMEM((CB, D), F32),
                  pltpu.VMEM((CB, D), F32), pltpu.VMEM((CB, D), F32))

    def ssm_bwd(ddt_ref, yt_ref):
        ddt_ref[...] = jnp.zeros(ddt_ref.shape, F32)

        def chunk(c, cc):
            ns = pl.ds(pl.multiple_of((c % 4) * 32, 32), 32)
            ds_ = pl.ds(pl.multiple_of((c // 4) * 128, 128), 128)
            pr = jnp.ones((32, 128), F32)
            z = jnp.zeros((32, 128), F32)
            st = (pr, z, z, z, z, z)
            for (j0, j1, p) in SEGS:
                mr = mul_ref[p, 0, ns, ds_]
                mi = mul_ref[p, 1, ns, ds_]
                yr, yi = jnp.ones((32, 128), F32), jnp.zeros((32, 128), F32)
                for o in range(16):
                    yt_ref[0, o] = yr
                    yt_ref[1, o] = yi
                    yr, yi = yr * mr - yi * mi, yr * mi + yi * mr

                def step(j, carry, yr=yr, yi=yi):
                    pr, pi_, s0r, s0i, s1r, s1i = carry
                    js = pl.ds(pl.multiple_of(j * 16, 16), 16)
                    g0t = gp_ref[0, c // 4, js, :]
                    g1t = gp_ref[1, c // 4, js, :]
                    t0r = t0i = t1r = t1i = None
                    for o in range(16):
                        g0 = g0t[o:o + 1, :]
                        g1 = g1t[o:o + 1, :]
                        a_, b_ = yt_ref[0, o], yt_ref[1, o]
                        if o == 0:
                            t0r, t0i, t1r, t1i = g0 * a_, g0 * b_, g1 * a_, g1 * b_
                        else:
                            t0r, t0i = t0r + g0 * a_, t0i + g0 * b_
                            t1r, t1i = t1r + g1 * a_, t1i + g1 * b_
                    return (pr * yr - pi_ * yi, pr * yi + pi_ * yr,
                            s0r + pr * t0r - pi_ * t0i, s0i + pr * t0i + pi_ * t0r,
                            s1r + pr * t1r - pi_ * t1i, s1i + pr * t1i + pi_ * t1r)
                st = lax.fori_loop(j0, j1, step, st)
            _, _, s0r, s0i, s1r, s1i = st
            dtc = jnp.exp(ldt_ref[:, ds_].astype(F32)).astype(BF).astype(F32)
            ar, ai = are_ref[ns, ds_].astype(F32), aim_ref[ns, ds_].astype(F32)
            b_r, b_i = bre_ref[ns, ds_].astype(F32), bim_ref[ns, ds_].astype(F32)
            cr, ci = cre_ref[ns, ds_].astype(F32), cim_ref[ns, ds_].astype(F32)
            br, bi = dtc * b_r, dtc * b_i
            dcre_ref[ns, ds_] = (s0r * br - s0i * bi)
            dcim_ref[ns, ds_] = (-(s0r * bi + s0i * br))
            dbr = cr * s0r - ci * s0i
            dbi = -(cr * s0i + ci * s0r)
            dbre_ref[ns, ds_] = (dtc * dbr)
            dbim_ref[ns, ds_] = (dtc * dbi)
            wr = cr * br - ci * bi
            wi = cr * bi + ci * br
            dlr = wr * s1r - wi * s1i
            dli = -(wr * s1i + wi * s1r)
            dare_ref[ns, ds_] = (dtc * dlr)
            daim_ref[ns, ds_] = (dtc * dli)
            ddt_ref[:, ds_] += jnp.sum(dlr * ar + dli * ai + dbr * b_r + dbi * b_i, axis=0, keepdims=True)
            return cc
        _loop('chunkb', 0, 20, chunk)
        dldt_ref[...] = (ddt_ref[...] * dt).astype(BF)
        for i, ref in enumerate((dare_o, daim_o, dbre_o, dbim_o, dcre_o, dcim_o)):
            ref[...] = gsc_ref[i, :, 0:D].T.astype(BF)
    pl.run_scoped(ssm_bwd, pltpu.VMEM((1, DP), F32), pltpu.VMEM((2, 16, 32, 128), F32))
    for cp in cout:
        cp.wait()


@jax.jit
def pallas_sequential_preLN__ssm_conv_s4__mixer_gmlp__prompt_kernel(
    A_u: jax.Array,
    A_A_re: jax.Array,
    A_A_im: jax.Array,
    A_B_re: jax.Array,
    A_B_im: jax.Array,
    A_C_re: jax.Array,
    A_C_im: jax.Array,
    A_log_dt: jax.Array,
    A_Dskip: jax.Array,
    B_x: jax.Array,
    B_w_in: jax.Array,
    B_w_sp: jax.Array,
    B_b_sp: jax.Array,
    B_w_out: jax.Array,
    grad_out: jax.Array,
):
    args = (A_u[0].T, grad_out[0].T, A_A_re, A_A_im, A_B_re, A_B_im, A_C_re, A_C_im,
            jnp.pad(A_log_dt[None, :], ((0, 0), (0, DP - D))), A_Dskip[None, :],
            B_w_in, B_w_sp, B_b_sp[:, None], B_w_out.T)
    sds = lambda *s: jax.ShapeDtypeStruct(s, BF)
    out_shape = (sds(D, L), sds(D, L), sds(D, N), sds(D, N), sds(D, N), sds(D, N), sds(D, N), sds(D, N),
                 sds(1, DP), sds(1, D), sds(D, FF), sds(L, L), sds(L, 1), sds(D, FH))
    vm = pl.BlockSpec(memory_space=pltpu.VMEM)
    an = pl.BlockSpec(memory_space=pl.ANY)
    res = pl.pallas_call(
        _kernel,
        in_specs=[an, an] + [vm] * 8 + [an, an, vm, an],
        out_specs=(an, an) + (vm,) * 8 + (an, an, vm, an),
        out_shape=out_shape,
        scratch_shapes=[pltpu.VMEM((PB, 2 * CB, D), BF), pltpu.VMEM((PB, 2 * CB, D), BF), pltpu.VMEM((L, D), F32),
                        pltpu.VMEM((4, 2, N, DP), F32), pltpu.VMEM((2, 5, NJ, 128), F32),
                        pltpu.VMEM((D, FF), BF),
                        pltpu.VMEM((L, L), BF), pltpu.VMEM((D, FH), BF),
                        pltpu.VMEM((D, L), BF), pltpu.VMEM((D, L), BF), pltpu.VMEM((D, FH), BF),
                        pltpu.VMEM((L, D), BF), pltpu.VMEM((L, D), BF), pltpu.VMEM((L, D), BF),
                        pltpu.VMEM((L, FF), BF), pltpu.VMEM((L, FH), BF), pltpu.VMEM((L, FH), BF),
                        pltpu.VMEM((6, N, DP), F32), pltpu.VMEM((6, N, DP), F32),
                        pltpu.SemaphoreType.DMA((10,))],
        compiler_params=pltpu.CompilerParams(vmem_limit_bytes=120 * 1024 * 1024),
    )(*args)
    (out, dx, dare, daim, dbre, dbim, dcre, dcim, dldt, ddsk, dwin, dwsp, dbsp, dwout) = res
    return (out.T[None], dx.T[None], dare, daim, dbre, dbim, dcre, dcim,
            dldt[0, :D], ddsk[0], dwin, dwsp, dbsp[:, 0], dwout.T)
```
